```python
import jax
import jax.numpy as jnp

def _softmax(x, axis=-1):
    return jax.nn.softmax(x, axis=axis)
def _gelu(x):
    return jax.nn.gelu(x, approximate=True)
def _silu(x):
    return jax.nn.silu(x)
def _sigmoid(x):
    return jax.nn.sigmoid(x)
def _layernorm(x, axis=-1, eps=1e-5):
    m = jnp.mean(x, axis=axis, keepdims=True)
    v = jnp.var(x, axis=axis, keepdims=True)
    return (x - m) / jnp.sqrt(v + eps)
def _scatter_add(tgt, idx, src, axis=0):
    return tgt.at[idx].add(src)
def _segment_sum(src, seg, n):
    return jax.ops.segment_sum(src, seg, n)
class _Rng:
    def __init__(self, key):
        self._k = key
    def _next(self):
        self._k, sub = jax.random.split(self._k)
        return sub
    def normal(self, shape):
        return jax.random.normal(self._next(), shape, dtype=jnp.bfloat16)
    def randint(self, lo, hi, shape):
        return jax.random.randint(self._next(), shape, lo, hi, dtype=jnp.int32)
    def uniform(self, shape, lo=0.0, hi=1.0):
        return jax.random.uniform(self._next(), shape, jnp.bfloat16, lo, hi)
    def permutation(self, n):
        return jax.random.permutation(self._next(), n)


kernel_name = 'standalone__adm_resblock__diffusion'

def setup_inputs():
    _rng = _Rng(jax.random.key(int.from_bytes(__import__("os").urandom(4), "little")))
    _w = (lambda a: (lambda t: t.astype(jnp.bfloat16) if jnp.issubdtype(t.dtype, jnp.floating) else t)(jnp.asarray(a)))
    B, C, HW, E = 2, 512, 64, 1152
    sc = (9.0 * C) ** -0.5
    return {
        "x": _w((lambda *s: _rng.normal(s) * 0.05)(B, C, HW, HW)),
        "t_emb": _w((lambda *s: _rng.normal(s) * 0.05)(B, E)),
        "g1": _w(1.0 + 0.1 * (lambda *s: _rng.normal(s) * 0.05)(C)),
        "be1": _w(0.1 * (lambda *s: _rng.normal(s) * 0.05)(C)),
        "w1": _w((lambda *s: _rng.normal(s) * 0.05)(C, C, 3, 3) * sc),
        "w_emb": _w((lambda *s: _rng.normal(s) * 0.05)(E, C) * (E ** -0.5)),
        "g2": _w(1.0 + 0.1 * (lambda *s: _rng.normal(s) * 0.05)(C)),
        "be2": _w(0.1 * (lambda *s: _rng.normal(s) * 0.05)(C)),
        "w2": _w((lambda *s: _rng.normal(s) * 0.05)(C, C, 3, 3) * sc),
    }

def reference(x, t_emb, g1, be1, w1, w_emb, g2, be2, w2):
    B, C, H, W = x.shape
    G, eps = 4, 1e-5
    def gn(z, gamma, beta):
        zr = z.reshape(B, G, (C // G) * H * W)
        mu = zr.mean(-1).reshape(B, G, 1)
        var = ((zr - mu) ** 2).mean(-1).reshape(B, G, 1)
        zn = ((zr - mu) / jnp.sqrt(var + eps)).reshape(B, C, H, W)
        return zn * gamma.reshape(1, C, 1, 1) + beta.reshape(1, C, 1, 1)
    def conv3(z, w):
        zp = jnp.pad(z, ((0, 0), (0, 0), (1, 1), (1, 1)))
        taps = [jnp.einsum("bchw,oc->bohw", zp[:, :, i:i+H, j:j+W], w[:, :, i, j]) for i in range(3) for j in range(3)]
        out = taps[0]
        for t in taps[1:]:
            out = out + t
        return out
    h = conv3(_silu(gn(x, g1, be1)), w1)
    emb = _silu(t_emb) @ w_emb
    h = h + emb.reshape(B, C, 1, 1)
    h = conv3(_silu(gn(h, g2, be2)), w2)
    return x + h
```

```python
import functools

import jax
import jax.numpy as jnp
from jax.experimental import pallas as pl
from jax.experimental.pallas import tpu as pltpu

F32, BF16, U32 = jnp.float32, jnp.bfloat16, jnp.uint32

NB, C, HW, NG = 2, 512, 64, 4
EPS = 1e-5
TR = 8
M = 16 * TR
TOK = 16
M_PITCH = M + 16
T_ROWS, T_PITCH = 33, 13
TICKS = M // 8

PA, PB = 2.0 / 3.0, 1.5
A2, B2 = PA * PA, PB * PB
DD = A2 - B2


def _xf_in(d):
    p2, q2 = B2 * d[2], A2 * d[2]
    ea, eb = d[4] - p2, d[4] - q2
    p3, q3 = A2 * d[3], B2 * d[3]
    ua, ub = d[1] - p3, d[1] - q3
    v0 = (ea if d[0] is None else d[0] + ea) - q2
    v5 = (ua if d[5] is None else d[5] + ua) - q3
    oa, ob = PB * ua, PA * ub
    return [v0, ea - oa, ea + oa, eb - ob, eb + ob, v5]


def _xf_out(m):
    sa, da, sb, db = m[1] + m[2], m[1] - m[2], m[3] + m[4], m[3] - m[4]
    return [m[0] + sa + sb, PA * da + PB * db, A2 * sa + B2 * sb,
            (PA ** 3) * da + (PB ** 3) * db + m[5]]


def _xf_w(g):
    t = g[2] * (1.0 / (2 * DD))
    ea = g[0] * (1.0 / (2 * A2 * DD)) + t
    eb = g[0] * (-1.0 / (2 * B2 * DD)) - t
    oa, ob = g[1] * (PA / (2 * A2 * DD)), g[1] * (-PB / (2 * B2 * DD))
    return [g[0], ea + oa, ea - oa, eb + ob, eb - ob, g[2]]


def _unpack(w, half):
    return pltpu.unpack_elementwise(w, index=half, packed_dtype=BF16, unpacked_dtype=F32)


def _pack(lo, hi):
    return pltpu.pack_elementwise([lo, hi], packed_dtype=BF16)


def _vreg(i):
    return pl.ds(TOK + 8 * i, 8)


def _mean_all(v):
    return jnp.sum(jnp.sum(v, axis=0, keepdims=True), axis=1, keepdims=True) * (1.0 / v.size)


class _Item:
    def __init__(self, cost, src, dst, fn):
        self.cost, self.src, self.dst, self.fn = cost, src, dst, fn


class _Pacer:
    def __init__(self, zero):
        self.at = pl.multiple_of(zero * 8, 8)

    def release(self, buf, value):
        if value.dtype != buf.dtype:
            value = pltpu.bitcast(value, buf.dtype)
        buf[pl.ds(self.at, 8), pl.ds(0, 128)] = value

    def done(self, buf):
        return buf[pl.ds(self.at + 8, 8), pl.ds(0, 128)]


def _merge(streams):
    keyed = []
    for groups, lo, hi in streams:
        total = sum(it.cost for grp in groups for it in grp)
        acc = 0
        for grp in groups:
            cost = sum(it.cost for it in grp)
            keyed.append((lo + (hi - lo) * (acc + cost / 2) / total, len(keyed), grp))
            acc += cost
    keyed.sort(key=lambda t: t[:2])
    return [it for _, _, grp in keyed for it in grp]


def _kernel(cfg, x_hbm, t_hbm, g1_hbm, be1_hbm, w1_hbm, wemb_hbm, g2_hbm, be2_hbm, w2_hbm, o_hbm,
            xs0, xs1, h0, h1, wr1, wr2, u1, u2, v0, v1, m0, m1, tb, ws, osb, coef, stat,
            t_s, g1_s, be1_s, g2_s, be2_s, wemb_s, emb_s, sems):
    xs_bf, wr_bf = (xs0, xs1), (wr1, wr2)
    xs = tuple(r.bitcast(U32) for r in xs_bf)
    wr = tuple(r.bitcast(U32) for r in wr_bf)
    hs, us, vs, ms = (h0, h1), (u1, u2), (v0, v1), (m0, m1)
    gammas, betas = (g1_s, g2_s), (be1_s, be2_s)
    part = functools.partial

    n_sem = [0]

    def copy(src, dst):
        n_sem[0] += 1
        return pltpu.make_async_copy(src, dst, sems.at[n_sem[0] - 1])

    def x_copy(b, g, r0, nr):
        return copy(x_hbm.at[b, pl.ds(r0 * HW, nr * HW), pl.ds(g * 128, 128)],
                    xs_bf[b].at[pl.ds(2 * TOK + (g * HW + r0) * HW, nr * HW)])

    def w_copy(cv, n, g):
        return copy((w1_hbm, w2_hbm)[cv].at[:, pl.ds(n * 128, 128), pl.ds(g * 128, 128)],
                    wr_bf[cv].at[pl.ds(1 + g * 9, 9), pl.ds(n * 128, 128)])

    xp = cfg["x_pieces"]
    xr = HW // xp
    small = [copy(s, d) for s, d in ((g1_hbm, g1_s), (be1_hbm, be1_s), (g2_hbm, g2_s), (be2_hbm, be2_s),
                                     (t_hbm, t_s))]
    w_dma = {(cv, n, g): w_copy(cv, n, g) for cv in range(2) for n in range(NG) for g in range(NG)}
    x0_dma = {(g, q): x_copy(0, g, q * xr, xr) for g in range(NG) for q in range(xp)}
    x1_dma = [x_copy(1, g, 0, HW) for g in range(NG)]
    wemb_dma = copy(wemb_hbm, wemb_s)
    first = []
    for g in range(NG):
        first += [w_dma[0, 0, g]] + [x0_dma[g, q] for q in range(xp)]
    for d in first[:1] + small + first[1:]:
        d.start()
    for d in ([w_dma[0, n, g] for n in range(1, NG) for g in range(NG)] + x1_dma + [wemb_dma]
              + [w_dma[1, n, g] for n in range(NG) for g in range(NG)]):
        d.start()

    zero = jax.lax.fori_loop(0, 2, lambda i, z: z + (i >> 10), jnp.int32(0))
    pace = _Pacer(zero)
    wr_tok = tuple(r.at[0] for r in wr)
    for buf in (*xs, *hs, *wr_tok, *us, *vs, *ms, tb, ws, osb):
        buf[pl.ds(0, TOK), pl.ds(0, 128)] = jnp.zeros((TOK, 128), buf.dtype)

    sub = jax.lax.broadcasted_iota(jnp.int32, (8, 128), 0)

    def w_first(cv, n, g, ob, j, slot):
        w = [wr[cv][1 + g * 9 + 3 * i + j, pl.ds(n * 64 + ob * 8, 8)] for i in range(3)]
        for half in range(2):
            c = _xf_w([_unpack(wi, half) for wi in w])
            for xi in range(6):
                ws[_vreg(slot * 36 + xi * 6 + half * 3 + j)] = c[xi]

    def w_second(cv, n, g, ob, xi, slot):
        u = [_xf_w([ws[_vreg(slot * 36 + xi * 6 + half * 3 + j)] for j in range(3)]) for half in range(2)]
        for nu in range(6):
            row = TOK + ((n * 36 + xi * 6 + nu) * 8 + ob) * 8
            us[cv][pl.ds(row, 8), pl.ds(g * 128, 128)] = _pack(u[0][nu], u[1][nu])

    def w_groups(units):
        out = []
        for q in range(len(units) + 1):
            if q < len(units):
                cv, n, g, ob = units[q]
                grp = [_Item(0, None, None, w_dma[cv, n, g].wait)] if ob == 0 else []
                out.append(grp + [_Item(cfg["c_w1"], wr_tok[cv], ws, part(w_first, *units[q], j, q % 2))
                                  for j in range(3)])
            if q > 0:
                for x0 in (0, 3):
                    out.append([_Item(cfg["c_w2"], ws, us[units[q - 1][0]],
                                      part(w_second, *units[q - 1], xi, (q - 1) % 2))
                                for xi in range(x0, x0 + 3)])
        return out

    def x_words(b, g, h):
        return [xs[b][pl.ds(TOK + (g * HW + h) * 32 + jp, 8, stride=4)] for jp in range(4)]

    def set_coef(cv, b, g, mean, var, bias):
        gamma = gammas[cv][...].astype(F32)[g * 128:(g + 1) * 128][None, :]
        beta = betas[cv][...].astype(F32)[g * 128:(g + 1) * 128][None, :]
        mu = _mean_all(mean)
        dev = mean - mu
        var = _mean_all(jnp.maximum(var, 0.0) + dev * dev)
        scale = gamma * jax.lax.rsqrt(var + EPS)
        shift = beta + (bias - mu) * scale
        k = ((cv * NB + b) * NG + g) * 2
        coef[k] = jnp.broadcast_to(0.5 * scale, (8, 128))
        coef[k + 1] = jnp.broadcast_to(0.5 * shift, (8, 128))

    def x_stat_rows(acc, b, g, r0, nr):
        base = TOK + (g * HW + r0) * 32
        for q in range(nr * 4):
            w = xs[b][pl.ds(base + 8 * q, 8)]
            lo, hi = _unpack(w, 0), _unpack(w, 1)
            if not acc:
                acc.update(ref=lo, s1=[None, None], s2=[None, None])
            lo, hi = lo - acc["ref"], hi - acc["ref"]
            for key, val in (("s1", lo + hi), ("s2", lo * lo + hi * hi)):
                old = acc[key][q % 2]
                acc[key][q % 2] = val if old is None else old + val
        stat[_vreg(2 * NB * NG)] = acc["s2"][0]

    def x_stat_end(acc, b, g):
        inv = 1.0 / (HW * 8)
        m1, m2 = (acc["s1"][0] + acc["s1"][1]) * inv, (acc["s2"][0] + acc["s2"][1]) * inv
        set_coef(0, b, g, acc["ref"] + m1, m2 - m1 * m1, 0.0)

    def x_stat_groups(b, g, waits):
        acc, out, nr = {}, [], cfg["stat_rows"]
        for r0 in range(0, HW, nr):
            grp = [_Item(0, None, None, waits.pop(r0).wait)] if r0 in waits else []
            out.append(grp + [_Item(40 * nr, xs[b], stat, part(x_stat_rows, acc, b, g, r0, nr))])
        out.append([_Item(30, None, None, part(x_stat_end, acc, b, g))])
        return out

    def h_stat_end(b, g):
        inv = 1.0 / (HW * 8)
        m1, m2 = stat[_vreg((b * NG + g) * 2)] * inv, stat[_vreg((b * NG + g) * 2 + 1)] * inv
        e = emb_s[pl.ds(b, 1), pl.ds(g * 128, 128)]
        set_coef(1, b, g, m1 + e, m2 - m1 * m1, e)

    def time_emb():
        wemb_dma.wait()
        t = t_s[...].astype(F32)
        emb_s[...] = jnp.dot((t * jax.nn.sigmoid(t)).astype(BF16), wemb_s[...], preferred_element_type=F32)

    def t_vreg(g, h, nu, p):
        return _vreg((g * T_ROWS + h % T_ROWS) * T_PITCH + nu * 2 + p)

    def in_row(cv, b, g, h):
        k = ((cv * NB + b) * NG + g) * 2
        scale, shift = coef[k], coef[k + 1]
        if cv == 0:
            z = [_unpack(w, half) for w in x_words(b, g, h) for half in range(2)]
        else:
            z = [hs[b][_vreg((h * NG + g) * 8 + j)] for j in range(8)]
        a = []
        for zj in z:
            u = zj * scale + shift
            a.append(u + u * jnp.tanh(u))
        left = jnp.where(sub == 0, 0.0, pltpu.roll(a[7], 1, 0))
        right = jnp.where(sub == 7, 0.0, pltpu.roll(a[0], 7, 0))
        cols = [left] + a + [right]
        for p in range(2):
            v = _xf_in(cols[4 * p:4 * p + 6])
            for nu in range(6):
                tb[t_vreg(g, h, nu, p)] = v[nu]

    def in_col(vn, g, r, nu):
        rows = range(4 * r - 1, 4 * r + 5)
        v = [_xf_in([tb[t_vreg(g, h, nu, p)] if 0 <= h < HW else None for h in rows]) for p in range(2)]
        for xi in range(6):
            row = TOK + ((xi * 6 + nu) * TR + r % TR) * 8
            vn[pl.ds(row, 8), pl.ds(g * 128, 128)] = _pack(v[0][xi], v[1][xi])

    def in_groups(c, g):
        cv, b, r0 = c // 4, (c // 2) % 2, (c % 2) * TR
        src, cost = (xs[b], cfg["c_rowx"]) if cv == 0 else (hs[b], cfg["c_rowh"])
        row = lambda h: [_Item(cost, src, tb, part(in_row, cv, b, g, h))]
        out = [row(0)] if r0 == 0 else []
        for r in range(r0, r0 + TR + 1):
            rows = [row(h) for h in range(4 * r + 1, min(4 * r + 5, HW))] if r < r0 + TR else []
            cols = [[_Item(cfg["c_col"], tb, vs[c % 2], part(in_col, vs[c % 2], g, r - 1, nu))]
                    for nu in range(6)] if r > r0 else []
            while rows or cols:
                if rows:
                    out.append(rows.pop(0))
                if cols:
                    out.append(cols.pop(0))
                if cols and len(rows) % 2 == 0:
                    out.append(cols.pop(0))
        return out

    def out_first(mp, r, p, xis, slot):
        for xi in xis:
            y = _xf_out([mp[pl.ds(TOK + (xi * 6 + nu) * M_PITCH + 16 * (r % TR) + p, 8, stride=2)]
                         for nu in range(6)])
            for j in range(4):
                osb[_vreg(slot * 24 + j * 6 + xi)] = y[j]

    def out_second(acc, cv, b, n, r, p, jp, slot):
        y = [_xf_out([osb[_vreg(slot * 24 + j * 6 + xi)] for xi in range(6)]) for j in (2 * jp, 2 * jp + 1)]
        for i in range(4):
            h = 4 * r + i
            if cv == 0:
                for q in range(2):
                    hs[b][_vreg((h * NG + n) * 8 + 4 * p + 2 * jp + q)] = y[q][i]
            else:
                at = pl.ds(TOK + (n * HW + h) * 32 + 2 * p + jp, 8, stride=4)
                w = xs[b][at]
                xs[b][at] = _pack(_unpack(w, 0) + y[0][i], _unpack(w, 1) + y[1][i])
        if cv == 0:
            for q in range(2):
                yq = y[q]
                acc[0] = acc[0] + ((yq[0] + yq[1]) + (yq[2] + yq[3]))
                acc[1] = acc[1] + ((yq[0] * yq[0] + yq[1] * yq[1]) + (yq[2] * yq[2] + yq[3] * yq[3]))

    out_dmas = []

    def out_groups(c, n):
        cv, b, r0 = c // 4, (c // 2) % 2, (c % 2) * TR
        mp, acc, k = ms[n % 2], [], (b * NG + n) * 2

        def begin():
            for q in range(2):
                acc.append(stat[_vreg(k + q)] if r0 else jnp.zeros((8, 128), F32))

        def end():
            for q in range(2):
                stat[_vreg(k + q)] = acc[q]

        def send(h0, nr):
            out_dmas.append(copy(xs_bf[b].at[pl.ds(2 * TOK + (n * HW + h0) * HW, nr * HW)],
                                 o_hbm.at[b, pl.ds(h0 * HW, nr * HW), pl.ds(n * 128, 128)]))
            out_dmas[-1].start()

        units = [(r, p) for r in range(r0, r0 + TR) for p in range(2)]
        send_rows = cfg["last_send"] if (c, n) == (7, NG - 1) else TR
        out = [[_Item(0, None, None, begin)]] if cv == 0 else []
        for q in range(len(units) + 1):
            for part_id in range(2):
                if q < len(units):
                    out.append([_Item(cfg["c_o1"], mp, osb,
                                      part(out_first, mp, *units[q], range(3 * part_id, 3 * part_id + 3), q % 2))])
                if q > 0:
                    out.append([_Item(cfg["c_o2"], osb, (hs, xs)[cv][b],
                                      part(out_second, acc, cv, b, n, *units[q - 1], part_id, (q - 1) % 2))])
            if cv == 1 and q > 0 and q % (2 * send_rows) == 0:
                out[-1].append(_Item(0, None, None, part(send, 4 * (r0 + q // 2 - send_rows), 4 * send_rows)))
        if cv == 0:
            out[-1].append(_Item(0, None, None, end))
        return out

    def matmul(c, n, k, before_block):
        vc = vs[c % 2]
        blocks = []
        for rb in range(TR):
            before_block(vc, 2 * rb)
            blocks.append(vc[pl.ds(TOK + (k * TR + rb) * 8, 8)])
        lhs = pltpu.bitcast(jnp.concatenate(blocks, axis=0), BF16)
        rhs = pltpu.bitcast(us[c // 4][pl.ds(TOK + (n * 36 + k) * 64, 64)], BF16)
        res = jax.lax.dot_general(lhs, rhs, (((1,), (1,)), ((), ())), preferred_element_type=F32)
        ms[n % 2][pl.ds(TOK + k * M_PITCH, M)] = res
        return res

    def run_alone(items, window):
        finished, acc = [], 0
        for it in items:
            ready = [v for t, v in finished if t <= acc - window]
            if it.src is not None and ready:
                pace.release(it.src, ready[-1])
            it.fn()
            acc += it.cost
            if it.dst is not None:
                finished.append((acc, pace.done(it.dst)))
                del finished[:-24]

    clock, pending, todo = [], [], []

    def before_block(vc, dt):
        now = len(clock) * TICKS + dt
        for t, _, value in pending:
            if t <= now:
                pace.release(vc, value)
        pending[:] = [p for p in pending if p[0] > now]

    def advance(tick):
        while todo and len(clock) * TICKS <= tick:
            clock.append(matmul(*todo.pop(0), before_block))

    def run_phase(p, items):
        span, lead, slack, win = 36 * TICKS, cfg["lead"], cfg["slack"], cfg["win"]
        total, acc, last = sum(it.cost for it in items), 0, {}
        for it in items:
            start = p * span + int(acc / total * span) // win * win - lead
            acc += it.cost
            advance(start)
            if it.src is not None and start >= 0 and last.get(id(it.src)) != start:
                last[id(it.src)] = start
                q = start % TICKS
                pace.release(it.src, clock[start // TICKS][8 * q:8 * q + 8])
            it.fn()
            if it.dst is not None:
                due = -(-(p * span + int(acc / total * span) - lead + slack) // 2) * 2
                pending[:] = [e for e in pending if e[:2] != (due, id(it.dst))]
                pending.append((due, id(it.dst), pace.done(it.dst)))

    w_units = lambda cv, n, gs: [(cv, n, g, ob) for g in gs for ob in range(8)]

    head = [[_Item(0, None, None, d.wait) for d in small]]
    for g in range(NG):
        head += w_groups(w_units(0, 0, [g]))
        head += x_stat_groups(0, g, {q * xr: x0_dma[g, q] for q in range(xp)})
        head += in_groups(0, g)
    run_alone([it for grp in head for it in grp], cfg["alone"])

    w2 = [u for n in range(NG) for u in w_units(1, n, range(NG))]
    w2_share = dict(cfg["w2_share"])
    assert sum(w2_share.values()) == len(w2)
    for p in range(32):
        c, n = divmod(p, NG)
        todo.extend((c, n, k) for k in range(36))
        streams = []
        if c < 7:
            lead_in = []
            if c == 1:
                lead_in = x_stat_groups(1, n, {0: x1_dma[n]})
            if c in (3, 5):
                lead_in = [[_Item(30, None, None, part(h_stat_end, (c - 3) // 2, n))]]
            streams.append((lead_in + in_groups(c + 1, n), 0.0, cfg["in_end"] if n == NG - 1 else 1.0))
        if p > 0:
            streams.append((out_groups(*divmod(p - 1, NG)), cfg["out_start"], 1.0))
        if p < NG - 1:
            streams.append((w_groups(w_units(0, n + 1, range(NG))), 0.0, cfg["w_end"]))
        if w2_share.get(p):
            streams.append((w_groups([w2.pop(0) for _ in range(w2_share[p])]), 0.0, cfg["w_end"]))
        if p == cfg["emb_phase"]:
            streams.append(([[_Item(1, None, None, time_emb)]], 0.5, 0.5))
        run_phase(p, _merge(streams))
        advance((p + 1) * 36 * TICKS - 1)
    run_alone([it for grp in out_groups(7, NG - 1) for it in grp], cfg["alone"])
    for d in out_dmas:
        d.wait()


_CFG = dict(
    lead=16, slack=24, win=2, alone=160, in_end=0.95, out_start=0.04, w_end=0.93,
    c_rowx=80, c_rowh=72, c_col=42, c_o1=48, c_o2=56, c_w1=28, c_w2=28,
    x_pieces=2, stat_rows=2, last_send=2, emb_phase=9,
    w2_share=tuple((p, 12) for p in range(8, 16)) + ((16, 12), (17, 12), (18, 8)),
)


def _resblock(cfg, x, t_emb, g1, be1, w1, w_emb, g2, be2, w2):
    assert x.shape == (NB, C, HW, HW) and w1.shape == w2.shape == (C, C, 3, 3)
    emb_dim = t_emb.shape[1]
    vmem = pltpu.VMEM
    scratch = (
        [vmem((2 * TOK + NG * HW * HW, 128), BF16)] * 2
        + [vmem((TOK + HW * NG * 64, 128), F32)] * 2
        + [vmem((1 + NG * 9, C, 128), BF16)] * 2
        + [vmem((TOK + NG * 36 * 64, C), U32)] * 2
        + [vmem((TOK + 36 * M // 2, C), U32)] * 2
        + [vmem((TOK + 36 * M_PITCH, 128), F32)] * 2
        + [vmem((TOK + NG * T_ROWS * T_PITCH * 8, 128), F32),
           vmem((TOK + 2 * 36 * 8, 128), F32),
           vmem((TOK + 2 * 24 * 8, 128), F32),
           vmem((2 * NB * NG * 2, 8, 128), F32),
           vmem((TOK + (2 * NB * NG + 1) * 8, 128), F32),
           vmem((NB, emb_dim), BF16)]
        + [vmem((C,), BF16)] * 4
        + [vmem((emb_dim, C), BF16), vmem((NB, C), F32), pltpu.SemaphoreType.DMA((96,))]
    )
    as_taps = lambda w: jnp.transpose(w, (2, 3, 0, 1)).reshape(9, C, C)
    out = pl.pallas_call(
        functools.partial(_kernel, cfg),
        out_shape=jax.ShapeDtypeStruct((NB, HW * HW, C), x.dtype),
        in_specs=[pl.BlockSpec(memory_space=pl.ANY)] * 9,
        out_specs=pl.BlockSpec(memory_space=pl.ANY),
        scratch_shapes=scratch,
        compiler_params=pltpu.CompilerParams(vmem_limit_bytes=112 * 2 ** 20),
    )(jnp.transpose(x, (0, 2, 3, 1)).reshape(NB, HW * HW, C), t_emb, g1, be1, as_taps(w1), w_emb,
      g2, be2, as_taps(w2))
    return jnp.transpose(out.reshape(NB, HW, HW, C), (0, 3, 1, 2))


@jax.jit
def pallas_standalone__adm_resblock__diffusion_kernel(
    x: jax.Array,
    t_emb: jax.Array,
    g1: jax.Array,
    be1: jax.Array,
    w1: jax.Array,
    w_emb: jax.Array,
    g2: jax.Array,
    be2: jax.Array,
    w2: jax.Array,
):
    return _resblock(_CFG, x, t_emb, g1, be1, w1, w_emb, g2, be2, w2)
```

```python
import functools

import jax
import jax.numpy as jnp
from jax.experimental import pallas as pl
from jax.experimental.pallas import tpu as pltpu

F32, BF16, U32 = jnp.float32, jnp.bfloat16, jnp.uint32

NB, C, HW, NG = 2, 512, 64, 4
EPS = 1e-5
TR = 8
M = 16 * TR
TOK = 16
M_PITCH = M + 16
T_ROWS = 33
TICKS = M // 8
SPAN = 36 * TICKS

PA, PB = 2.0 / 3.0, 1.5
A2, B2, B3 = PA * PA, PB * PB, PB * PB * PB
DD = A2 - B2


def _xf_in(d):
    p2, q2 = B2 * d[2], A2 * d[2]
    ea, eb = d[4] - p2, d[4] - q2
    p3, q3 = A2 * d[3], B2 * d[3]
    ua, ub = d[1] - p3, d[1] - q3
    v0 = (ea if d[0] is None else d[0] + ea) - q2
    v5 = (ua if d[5] is None else d[5] + ua) - q3
    oa, ob = PB * ua, PA * ub
    return [v0, ea - oa, ea + oa, eb - ob, eb + ob, v5]


def _xf_out(m):
    sa, da, sb, db = m[1] + m[2], m[1] - m[2], m[3] + m[4], m[3] - m[4]
    return [(m[0] + sb) + B3 * sa, PB * da + db, sa + PB * sb, (da + m[5]) + B3 * db]


def _xf_w(g):
    ca, cb = PA ** 3 / (2 * A2 * DD), -1.0 / (2 * B2 * DD)
    ea, eb = ca * g[0] + (ca * A2) * g[2], cb * g[0] + (cb * B2) * g[2]
    oa, ob = (ca * PA) * g[1], (cb * PB) * g[1]
    return [g[0], ea + oa, ea - oa, eb + ob, eb - ob, g[2]]


def _unpack(w, half):
    return pltpu.unpack_elementwise(w, index=half, packed_dtype=BF16, unpacked_dtype=F32)


def _pack(lo, hi):
    return pltpu.pack_elementwise([lo, hi], packed_dtype=BF16)


def _mean_all(v):
    return jnp.sum(jnp.sum(v, axis=0, keepdims=True), axis=1, keepdims=True) * (1.0 / v.size)


class _Item:
    def __init__(self, cost, src, dst, fn):
        self.cost, self.src, self.dst, self.fn = cost, src, dst, fn

    def slack(self, cfg):
        return cfg["slack"] + dict(cfg["dslack"]).get(getattr(getattr(self.fn, "func", None), "__name__", ""), 0)


class _Pacer:
    def __init__(self, zero):
        self.zero, self.row = zero, pl.multiple_of(zero * 8, 8)

    def _slot(self, buf, which):
        lanes = pl.ds(0, 128)
        if len(buf.shape) == 2:
            return (pl.ds(self.row + 8 * which, 8), lanes)
        if buf.shape[-2] > 8:
            return (self.zero,) + (0,) * (len(buf.shape) - 3) + (pl.ds(8 * which, 8), lanes)
        return (self.zero,) + (0,) * (len(buf.shape) - 4) + (which, pl.ds(0, 8), lanes)

    def init(self, buf):
        for which in range(2):
            buf[self._slot(buf, which)] = jnp.zeros((8, 128), buf.dtype)

    def release(self, buf, value):
        if value.dtype != buf.dtype:
            value = pltpu.bitcast(value, buf.dtype)
        buf[self._slot(buf, 0)] = value

    def done(self, buf):
        return buf[self._slot(buf, 1)]


def _spread(streams):
    keyed = []
    for groups, lo, hi in streams:
        total = max(sum(it.cost for grp in groups for it in grp), 1)
        acc = 0
        for grp in groups:
            cost = sum(it.cost for it in grp)
            keyed.append((lo + (hi - lo) * (acc + cost / 2) / total, len(keyed), grp))
            acc += cost
    keyed.sort(key=lambda t: t[:2])
    phases = {}
    for time, _, grp in keyed:
        phases.setdefault(int(time // 1), []).extend(grp)
    return phases


def _kernel(cfg, x_hbm, t_hbm, g1_hbm, be1_hbm, w1_hbm, wemb_hbm, g2_hbm, be2_hbm, w2_hbm, o_hbm,
            xs0, xs1, h0, h1, wr1, wr2, u1, u2, v0, v1, tb, ws, osb, coef, stat,
            t_s, g1_s, be1_s, g2_s, be2_s, wemb_s, emb_s, sems, *ms):
    xs_bf, wr_bf = (xs0, xs1), (wr1, wr2)
    xs = tuple(r.bitcast(U32) for r in xs_bf)
    wr = tuple(r.bitcast(U32) for r in wr_bf)
    hs, us, vs = (h0, h1), (u1, u2), (v0, v1)
    gammas, betas = (g1_s, g2_s), (be1_s, be2_s)
    part = functools.partial
    lanes = lambda g: pl.ds(g * 128, 128)

    n_sem = [0]

    def copy(src, dst):
        n_sem[0] += 1
        return pltpu.make_async_copy(src, dst, sems.at[n_sem[0] - 1])

    def x_copy(b, g, r0, nr):
        return copy(x_hbm.at[b, pl.ds(r0 * HW, nr * HW), lanes(g)],
                    xs_bf[b].at[pl.ds(2 * TOK + (g * HW + r0) * HW, nr * HW)])

    def w_copy(cv, n, g):
        return copy((w1_hbm, w2_hbm)[cv].at[:, lanes(n), lanes(g)], wr_bf[cv].at[pl.ds(1 + g * 9, 9), lanes(n)])

    xp = cfg["x_pieces"]
    xr = HW // xp
    small = [copy(s, d) for s, d in ((g1_hbm, g1_s), (be1_hbm, be1_s), (g2_hbm, g2_s), (be2_hbm, be2_s),
                                     (t_hbm, t_s))]
    w_dma = {(cv, n, g): w_copy(cv, n, g) for cv in range(2) for n in range(NG) for g in range(NG)}
    x0_dma = {(g, q): x_copy(0, g, q * xr, xr) for g in range(NG) for q in range(xp)}
    x1_dma = [x_copy(1, g, 0, HW) for g in range(NG)]
    wemb_dma = copy(wemb_hbm, wemb_s)
    first = []
    for what, g in cfg["head"]:
        first += [w_dma[0, 0, g]] if what == "w" else [x0_dma[g, q] for q in range(xp)] if what == "s" else []
    for d in first[:1] + small + first[1:]:
        d.start()
    for d in ([w_dma[0, n, g] for n in range(1, NG) for g in range(NG)] + x1_dma + [wemb_dma]
              + [w_dma[1, n, g] for n in range(NG) for g in range(NG)]):
        d.start()

    pace = _Pacer(jax.lax.fori_loop(0, 2, lambda i, z: z + (i >> 10), jnp.int32(0)))
    for buf in (*xs, *hs, *wr, *us, *vs, *ms, tb, ws, osb, stat):
        pace.init(buf)

    sub = jax.lax.broadcasted_iota(jnp.int32, (8, 128), 0)

    def w_store(cv, n, g, ob, xi0, nxi, c):
        u = [_xf_w(ch) for ch in c]
        for nu in range(6):
            us[cv][pl.ds(1 + n * 36 + nu * 6 + xi0, nxi), pl.ds(ob * 8, 8), lanes(g)] = _pack(u[0][nu], u[1][nu])

    def w_first(cv, n, g, ob, slot):
        w = [wr[cv][pl.ds(1 + g * 9 + 3 * i, 3), pl.ds(n * 64 + ob * 8, 8)] for i in range(3)]
        c = [_xf_w([_unpack(wi, half) for wi in w]) for half in range(2)]
        for half in range(2):
            for xi in (range(1, 5) if cfg["w_direct"] else range(6)):
                ws[1 + slot * 6 + xi, pl.ds(half * 3, 3)] = c[half][xi]
        if cfg["w_direct"]:
            for xi in (0, 5):
                w_store(cv, n, g, ob, xi, 1, [[ch[xi][j:j + 1] for j in range(3)] for ch in c])

    def w_second(cv, n, g, ob, xi0, nxi, slot):
        w_store(cv, n, g, ob, xi0, nxi,
                [[ws[pl.ds(1 + slot * 6 + xi0, nxi), half * 3 + j] for j in range(3)] for half in range(2)])

    w_count = [0]

    def w_groups(cv, n, gs):
        units, out = [(cv, n, g, ob) for g in gs for ob in range(8)], []
        nxi = cfg["w_nxi"]
        for q in range(len(units) + 1):
            slot = w_count[0] % 2
            if q < len(units):
                grp = [_Item(0, None, None, w_dma[units[q][:3]].wait)] if units[q][3] == 0 and (cv, n) == (0, 0) else []
                cost = cfg["c_w1"] + (2 * cfg["c_w2"] if cfg["w_direct"] else 0)
                out.append(grp + [_Item(cost, wr[cv], (ws, us[cv]) if cfg["w_direct"] else ws, part(w_first, *units[q], slot))])
                w_count[0] += 1
            if q > 0:
                out += [[_Item(cfg["c_w2"] * nxi, ws, us[cv], part(w_second, *units[q - 1], xi0, nxi, 1 - slot))]
                        for xi0 in (range(1, 5, nxi) if cfg["w_direct"] else range(0, 6, nxi))]
        return out

    def set_coef(cv, b, g, mean, var, bias):
        gamma = gammas[cv][...].astype(F32)[g * 128:(g + 1) * 128][None, :]
        beta = betas[cv][...].astype(F32)[g * 128:(g + 1) * 128][None, :]
        mu = _mean_all(mean)
        dev = mean - mu
        scale = gamma * jax.lax.rsqrt(_mean_all(jnp.maximum(var, 0.0) + dev * dev) + EPS)
        shift = beta + (bias - mu) * scale
        k = (cv * NB + b) * NG + g
        coef[k, 0] = jnp.broadcast_to(0.5 * shift, (8, 128))
        for q, power in enumerate((0, 0, 1, 1, 1, 1, 2, 2) if cv else (0,)):
            coef[k, 1 + q] = jnp.broadcast_to((0.5 * PB ** power) * scale, (8, 128))

    def x_stat_rows(acc, b, g, r0, nr):
        for r in range(r0, r0 + nr):
            w = xs[b][pl.ds(TOK + (g * HW + r) * 32, 32)].reshape(2, 2, 8, 128)
            lo, hi = _unpack(w, 0), _unpack(w, 1)
            if not acc:
                acc.append(lo[0])
            lo, hi = lo - acc[0], hi - acc[0]
            s1, s2 = lo + hi, lo * lo + hi * hi
            s1, s2 = s1[0] + s1[1], s2[0] + s2[1]
            acc[1:] = [acc[1] + s1, acc[2] + s2] if acc[1:] else [s1, s2]
        stat[0, pl.ds(2, 2)] = acc[1]
        stat[0, pl.ds(4, 2)] = acc[2]

    def x_stat_end(acc, b, g):
        if not acc: return
        ref, m1, m2 = acc[0], acc[1] * (1.0 / (HW * 4)), acc[2] * (1.0 / (HW * 4))
        set_coef(0, b, g, (ref + m1).reshape(16, 128), (m2 - m1 * m1).reshape(16, 128), 0.0)

    def x_stat_groups(b, g, waits):
        acc, out, nr = [], [], cfg["stat_rows"]
        for r0 in range(0, HW, nr):
            grp = [_Item(0, None, None, waits[r0].wait)] if r0 in waits else []
            out.append(grp + [_Item(cfg["c_st"] * nr, xs[b], stat, part(x_stat_rows, acc, b, g, r0, nr))])
        out.append([_Item(30, None, None, part(x_stat_end, acc, b, g))])
        return out

    def h_stat_end(b, g):
        s = stat[1 + b * NG + g]
        inv = 1.0 / (HW * 8)
        m1 = (s[0] + PB * (s[1] + PB * s[2])) * inv
        m2 = (s[3] + B2 * (s[4] + B2 * s[5])) * inv
        e = emb_s[pl.ds(b, 1), lanes(g)]
        set_coef(1, b, g, m1 + e, m2 - m1 * m1, e)

    def time_emb():
        t = t_s[...].astype(F32)
        emb_s[...] = jnp.dot((t * jax.nn.sigmoid(t)).astype(BF16), wemb_s[...], preferred_element_type=F32)

    def silu(z, scale, shift):
        u = z * scale + shift
        return u + u * jnp.tanh(u)

    def in_row(cv, b, g, h):
        k = (cv * NB + b) * NG + g
        if cv == 0:
            at = TOK + (g * HW + h) * 32
            w = jnp.concatenate([xs[b][pl.ds(at + jp, 8, stride=4)] for jp in range(4)]).reshape(2, 2, 8, 128)
            scale, shift = coef[k, 1], coef[k, 0]
            lo, hi = silu(_unpack(w, 0), scale, shift), silu(_unpack(w, 1), scale, shift)
            d = [lo[:, 0], hi[:, 0], lo[:, 1], hi[:, 1]]
        else:
            a = silu(hs[b][1 + h * NG + g], coef[k, pl.ds(1 if h % 4 in (0, 3) else 5, 4)], coef[k, 0])
            d = [a[:, 0], a[:, 2], a[:, 3], a[:, 1]]
        left = jnp.where(sub == 0, 0.0, pltpu.roll(d[3][1], 1, 0))
        right = jnp.where(sub == 7, 0.0, pltpu.roll(d[0][0], 7, 0))
        v = _xf_in([jnp.stack([left, d[3][0]])] + d + [jnp.stack([d[0][1], right])])
        for nu in range(6):
            tb[1 + g * T_ROWS + h % T_ROWS, :, nu] = v[nu]

    def in_col(vn, g, r, nu0, nnu):
        rows = range(4 * r - 1, 4 * r + 5)
        v = [_xf_in([tb[1 + g * T_ROWS + h % T_ROWS, p, pl.ds(nu0, nnu)] if 0 <= h < HW else None for h in rows])
             for p in range(2)]
        for xi in range(6):
            vn[pl.ds(1 + xi * 6 + nu0, nnu), pl.ds(r % TR * 8, 8), lanes(g)] = _pack(v[0][xi], v[1][xi])

    def in_groups(c, g):
        cv, b, r0 = c // 4, (c // 2) % 2, (c % 2) * TR
        src, cost = (xs[b], cfg["c_rowx"]) if cv == 0 else (hs[b], cfg["c_rowh"])
        row = lambda h: [_Item(cost, src, tb, part(in_row, cv, b, g, h))]
        out, nnu = [row(0)] if r0 == 0 else [], cfg["nnu"]
        for r in range(r0, r0 + TR + 1):
            rows = [row(h) for h in range(4 * r + 1, min(4 * r + 5, HW))] if r < r0 + TR else []
            cols = [[_Item(cfg["c_col"] * nnu, tb, vs[c % 2], part(in_col, vs[c % 2], g, r - 1, nu0, nnu))]
                    for nu0 in range(0, 6, nnu)] if r > r0 else []
            out += [grp for _, grp in sorted(
                [((q + 0.25) / len(rows), grp) for q, grp in enumerate(rows)]
                + [((q + 0.75) / len(cols), grp) for q, grp in enumerate(cols)], key=lambda t: t[0])]
        return out

    def out_first(cv, mp, r, p, xi0, nxi, slot):
        y = _xf_out([mp[pl.ds(1 + nu * 6 + xi0, nxi), pl.ds(r % TR * 16 + p, 8, stride=2)] for nu in range(6)])
        for q, j in enumerate((0, 1, 2, 3) if cv else (0, 3, 1, 2)):
            osb[1 + slot * 4 + q, pl.ds(xi0, nxi)] = y[j]

    def out_second(acc, cv, b, n, r, p, jp, slot):
        y = _xf_out([osb[pl.ds(1 + slot * 4 + 2 * jp, 2), xi] for xi in range(6)])
        if not acc: acc.extend(jnp.zeros((8, 128), F32) for q in range(6))
        if cv == 0:
            for i in range(4):
                hs[b][1 + (4 * r + i) * NG + n, p, pl.ds(2 * jp, 2)] = y[i]
            for power, ya, yb in ((jp, y[0], y[3]), (jp + 1, y[1], y[2])):
                s1, s2 = ya + yb, ya * ya + yb * yb
                acc[power] = acc[power] + (s1[0] + s1[1])
                acc[3 + power] = acc[3 + power] + (s2[0] + s2[1])
        else:
            for i in range(4):
                at = pl.ds(TOK + (n * HW + 4 * r + i) * 32 + 2 * p + jp, 8, stride=4)
                w, res = xs[b][at], []
                for q in range(2):
                    power = (i in (1, 2)) + (2 * jp + q in (1, 2))
                    res.append(_unpack(w, q) + (y[i][q] * PB ** power if power else y[i][q]))
                xs[b][at] = _pack(*res)

    out_dmas, os_count = [], [0]

    def out_groups(phase):
        c, n = divmod(phase, NG)
        cv, b, r0 = c // 4, (c // 2) % 2, (c % 2) * TR
        mp, acc, nxi = ms[phase % len(ms)], [], cfg["o_nxi"]

        def begin():
            acc.extend(stat[1 + b * NG + n, q] if r0 else jnp.zeros((8, 128), F32) for q in range(6))

        def end():
            for q in range(6):
                stat[1 + b * NG + n, q] = acc[q]

        def send(h0, nr):
            out_dmas.append(copy(xs_bf[b].at[pl.ds(2 * TOK + (n * HW + h0) * HW, nr * HW)],
                                 o_hbm.at[b, pl.ds(h0 * HW, nr * HW), lanes(n)]))
            out_dmas[-1].start()

        units = [(r, p) for r in range(r0, r0 + TR) for p in range(2)]
        send_rows = cfg["last_send"] if phase == 31 else TR
        out = [[_Item(0, None, None, begin)]] if cv == 0 else []
        for q in range(len(units) + 1):
            slot = os_count[0] % 2
            firsts = [[_Item(cfg["c_o1"] * nxi, mp, osb, part(out_first, cv, mp, *units[q], xi0, nxi, slot))]
                      for xi0 in range(0, 6, nxi)] if q < len(units) else []
            seconds = [[_Item(cfg["c_o2"], osb, (hs, xs)[cv][b],
                              part(out_second, acc, cv, b, n, *units[q - 1], jp, 1 - slot))]
                       for jp in range(2)] if q > 0 else []
            os_count[0] += bool(firsts)
            out += [grp for _, grp in sorted(
                [((k + 0.25) / len(firsts), grp) for k, grp in enumerate(firsts)]
                + [((k + 0.75) / len(seconds), grp) for k, grp in enumerate(seconds)], key=lambda t: t[0])]
            if cv == 1 and q > 0 and q % (2 * send_rows) == 0:
                out[-1].append(_Item(0, None, None, part(send, 4 * (r0 + q // 2 - send_rows), 4 * send_rows)))
        if cv == 0:
            out[-1].append(_Item(0, None, None, end))
        return out

    def matmul(phase, xi, nu, dues):
        c, n = divmod(phase, NG)
        vc = vs[c % 2]
        cuts = sorted({0, TR} | set(dues))
        blocks = []
        for lo, hi in zip(cuts, cuts[1:]):
            for value in dues.get(lo, ()):
                pace.release(vc, value)
            blocks.append(vc[1 + xi * 6 + nu, pl.ds(lo * 8, (hi - lo) * 8)])
        lhs = pltpu.bitcast(jnp.concatenate(blocks, axis=0), BF16)
        rhs = pltpu.bitcast(us[c // 4][1 + n * 36 + nu * 6 + xi], BF16)
        res = jax.lax.dot_general(lhs, rhs, (((1,), (1,)), ((), ())), preferred_element_type=F32)
        ms[phase % len(ms)][1 + nu * 6 + xi, pl.ds(0, M)] = res
        return res

    dsts = lambda it: it.dst if isinstance(it.dst, tuple) else () if it.dst is None else (it.dst,)

    def run_alone(groups, window):
        finished, acc = [], 0
        for it in (it for grp in groups for it in grp):
            ready = [v for t, v in finished if t <= acc - window]
            if it.src is not None and ready:
                pace.release(it.src, ready[-1])
            it.fn()
            acc += it.cost
            for dst in dsts(it):
                finished.append((acc, pace.done(dst)))
            del finished[:-24]

    clock, pending, todo, chain = [], {}, [], []

    def advance(tick):
        while todo and (base + len(clock)) * TICKS <= tick:
            now, dues = (base + len(clock)) * TICKS, {}
            for key in [key for key in pending if key[0] < now + TICKS]:
                dues.setdefault(max(key[0] - now, 0) // 2, []).append(pending.pop(key))
            for rb in range(0, TR if cfg["pop_lag"] else 0, cfg["pop_every"]):
                t = min(now + 2 * rb - cfg["pop_lag"], now - 1)
                if t >= base * TICKS:
                    dues.setdefault(rb, []).append(clock[t // TICKS - base][t % TICKS * 8:t % TICKS * 8 + 8])
            clock.append(matmul(*todo.pop(0), dues))

    def run_phase(p, items):
        lead, slack, win = cfg["lead"], cfg["slack"], cfg["win"]
        total, acc, plan, releases = sum(it.cost for it in items), 0, [], {}
        for it in items:
            start = p * SPAN + int(acc / total * SPAN) // win * win - lead
            acc += it.cost
            plan.append((it, start, -(-(p * SPAN + int(acc / total * SPAN) - lead + it.slack(cfg)) // 2) * 2))
            if it.src is not None and start >= base * TICKS and len(plan) % cfg["clk_every"] == 0:
                releases[start, id(it.src)] = it.src
        for it, start, due in plan:
            for key in [key for key in releases if key[0] <= start + cfg["ahead"]]:
                advance(key[0])
                q = key[0] % TICKS
                pace.release(releases.pop(key), clock[key[0] // TICKS - base][8 * q:8 * q + 8])
            advance(start)
            if cfg["chain"] and it.src is not None and len(chain) >= cfg["chain"]:
                pace.release(it.src, chain[-cfg["chain"]])
            it.fn()
            for dst in dsts(it):
                pending[due, id(dst)] = pace.done(dst)
                chain.append(pending[due, id(dst)])
            del chain[:-32]

    p_lo, p_hi = cfg["only"]
    base = max(p_lo, 0) * 36

    head = [[_Item(0, None, None, d.wait) for d in small]]
    for what, g in cfg["head"]:
        head += (w_groups(0, 0, [g]) if what == "w" else in_groups(0, g) if what == "i" else
                 x_stat_groups(0, g, {q * xr: x0_dma[g, q] for q in range(xp)}))
    if p_lo < 0:
        run_alone(head, cfg["alone"])

    streams = []
    for c in range(1, 8):
        groups = []
        for g in range(NG):
            if c in (4, 6):
                groups.append([_Item(30, None, None, part(h_stat_end, (c - 4) // 2, g))])
            groups += in_groups(c, g)
        streams.append((groups, *cfg["t_in"][c - 1]))
    streams.append(([grp for g in range(NG) for grp in x_stat_groups(1, g, {})], *cfg["t_stat"]))
    w_times = cfg["t_w"]
    for k, (cv, n) in enumerate([(cv, n) for cv in range(2) for n in range(NG)][1:]):
        streams.append((w_groups(cv, n, range(NG)), *w_times[k]))
    t_out = cfg["t_out"]
    for p in range(31):
        assert p + 1 <= t_out[p] and t_out[p + 1] <= p + len(ms)
        streams.append((out_groups(p), t_out[p], t_out[p + 1]))
    streams.append(([[_Item(1, None, None, time_emb)]], cfg["t_emb"], cfg["t_emb"]))
    w_of = lambda cv, ns: [w_dma[cv, n, g] for n in ns for g in range(NG)]
    for time, dmas in ((w_times[0][0], w_of(0, [1])), (w_times[1][0], w_of(0, [2, 3])),
                       (cfg["t_stat"][0], x1_dma), (w_times[3][0], [wemb_dma] + w_of(1, [0, 1])),
                       (cfg["t_w2b"], w_of(1, [2])), (cfg["t_w2c"], w_of(1, [3]))):
        streams.insert(0, ([[_Item(0, None, None, d.wait) for d in dmas]], time, time))
    for time in cfg["t_split"]:
        streams.insert(0, ([[_Item(0, None, None, lambda: out_dmas.pop(0).wait() if out_dmas else None)]], time, time))
    phases = _spread(streams)
    if cfg.get("show"):
        print("load", [sum(it.cost for it in phases[p]) + 1728 for p in sorted(phases)])
    for p in range(max(p_lo, 0), min(p_hi, 32)):
        todo.extend((p, xi, nu) for xi in range(6) for nu in range(6))
        run_phase(p, phases[p])
        advance((p + 1) * SPAN - 1)
    if p_hi > 32:
        run_alone([phases.get(32, [])] + out_groups(31), cfg["alone"])
    for d in out_dmas:
        d.wait()


def _lin(points, n):
    out = []
    for i in range(n):
        (i0, v0), (i1, v1) = next((a, b) for a, b in zip(points, points[1:]) if a[0] <= i <= b[0])
        out.append(v0 + (v1 - v0) * (i - i0) / (i1 - i0))
    return tuple(out)


_CFG = dict(
    only=(-1, 33), lead=16, slack=40, win=2, alone=350, n_m=5, ahead=0, chain=7, clk_every=1, pop_every=2, pop_lag=22, dslack=(),
    c_rowx=88, c_rowh=80, c_col=42, c_o1=14, c_o2=52, c_w1=90, c_w2=30, c_st=40,
    nnu=1, o_nxi=3, w_nxi=1, w_direct=True,
    x_pieces=2, stat_rows=2, last_send=2, t_emb=8.0, t_w2b=12.0, t_w2c=16.0, t_split=(20.5, 24.5, 28.5),
    head=(("w", 0), ("s", 0), ("w", 1), ("i", 0), ("s", 1), ("w", 2), ("i", 1), ("s", 2), ("w", 3), ("i", 2),
          ("s", 3), ("i", 3)),
    t_in=((1.2, 3.98), (4.6, 7.98), (8.0, 11.98), (12.0, 15.98), (16.5, 19.98), (20.0, 23.98), (24.0, 27.98)),
    t_stat=(3.0, 6.4),
    t_w=((0.0, 0.93), (0.93, 1.9), (1.9, 2.9), (8.0, 11.0), (11.0, 14.0), (14.0, 16.6), (16.6, 18.9)),
    t_out=_lin(((0, 3.5), (4, 8.0), (12, 15.6), (15, 18.95), (16, 20.0), (27, 28.04), (31, 32.0)), 32),
)


def _resblock(cfg, x, t_emb, g1, be1, w1, w_emb, g2, be2, w2):
    assert x.shape == (NB, C, HW, HW) and w1.shape == w2.shape == (C, C, 3, 3)
    emb_dim = t_emb.shape[1]
    vmem = pltpu.VMEM
    scratch = (
        [vmem((2 * TOK + NG * HW * HW, 128), BF16)] * 2
        + [vmem((1 + HW * NG, 2, 4, 8, 128), F32)] * 2
        + [vmem((1 + NG * 9, C, 128), BF16)] * 2
        + [vmem((1 + NG * 36, 64, C), U32)] * 2
        + [vmem((1 + 36, M // 2, C), U32)] * 2
        + [vmem((1 + NG * T_ROWS, 2, 7, 8, 128), F32),
           vmem((1 + 2 * 6, 7, 8, 128), F32),
           vmem((1 + 2 * 4, 7, 8, 128), F32),
           vmem((2 * NB * NG, 9, 8, 128), F32),
           vmem((1 + NB * NG, 6, 8, 128), F32),
           vmem((NB, emb_dim), BF16)]
        + [vmem((C,), BF16)] * 4
        + [vmem((emb_dim, C), BF16), vmem((NB, C), F32), pltpu.SemaphoreType.DMA((96,))]
        + [vmem((1 + 36, M_PITCH, 128), F32)] * cfg["n_m"]
    )
    as_taps = lambda w: jnp.transpose(w, (2, 3, 0, 1)).reshape(9, C, C)
    out = pl.pallas_call(
        functools.partial(_kernel, cfg),
        out_shape=jax.ShapeDtypeStruct((NB, HW * HW, C), x.dtype),
        in_specs=[pl.BlockSpec(memory_space=pl.ANY)] * 9,
        out_specs=pl.BlockSpec(memory_space=pl.ANY),
        scratch_shapes=scratch,
        compiler_params=pltpu.CompilerParams(vmem_limit_bytes=120 * 2 ** 20),
    )(jnp.transpose(x, (0, 2, 3, 1)).reshape(NB, HW * HW, C), t_emb, g1, be1, as_taps(w1), w_emb,
      g2, be2, as_taps(w2))
    return jnp.transpose(out.reshape(NB, HW, HW, C), (0, 3, 1, 2))


@jax.jit
def pallas_standalone__adm_resblock__diffusion_kernel(
    x: jax.Array,
    t_emb: jax.Array,
    g1: jax.Array,
    be1: jax.Array,
    w1: jax.Array,
    w_emb: jax.Array,
    g2: jax.Array,
    be2: jax.Array,
    w2: jax.Array,
):
    return _resblock(_CFG, x, t_emb, g1, be1, w1, w_emb, g2, be2, w2)
```

```python
import functools

import jax
import jax.numpy as jnp
from jax.experimental import pallas as pl
from jax.experimental.pallas import tpu as pltpu

F32, BF16, U32 = jnp.float32, jnp.bfloat16, jnp.uint32

NB, C, HW, NG = 2, 512, 64, 4
EPS = 1e-5
TR = 8
M = 16 * TR
M_PITCH = M + 16
T_ROWS = 33
TICKS = M // 8
SPAN = 36 * TICKS

PA, PB = 2.0 / 3.0, 1.5
A2, B2, B3 = PA * PA, PB * PB, PB * PB * PB
DD = A2 - B2


def _xf_in(d):
    p2, q2 = B2 * d[2], A2 * d[2]
    ea, eb = d[4] - p2, d[4] - q2
    p3, q3 = A2 * d[3], B2 * d[3]
    ua, ub = d[1] - p3, d[1] - q3
    v0 = (ea if d[0] is None else d[0] + ea) - q2
    v5 = (ua if d[5] is None else d[5] + ua) - q3
    oa, ob = PB * ua, PA * ub
    return [v0, ea - oa, ea + oa, eb - ob, eb + ob, v5]


def _xf_out(m):
    sa, da, sb, db = m[1] + m[2], m[1] - m[2], m[3] + m[4], m[3] - m[4]
    return [(m[0] + sb) + B3 * sa, PB * da + db, sa + PB * sb, (da + m[5]) + B3 * db]


def _xf_w(g):
    ca, cb = PA ** 3 / (2 * A2 * DD), -1.0 / (2 * B2 * DD)
    ea, eb = ca * g[0] + (ca * A2) * g[2], cb * g[0] + (cb * B2) * g[2]
    oa, ob = (ca * PA) * g[1], (cb * PB) * g[1]
    return [g[0], ea + oa, ea - oa, eb + ob, eb - ob, g[2]]


def _unpack(w, half):
    return pltpu.unpack_elementwise(w, index=half, packed_dtype=BF16, unpacked_dtype=F32)


def _pack(lo, hi):
    return pltpu.pack_elementwise([lo, hi], packed_dtype=BF16)


def _mean_all(v):
    return jnp.sum(jnp.sum(v, axis=0, keepdims=True), axis=1, keepdims=True) * (1.0 / v.size)


class _Item:
    def __init__(self, cost, src, dst, fn):
        self.cost, self.src, self.dst, self.fn = cost, src, dst, fn

    def slack(self, cfg):
        return cfg["slack"] + dict(cfg["dslack"]).get(getattr(getattr(self.fn, "func", None), "__name__", ""), 0)


class _Pacer:
    def __init__(self, zero):
        self.zero = zero

    def move(self, zero):
        self.zero = zero

    def _slot(self, buf, which):
        lanes = pl.ds(0, 128)
        if buf.shape[-2] > 8:
            return (self.zero,) + (0,) * (len(buf.shape) - 3) + (pl.ds(8 * which, 8), lanes)
        return (self.zero,) + (0,) * (len(buf.shape) - 4) + (which, pl.ds(0, 8), lanes)

    def init(self, buf):
        for which in range(2):
            buf[self._slot(buf, which)] = jnp.zeros((8, 128), buf.dtype)

    def release(self, buf, value):
        if value.dtype != buf.dtype:
            value = pltpu.bitcast(value, buf.dtype)
        buf[self._slot(buf, 0)] = value

    def done(self, buf):
        return buf[self._slot(buf, 1)]


def _spread(streams):
    keyed = []
    for groups, lo, hi in streams:
        total = max(sum(it.cost for grp in groups for it in grp), 1)
        acc = 0
        for grp in groups:
            cost = sum(it.cost for it in grp)
            keyed.append((lo + (hi - lo) * (acc + cost / 2) / total, len(keyed), grp))
            acc += cost
    keyed.sort(key=lambda t: t[:2])
    phases = {}
    for time, _, grp in keyed:
        phases.setdefault(int(time // 1), []).extend(grp)
    return phases


def _kernel(cfg, x_hbm, t_hbm, g1_hbm, be1_hbm, w1_hbm, wemb_hbm, g2_hbm, be2_hbm, w2_hbm, o_hbm,
            xs0, xs1, h0, h1, wr1, wr2, u1, u2, v0, v1, tb, ws, osb, coef, stat,
            t_s, g1_s, be1_s, g2_s, be2_s, wemb_s, emb_s, affine, sems, *ms):
    xs_bf, wr_bf = (xs0, xs1), (wr1, wr2)
    xs = tuple(r.bitcast(U32) for r in xs_bf)
    wr = tuple(r.bitcast(U32) for r in wr_bf)
    hs, us, vs = (h0, h1), (u1, u2), (v0, v1)
    part = functools.partial
    lanes = lambda g: pl.ds(g * 128 if isinstance(g, int) else pl.multiple_of(g * 128, 128), 128)

    xp = cfg["x_pieces"]
    xr = HW // xp
    n_head = NG * (xp + 1)

    def x_copy(b, g, r0, nr, sem):
        return pltpu.make_async_copy(x_hbm.at[b, pl.ds(r0, nr), :, lanes(g)],
                                     xs_bf[b].at[pl.ds(1 + g * HW + r0, nr)], sems.at[sem])

    def w_copy(cv, n0, n1, g, sem):
        rows = pl.ds(n0 * 128, (n1 - n0) * 128)
        return pltpu.make_async_copy((w1_hbm, w2_hbm)[cv].at[:, rows, lanes(g)],
                                     wr_bf[cv].at[pl.ds(1 + g * 9, 9), rows], sems.at[sem])

    x0_copy = lambda g, q: x_copy(0, g, q * xr, xr, g * (xp + 1) + q)
    w0_copy = lambda g: w_copy(0, 0, 1, g, g * (xp + 1) + xp)
    w_of = lambda cv, n0, n1, sem: [w_copy(cv, n0, n1, g, n_head + sem) for g in range(NG)]
    small = [pltpu.make_async_copy(s, d, sems.at[n_head]) for s, d in
             ((g1_hbm, g1_s), (be1_hbm, be1_s), (g2_hbm, g2_s), (be2_hbm, be2_s), (t_hbm, t_s))]
    late = [w_of(0, 1, 2, 1), w_of(0, 2, 4, 2),
            [x_copy(1, g, 0, HW, n_head + 3) for g in range(NG)]
            + [pltpu.make_async_copy(wemb_hbm, wemb_s, sems.at[n_head + 3])] + w_of(1, 0, 1, 3),
            w_of(1, 1, 3, 4), w_of(1, 3, 4, 5)]
    first = []
    for g in range(NG):
        xw = [x0_copy(g, q) for q in range(xp)], [w0_copy(g)]
        first += xw[1] + xw[0] if cfg["w_lead"] else xw[0] + xw[1]
    for d in first[:1] + small + first[1:] + [d for dmas in late for d in dmas]:
        d.start()

    sub = jax.lax.broadcasted_iota(jnp.int32, (8, 128), 0)

    def w_store(cv, n, g, ob, xi0, nxi, c):
        u = [_xf_w(ch) for ch in c]
        for nu in range(6):
            us[cv][pl.ds(1 + n * 36 + nu * 6 + xi0, nxi), pl.ds(ob * 8, 8), lanes(g)] = _pack(u[0][nu], u[1][nu])

    def w_first(cv, n, g, ob, slot):
        w = [wr[cv][pl.ds(1 + g * 9 + 3 * i, 3), pl.ds(n * 64 + ob * 8, 8)] for i in range(3)]
        c = [_xf_w([_unpack(wi, half) for wi in w]) for half in range(2)]
        for half in range(2):
            for xi in (range(1, 5) if cfg["w_direct"] else range(6)):
                ws[1 + slot * 6 + xi, pl.ds(half * 3, 3)] = c[half][xi]
        if cfg["w_direct"]:
            for xi in (0, 5):
                w_store(cv, n, g, ob, xi, 1, [[ch[xi][j:j + 1] for j in range(3)] for ch in c])

    def w_second(cv, n, g, ob, xi0, nxi, slot):
        w_store(cv, n, g, ob, xi0, nxi,
                [[ws[pl.ds(1 + slot * 6 + xi0, nxi), half * 3 + j] for j in range(3)] for half in range(2)])

    w_count = [0]

    def w_groups(cv, n, gs):
        units, out = [(cv, n, g, ob) for g in gs for ob in range(8)], []
        nxi = cfg["w_nxi"]
        for q in range(len(units) + 1):
            slot = w_count[0] % 2
            if q < len(units):
                cost = cfg["c_w1"] + (2 * cfg["c_w2"] if cfg["w_direct"] else 0)
                out.append([_Item(cost, wr[cv], (ws, us[cv]) if cfg["w_direct"] else ws, part(w_first, *units[q], slot))])
                w_count[0] += 1
            if q > 0:
                out += [[_Item(cfg["c_w2"] * nxi, ws, us[cv], part(w_second, *units[q - 1], xi0, nxi, 1 - slot))]
                        for xi0 in (range(1, 5, nxi) if cfg["w_direct"] else range(0, 6, nxi))]
        return out

    def set_coef(cv, b, g, mean, var, bias):
        gamma, beta = affine[2 * cv, g], affine[2 * cv + 1, g]
        mu = _mean_all(mean)
        dev = mean - mu
        scale = gamma * jax.lax.rsqrt(_mean_all(jnp.maximum(var, 0.0) + dev * dev) + EPS)
        shift = beta + (bias - mu) * scale
        k = (cv * NB + b) * NG + g
        coef[k, 0] = jnp.broadcast_to(0.5 * shift, (8, 128))
        for q, power in enumerate((0, 0, 1, 1, 1, 1, 2, 2) if cv else (0,)):
            coef[k, 1 + q] = jnp.broadcast_to((0.5 * PB ** power) * scale, (8, 128))

    def x_stat_rows(acc, b, g, r0, nr):
        for r in range(r0, r0 + nr):
            w = xs[b][1 + g * HW + r].reshape(2, 2, 8, 128)
            lo, hi = _unpack(w, 0), _unpack(w, 1)
            if not acc:
                acc.append(lo[0])
            lo, hi = lo - acc[0], hi - acc[0]
            s1, s2 = lo + hi, lo * lo + hi * hi
            s1, s2 = s1[0] + s1[1], s2[0] + s2[1]
            acc[1:] = [acc[1] + s1, acc[2] + s2] if acc[1:] else [s1, s2]
        stat[0, pl.ds(2, 2)] = acc[1]
        stat[0, pl.ds(4, 2)] = acc[2]

    def x_stat_end(acc, b, g):
        if not acc: return
        ref, m1, m2 = acc[0], acc[1] * (1.0 / (HW * 4)), acc[2] * (1.0 / (HW * 4))
        set_coef(0, b, g, (ref + m1).reshape(16, 128), (m2 - m1 * m1).reshape(16, 128), 0.0)

    def x_stat_groups(b, g, waits):
        acc, out, nr = [], [], cfg["stat_rows"]
        for r0 in range(0, HW, nr):
            grp = [_Item(0, None, None, waits[r0].wait)] if r0 in waits else []
            out.append(grp + [_Item(cfg["c_st"] * nr, xs[b], stat, part(x_stat_rows, acc, b, g, r0, nr))])
        out.append([_Item(30, None, None, part(x_stat_end, acc, b, g))])
        return out

    def h_stat_end(b, g):
        s = stat[1 + b * NG + g]
        inv = 1.0 / (HW * 8)
        m1 = (s[0] + PB * (s[1] + PB * s[2])) * inv
        m2 = (s[3] + B2 * (s[4] + B2 * s[5])) * inv
        e = emb_s[pl.ds(b, 1), lanes(g)]
        set_coef(1, b, g, m1 + e, m2 - m1 * m1, e)

    def time_emb():
        t = t_s[...].astype(F32)
        emb_s[...] = jnp.dot((t * jax.nn.sigmoid(t)).astype(BF16), wemb_s[...], preferred_element_type=F32)

    def silu(z, scale, shift):
        u = z * scale + shift
        return u + u * jnp.tanh(u)

    def in_row(cv, b, g, h):
        k = (cv * NB + b) * NG + g
        if cv == 0:
            row = 1 + g * HW + h
            w = jnp.concatenate([xs[b][row, pl.ds(jp, 8, stride=4)] for jp in range(4)]).reshape(2, 2, 8, 128)
            scale, shift = coef[k, 1], coef[k, 0]
            lo, hi = silu(_unpack(w, 0), scale, shift), silu(_unpack(w, 1), scale, shift)
            d = [lo[:, 0], hi[:, 0], lo[:, 1], hi[:, 1]]
        else:
            a = silu(hs[b][1 + h * NG + g], coef[k, pl.ds(1 if h % 4 in (0, 3) else 5, 4)], coef[k, 0])
            d = [a[:, 0], a[:, 2], a[:, 3], a[:, 1]]
        left = jnp.where(sub == 0, 0.0, pltpu.roll(d[3][1], 1, 0))
        right = jnp.where(sub == 7, 0.0, pltpu.roll(d[0][0], 7, 0))
        v = _xf_in([jnp.stack([left, d[3][0]])] + d + [jnp.stack([d[0][1], right])])
        for nu in range(6):
            tb[1 + g * T_ROWS + h % T_ROWS, :, nu] = v[nu]

    def in_col(vn, g, r, nu0, nnu):
        rows = range(4 * r - 1, 4 * r + 5)
        v = [_xf_in([tb[1 + g * T_ROWS + h % T_ROWS, p, pl.ds(nu0, nnu)] if 0 <= h < HW else None for h in rows])
             for p in range(2)]
        for xi in range(6):
            vn[pl.ds(1 + xi * 6 + nu0, nnu), pl.ds(r % TR * 8, 8), lanes(g)] = _pack(v[0][xi], v[1][xi])

    def in_groups(c, g):
        cv, b, r0 = c // 4, (c // 2) % 2, (c % 2) * TR
        src, cost = (xs[b], cfg["c_rowx"]) if cv == 0 else (hs[b], cfg["c_rowh"])
        row = lambda h: [_Item(cost, src, tb, part(in_row, cv, b, g, h))]
        out, nnu = [row(0)] if r0 == 0 else [], cfg["nnu"]
        for r in range(r0, r0 + TR + 1):
            rows = [row(h) for h in range(4 * r + 1, min(4 * r + 5, HW))] if r < r0 + TR else []
            cols = [[_Item(cfg["c_col"] * nnu, tb, vs[c % 2], part(in_col, vs[c % 2], g, r - 1, nu0, nnu))]
                    for nu0 in range(0, 6, nnu)] if r > r0 else []
            out += [grp for _, grp in sorted(
                [((q + 0.25) / len(rows), grp) for q, grp in enumerate(rows)]
                + [((q + 0.75) / len(cols), grp) for q, grp in enumerate(cols)], key=lambda t: t[0])]
        return out

    def out_first(cv, mp, r, p, xi0, nxi, slot):
        y = _xf_out([mp[pl.ds(1 + nu * 6 + xi0, nxi), pl.ds(r % TR * 16 + p, 8, stride=2)] for nu in range(6)])
        for q, j in enumerate((0, 1, 2, 3) if cv else (0, 3, 1, 2)):
            osb[1 + slot * 4 + q, pl.ds(xi0, nxi)] = y[j]

    def out_second(acc, cv, b, n, r, p, jp, slot):
        y = _xf_out([osb[pl.ds(1 + slot * 4 + 2 * jp, 2), xi] for xi in range(6)])
        if not acc: acc.extend(jnp.zeros((8, 128), F32) for q in range(6))
        if cv == 0:
            for i in range(4):
                hs[b][1 + (4 * r + i) * NG + n, p, pl.ds(2 * jp, 2)] = y[i]
            for power, ya, yb in ((jp, y[0], y[3]), (jp + 1, y[1], y[2])):
                s1, s2 = ya + yb, ya * ya + yb * yb
                acc[power] = acc[power] + (s1[0] + s1[1])
                acc[3 + power] = acc[3 + power] + (s2[0] + s2[1])
        else:
            for i in range(4):
                at = (1 + n * HW + 4 * r + i, pl.ds(2 * p + jp, 8, stride=4))
                w, res = xs[b][at], []
                for q in range(2):
                    power = (i in (1, 2)) + (2 * jp + q in (1, 2))
                    res.append(_unpack(w, q) + (y[i][q] * PB ** power if power else y[i][q]))
                xs[b][at] = _pack(*res)

    out_dmas, os_count = [], [0]

    def out_groups(phase):
        c, n = divmod(phase, NG)
        cv, b, r0 = c // 4, (c // 2) % 2, (c % 2) * TR
        mp, acc, nxi = ms[phase % len(ms)], [], cfg["o_nxi"]

        def begin():
            acc.extend(stat[1 + b * NG + n, q] if r0 else jnp.zeros((8, 128), F32) for q in range(6))

        def end():
            for q in range(6):
                stat[1 + b * NG + n, q] = acc[q]

        def send(h0, nr):
            out_dmas.append(pltpu.make_async_copy(xs_bf[b].at[pl.ds(1 + n * HW + h0, nr)],
                                                  o_hbm.at[b, pl.ds(h0, nr), :, lanes(n)],
                                                  sems.at[min(phase - 16, len(cfg["t_split"]))]))
            out_dmas[-1].start()

        units = [(r, p) for r in range(r0, r0 + TR) for p in range(2)]
        send_rows = cfg["last_send"] if phase == 31 else TR
        out = [[_Item(0, None, None, begin)]] if cv == 0 else []
        for q in range(len(units) + 1):
            slot = os_count[0] % 2
            firsts = [[_Item(cfg["c_o1"] * nxi, mp, osb, part(out_first, cv, mp, *units[q], xi0, nxi, slot))]
                      for xi0 in range(0, 6, nxi)] if q < len(units) else []
            seconds = [[_Item(cfg["c_o2"], osb, (hs, xs)[cv][b],
                              part(out_second, acc, cv, b, n, *units[q - 1], jp, 1 - slot))]
                       for jp in range(2)] if q > 0 else []
            os_count[0] += bool(firsts)
            out += [grp for _, grp in sorted(
                [((k + 0.25) / len(firsts), grp) for k, grp in enumerate(firsts)]
                + [((k + 0.75) / len(seconds), grp) for k, grp in enumerate(seconds)], key=lambda t: t[0])]
            if cv == 1 and q > 0 and q % (2 * send_rows) == 0:
                out[-1].append(_Item(0, None, None, part(send, 4 * (r0 + q // 2 - send_rows), 4 * send_rows)))
        if cv == 0:
            out[-1].append(_Item(0, None, None, end))
        return out

    def matmul(phase, xi, nu, dues):
        c, n = divmod(phase, NG)
        vc = vs[c % 2]
        cuts = sorted({0, TR} | set(dues))
        blocks = []
        for lo, hi in zip(cuts, cuts[1:]):
            for value in dues.get(lo, ()):
                pace.release(vc, value)
            blocks.append(vc[1 + xi * 6 + nu, pl.ds(lo * 8, (hi - lo) * 8)])
        lhs = pltpu.bitcast(jnp.concatenate(blocks, axis=0), BF16)
        rhs = pltpu.bitcast(us[c // 4][1 + n * 36 + nu * 6 + xi], BF16)
        res = jax.lax.dot_general(lhs, rhs, (((1,), (1,)), ((), ())), preferred_element_type=F32)
        ms[phase % len(ms)][1 + nu * 6 + xi, pl.ds(0, M)] = res
        return res

    dsts = lambda it: it.dst if isinstance(it.dst, tuple) else () if it.dst is None else (it.dst,)

    def run_alone(groups, window):
        finished, acc = [], 0
        for it in (it for grp in groups for it in grp):
            ready = [v for t, v in finished if t <= acc - window]
            if it.src is not None and ready:
                pace.release(it.src, ready[-1])
            it.fn()
            acc += it.cost
            for dst in dsts(it):
                finished.append((acc, pace.done(dst)))
            del finished[:-24]

    clock, pending, todo, chain = [], {}, [], []

    def advance(tick):
        while todo and (base + len(clock)) * TICKS <= tick:
            now, dues = (base + len(clock)) * TICKS, {}
            for key in [key for key in pending if key[0] < now + TICKS]:
                dues.setdefault(max(key[0] - now, 0) // 2, []).append(pending.pop(key))
            for rb in range(0, TR if cfg["pop_lag"] else 0, cfg["pop_every"]):
                t = min(now + 2 * rb - cfg["pop_lag"], now - 1)
                if t >= base * TICKS:
                    dues.setdefault(rb, []).append(clock[t // TICKS - base][t % TICKS * 8:t % TICKS * 8 + 8])
            clock.append(matmul(*todo.pop(0), dues))

    def run_phase(p, items):
        lead, slack, win = cfg["lead"], cfg["slack"], cfg["win"]
        total, acc, plan, releases = sum(it.cost for it in items), 0, [], {}
        for it in items:
            start = p * SPAN + int(acc / total * SPAN) // win * win - lead
            acc += it.cost
            plan.append((it, start, -(-(p * SPAN + int(acc / total * SPAN) - lead + it.slack(cfg)) // 2) * 2))
            if it.src is not None and start >= base * TICKS and len(plan) % cfg["clk_every"] == 0:
                releases[start, id(it.src)] = it.src
        for it, start, due in plan:
            for key in [key for key in releases if key[0] <= start + cfg["ahead"]]:
                advance(key[0])
                q = key[0] % TICKS
                pace.release(releases.pop(key), clock[key[0] // TICKS - base][8 * q:8 * q + 8])
            advance(start)
            if cfg["chain"] and it.src is not None and len(chain) >= cfg["chain"]:
                pace.release(it.src, chain[-cfg["chain"]])
            it.fn()
            for dst in dsts(it):
                pending[due, id(dst)] = pace.done(dst)
                chain.append(pending[due, id(dst)])
            del chain[:-32]

    p_lo, p_hi = cfg["only"]
    base = max(p_lo, 0) * 36

    for d in small:
        d.wait()
    for q, ref in enumerate((g1_s, be1_s, g2_s, be2_s)):
        value = ref[...].astype(F32)
        for g in range(NG):
            affine[q, g] = jnp.broadcast_to(value[g * 128:(g + 1) * 128][None, :], (8, 128))
    pace = _Pacer(0)
    for buf in (*xs, *hs, *wr, *us, *vs, *ms, tb, ws, osb, stat):
        pace.init(buf)

    def head(g, _):
        pace.move(g >> 10)
        weights = [[_Item(0, None, None, w0_copy(g).wait)]] + w_groups(0, 0, [g])
        stats = x_stat_groups(0, g, {q * xr: x0_copy(g, q) for q in range(xp)})
        run_alone((weights + stats if cfg["w_lead"] else stats[:-1] + weights[:1] + stats[-1:] + weights[1:])
                  + in_groups(0, g), cfg["alone"])
        return g >> 10

    if p_lo >= 0:
        head = lambda g, z: z + (g >> 10)
    pace.move(jax.lax.fori_loop(0, NG, head, jnp.int32(0)))

    streams = []
    for c in range(1, 8):
        groups = []
        for g in range(NG):
            if c in (4, 6):
                groups.append([_Item(30, None, None, part(h_stat_end, (c - 4) // 2, g))])
            groups += in_groups(c, g)
        streams.append((groups, *cfg["t_in"][c - 1]))
    streams.append(([grp for g in range(NG) for grp in x_stat_groups(1, g, {})], *cfg["t_stat"]))
    w_times = cfg["t_w"]
    for k, (cv, n) in enumerate([(cv, n) for cv in range(2) for n in range(NG)][1:]):
        streams.append((w_groups(cv, n, range(NG)), *w_times[k]))
    t_out = cfg["t_out"]
    for p in range(31):
        assert p + 1 <= t_out[p] and t_out[p + 1] <= p + len(ms)
        streams.append((out_groups(p), t_out[p], t_out[p + 1]))
    streams.append(([[_Item(1, None, None, time_emb)]], cfg["t_emb"], cfg["t_emb"]))
    sc = [None, 0]
    def scope(name):
        if not cfg.get("scopes"): return
        if sc[0] is not None: sc[0].__exit__(None, None, None)
        sc[0] = jax.named_scope(f"s_{sc[1]:02d}{name}") if name else None
        sc[1] += 1
        if sc[0] is not None: sc[0].__enter__()
    def waits(dmas):
        scope("wait")
        for d in dmas: d.wait()
        scope("run")
    for time, dmas in zip(cfg["t_wait"], late):
        streams.insert(0, ([[_Item(0, None, None, part(waits, dmas))]], time, time))
    for time in cfg["t_split"]:
        streams.insert(0, ([[_Item(0, None, None, lambda: waits([out_dmas.pop(0)]) if out_dmas else None)]], time, time))
    phases = _spread(streams)
    if cfg.get("show"):
        print("load", [sum(it.cost for it in phases[p]) + 1728 for p in sorted(phases)])
    for p in range(max(p_lo, 0), min(p_hi, 32)):
        todo.extend((p, xi, nu) for xi in range(6) for nu in range(6))
        run_phase(p, phases[p])
        advance((p + 1) * SPAN - 1)
    scope("tail")
    if p_hi > 32:
        run_alone([phases.get(32, [])] + out_groups(31), cfg["alone"])
    scope("last")
    for d in out_dmas:
        d.wait()
    scope(None)


def _lin(points, n):
    out = []
    for i in range(n):
        (i0, v0), (i1, v1) = next((a, b) for a, b in zip(points, points[1:]) if a[0] <= i <= b[0])
        out.append(v0 + (v1 - v0) * (i - i0) / (i1 - i0))
    return tuple(out)


_CFG = dict(
    only=(-1, 33), lead=16, slack=40, win=2, alone=500, n_m=5, ahead=0, chain=7, clk_every=1, pop_every=2, pop_lag=22,
    dslack=(), c_rowx=88, c_rowh=80, c_col=42, c_o1=14, c_o2=52, c_w1=90, c_w2=30, c_st=40,
    nnu=1, o_nxi=3, w_nxi=1, w_direct=True, w_lead=False,
    x_pieces=2, stat_rows=2, last_send=2, t_emb=5.0,
    t_wait=(0.0, 1.0, 5.0, 10.0, 16.0), t_split=(22.0, 27.0),
    t_in=((0.0, 3.98), (5.7, 7.98), (8.0, 11.98), (12.0, 15.98), (16.4, 19.98), (20.0, 23.98), (24.0, 27.98)),
    t_stat=(5.0, 7.3),
    t_w=((0.0, 0.98), (1.0, 1.98), (2.0, 2.98), (9.8, 12.2), (12.2, 14.4), (14.4, 16.8), (16.8, 18.95)),
    t_out=_lin(((0, 3.0), (4, 5.05), (5, 8.4), (8, 9.9), (12, 15.0), (15, 18.95), (16, 19.8), (27, 28.04), (31, 32.0)), 32),
)


def _resblock(cfg, x, t_emb, g1, be1, w1, w_emb, g2, be2, w2):
    assert x.shape == (NB, C, HW, HW) and w1.shape == w2.shape == (C, C, 3, 3)
    emb_dim = t_emb.shape[1]
    vmem = pltpu.VMEM
    scratch = (
        [vmem((1 + NG * HW, HW, 128), BF16)] * 2
        + [vmem((1 + HW * NG, 2, 4, 8, 128), F32)] * 2
        + [vmem((1 + NG * 9, C, 128), BF16)] * 2
        + [vmem((1 + NG * 36, 64, C), U32)] * 2
        + [vmem((1 + 36, M // 2, C), U32)] * 2
        + [vmem((1 + NG * T_ROWS, 2, 7, 8, 128), F32),
           vmem((1 + 2 * 6, 7, 8, 128), F32),
           vmem((1 + 2 * 4, 7, 8, 128), F32),
           vmem((2 * NB * NG, 9, 8, 128), F32),
           vmem((1 + NB * NG, 6, 8, 128), F32),
           vmem((NB, emb_dim), BF16)]
        + [vmem((C,), BF16)] * 4
        + [vmem((emb_dim, C), BF16), vmem((NB, C), F32), vmem((4, NG, 8, 128), F32), pltpu.SemaphoreType.DMA((NG * (cfg["x_pieces"] + 1) + 6,))]
        + [vmem((1 + 36, M_PITCH, 128), F32)] * cfg["n_m"]
    )
    as_taps = lambda w: jnp.transpose(w, (2, 3, 0, 1)).reshape(9, C, C)
    out = pl.pallas_call(
        functools.partial(_kernel, cfg),
        out_shape=jax.ShapeDtypeStruct((NB, HW, HW, C), x.dtype),
        in_specs=[pl.BlockSpec(memory_space=pl.ANY)] * 9,
        out_specs=pl.BlockSpec(memory_space=pl.ANY),
        scratch_shapes=scratch,
        compiler_params=pltpu.CompilerParams(vmem_limit_bytes=120 * 2 ** 20),
    )(jnp.transpose(x, (0, 2, 3, 1)), t_emb, g1, be1, as_taps(w1), w_emb,
      g2, be2, as_taps(w2))
    return jnp.transpose(out, (0, 3, 1, 2))


@jax.jit
def pallas_standalone__adm_resblock__diffusion_kernel(
    x: jax.Array,
    t_emb: jax.Array,
    g1: jax.Array,
    be1: jax.Array,
    w1: jax.Array,
    w_emb: jax.Array,
    g2: jax.Array,
    be2: jax.Array,
    w2: jax.Array,
):
    return _resblock(_CFG, x, t_emb, g1, be1, w1, w_emb, g2, be2, w2)
```

```python
import functools

import jax
import jax.numpy as jnp
from jax.experimental import pallas as pl
from jax.experimental.pallas import tpu as pltpu

F32, BF16, U32 = jnp.float32, jnp.bfloat16, jnp.uint32

NB, C, HW, NG = 2, 512, 64, 4
EPS = 1e-5
TR = 8
M = 16 * TR
M_PITCH = M + 16
T_ROWS = 33
TICKS = M // 8
SPAN = 36 * TICKS

PA, PB = 2.0 / 3.0, 1.5
A2, B2, B3 = PA * PA, PB * PB, PB * PB * PB
DD = A2 - B2


def _xf_in(d):
    p2, q2 = B2 * d[2], A2 * d[2]
    ea, eb = d[4] - p2, d[4] - q2
    p3, q3 = A2 * d[3], B2 * d[3]
    ua, ub = d[1] - p3, d[1] - q3
    v0 = (ea if d[0] is None else d[0] + ea) - q2
    v5 = (ua if d[5] is None else d[5] + ua) - q3
    oa, ob = PB * ua, PA * ub
    return [v0, ea - oa, ea + oa, eb - ob, eb + ob, v5]


def _xf_out(m):
    sa, da, sb, db = m[1] + m[2], m[1] - m[2], m[3] + m[4], m[3] - m[4]
    return [(m[0] + sb) + B3 * sa, PB * da + db, sa + PB * sb, (da + m[5]) + B3 * db]


def _xf_w(g):
    ca, cb = PA ** 3 / (2 * A2 * DD), -1.0 / (2 * B2 * DD)
    ea, eb = ca * g[0] + (ca * A2) * g[2], cb * g[0] + (cb * B2) * g[2]
    oa, ob = (ca * PA) * g[1], (cb * PB) * g[1]
    return [g[0], ea + oa, ea - oa, eb + ob, eb - ob, g[2]]


def _unpack(w, half):
    return pltpu.unpack_elementwise(w, index=half, packed_dtype=BF16, unpacked_dtype=F32)


def _pack(lo, hi):
    return pltpu.pack_elementwise([lo, hi], packed_dtype=BF16)


def _mean_all(v):
    return jnp.sum(jnp.sum(v, axis=0, keepdims=True), axis=1, keepdims=True) * (1.0 / v.size)


class _Item:
    def __init__(self, cost, src, dst, fn):
        self.cost, self.src, self.dst, self.fn = cost, src, dst, fn

    def slack(self, cfg):
        return cfg["slack"] + dict(cfg["dslack"]).get(getattr(getattr(self.fn, "func", None), "__name__", ""), 0)


class _Pacer:
    def __init__(self, zero):
        self.zero = zero

    def move(self, zero):
        self.zero = zero

    def _slot(self, buf, which):
        lanes = pl.ds(0, 128)
        if buf.shape[-2] > 8:
            return (self.zero,) + (0,) * (len(buf.shape) - 3) + (pl.ds(8 * which, 8), lanes)
        return (self.zero,) + (0,) * (len(buf.shape) - 4) + (which, pl.ds(0, 8), lanes)

    def init(self, buf):
        for which in range(2):
            buf[self._slot(buf, which)] = jnp.zeros((8, 128), buf.dtype)

    def release(self, buf, value, which=0):
        if value.dtype != buf.dtype:
            value = pltpu.bitcast(value, buf.dtype)
        buf[self._slot(buf, which)] = value

    def done(self, buf):
        return buf[self._slot(buf, 1)]


def _spread(streams):
    keyed = []
    for groups, lo, hi in streams:
        total = max(sum(it.cost for grp in groups for it in grp), 1)
        acc = 0
        for grp in groups:
            cost = sum(it.cost for it in grp)
            keyed.append((lo + (hi - lo) * (acc + cost / 2) / total, len(keyed), grp))
            acc += cost
    keyed.sort(key=lambda t: t[:2])
    phases = {}
    for time, _, grp in keyed:
        phases.setdefault(int(time // 1), []).extend(grp)
    return phases


def _kernel(cfg, x_hbm, t_hbm, g1_hbm, be1_hbm, w1_hbm, wemb_hbm, g2_hbm, be2_hbm, w2_hbm, o_hbm,
            xs0, xs1, h0, h1, wr1, wr2, u1, u2, v0, v1, tb, ws, osb, coef, stat,
            t_s, g1_s, be1_s, g2_s, be2_s, wemb_s, emb_s, affine, sems, *ms):
    xs_bf, wr_bf = (xs0, xs1), (wr1, wr2)
    xs = tuple(r.bitcast(U32) for r in xs_bf)
    wr = tuple(r.bitcast(U32) for r in wr_bf)
    hs, us, vs = (h0, h1), (u1, u2), (v0, v1)
    part = functools.partial
    static = lambda g: g if isinstance(g, int) else None
    lanes = lambda g: pl.ds(g * 128 if isinstance(g, int) else pl.multiple_of(g * 128, 128), 128)

    xp = cfg["x_pieces"]
    xr = HW // xp
    n_head = NG * (xp + 1)

    def x_copy(b, g, r0, nr, sem):
        return pltpu.make_async_copy(x_hbm.at[b, pl.ds(r0, nr), :, lanes(g)],
                                     xs_bf[b].at[pl.ds(1 + g * HW + r0, nr)], sems.at[sem])

    def w_copy(cv, n0, n1, g, sem):
        rows = pl.ds(n0 * 128, (n1 - n0) * 128)
        return pltpu.make_async_copy((w1_hbm, w2_hbm)[cv].at[:, rows, lanes(g)],
                                     wr_bf[cv].at[pl.ds(1 + g * 9, 9), rows], sems.at[sem])

    x0_copy = lambda g, q: x_copy(0, g, q * xr, xr, g * (xp + 1) + q)
    w0_copy = lambda g: w_copy(0, 0, 1, g, g * (xp + 1) + xp)
    w_of = lambda cv, n0, n1, sem: [w_copy(cv, n0, n1, g, n_head + sem) for g in range(NG)]
    small = [pltpu.make_async_copy(s, d, sems.at[n_head]) for s, d in
             ((g1_hbm, g1_s), (be1_hbm, be1_s), (g2_hbm, g2_s), (be2_hbm, be2_s), (t_hbm, t_s))]
    late = [w_of(0, 1, 2, 1), w_of(0, 2, 4, 2),
            [x_copy(1, g, 0, HW, n_head + 3) for g in range(NG)]
            + [pltpu.make_async_copy(wemb_hbm, wemb_s, sems.at[n_head + 3])], w_of(1, 0, 3, 4), w_of(1, 3, 4, 5)]
    first = []
    for g in range(NG):
        xw = [x0_copy(g, q) for q in range(xp)], [w0_copy(g)]
        first += xw[1] + xw[0] if cfg["w_lead"] else xw[0] + xw[1]
    for d in first[:1] + small + first[1:] + [d for dmas in late for d in dmas]:
        d.start()

    ready = set()

    def need(*keys):
        assert p_lo >= 0 or all(key in ready for key in keys), keys

    sub = jax.lax.broadcasted_iota(jnp.int32, (8, 128), 0)

    def w_store(cv, n, g, ob, xi0, nxi, c):
        u = [_xf_w(ch) for ch in c]
        for nu in range(6):
            us[cv][pl.ds(1 + n * 36 + nu * 6 + xi0, nxi), pl.ds(ob * 8, 8), lanes(g)] = _pack(u[0][nu], u[1][nu])

    def w_first(cv, n, g, ob, slot):
        w = [wr[cv][pl.ds(1 + g * 9 + 3 * i, 3), pl.ds(n * 64 + ob * 8, 8)] for i in range(3)]
        c = [_xf_w([_unpack(wi, half) for wi in w]) for half in range(2)]
        for half in range(2):
            for xi in (range(1, 5) if cfg["w_direct"] else range(6)):
                ws[1 + slot * 6 + xi, pl.ds(half * 3, 3)] = c[half][xi]
        if cfg["w_direct"]:
            for xi in (0, 5):
                w_store(cv, n, g, ob, xi, 1, [[ch[xi][j:j + 1] for j in range(3)] for ch in c])

    def w_second(cv, n, g, ob, xi0, nxi, slot):
        w_store(cv, n, g, ob, xi0, nxi,
                [[ws[pl.ds(1 + slot * 6 + xi0, nxi), half * 3 + j] for j in range(3)] for half in range(2)])

    w_count = [0]

    def w_groups(cv, n, gs):
        units, out = [(cv, n, g, ob) for g in gs for ob in range(8)], []
        nxi = cfg["w_nxi"]
        for q in range(len(units) + 1):
            slot = w_count[0] % 2
            if q < len(units):
                cost = cfg["c_w1"] + (2 * cfg["c_w2"] if cfg["w_direct"] else 0)
                out.append([_Item(cost, wr[cv], (ws, us[cv]) if cfg["w_direct"] else ws, part(w_first, *units[q], slot))])
                w_count[0] += 1
            if q > 0:
                out += [[_Item(cfg["c_w2"] * nxi, ws, us[cv], part(w_second, *units[q - 1], xi0, nxi, 1 - slot))]
                        for xi0 in (range(1, 5, nxi) if cfg["w_direct"] else range(0, 6, nxi))]
        out[-1].append(_Item(0, None, None, part(ready.add, ("w", cv, n))))
        return out

    def set_coef(cv, b, g, mean, var, bias):
        gamma, beta = affine[2 * cv, g], affine[2 * cv + 1, g]
        mu = _mean_all(mean)
        dev = mean - mu
        scale = gamma * jax.lax.rsqrt(_mean_all(jnp.maximum(var, 0.0) + dev * dev) + EPS)
        shift = beta + (bias - mu) * scale
        k = (cv * NB + b) * NG + g
        ready.add(("coef", cv, b, static(g) if cv or b else None))
        coef[k, 0] = jnp.broadcast_to(0.5 * shift, (8, 128))
        for q, power in enumerate((0, 0, 1, 1, 1, 1, 2, 2) if cv else (0,)):
            coef[k, 1 + q] = jnp.broadcast_to((0.5 * PB ** power) * scale, (8, 128))

    def x_stat_rows(acc, b, g, r0, nr):
        for r in range(r0, r0 + nr):
            w = xs[b][1 + g * HW + r].reshape(2, 2, 8, 128)
            lo, hi = _unpack(w, 0), _unpack(w, 1)
            if not acc:
                acc.append(lo[0])
            lo, hi = lo - acc[0], hi - acc[0]
            s1, s2 = lo + hi, lo * lo + hi * hi
            s1, s2 = s1[0] + s1[1], s2[0] + s2[1]
            acc[1:] = [acc[1] + s1, acc[2] + s2] if acc[1:] else [s1, s2]
        stat[0, pl.ds(2, 2)] = acc[1]
        stat[0, pl.ds(4, 2)] = acc[2]

    def x_stat_end(acc, b, g):
        if not acc: return
        ref, m1, m2 = acc[0], acc[1] * (1.0 / (HW * 4)), acc[2] * (1.0 / (HW * 4))
        set_coef(0, b, g, (ref + m1).reshape(16, 128), (m2 - m1 * m1).reshape(16, 128), 0.0)

    def x_stat_groups(b, g, waits):
        acc, out, nr = [], [], cfg["stat_rows"]
        for r0 in range(0, HW, nr):
            grp = [_Item(0, None, None, waits[r0].wait)] if r0 in waits else []
            out.append(grp + [_Item(cfg["c_st"] * nr, xs[b], stat, part(x_stat_rows, acc, b, g, r0, nr))])
        out.append([_Item(30, None, None, part(x_stat_end, acc, b, g))])
        return out

    def h_stat_end(b, g):
        need("emb", ("out", (2 * b + 1) * NG + g))
        s = stat[1 + b * NG + g]
        inv = 1.0 / (HW * 8)
        m1 = (s[0] + PB * (s[1] + PB * s[2])) * inv
        m2 = (s[3] + B2 * (s[4] + B2 * s[5])) * inv
        e = emb_s[pl.ds(b, 1), lanes(g)]
        set_coef(1, b, g, m1 + e, m2 - m1 * m1, e)

    def emb_rows(acc, e0):
        t = t_s[:, pl.ds(e0, 128)].astype(F32)
        t = t * jax.nn.sigmoid(t)
        cols = [jnp.broadcast_to(t[b:b + 1], (128, 128)).T for b in range(NB)]
        for r in range(0, 128, 8):
            w = wemb_s[pl.ds(e0 + r, 8)].astype(F32)
            for b in range(NB):
                term = w * jnp.concatenate([cols[b][r:r + 8]] * NG, axis=1)
                acc[b] = acc[b] + term if b in acc else term
        for b in range(NB):
            stat[0, pl.ds(2, NG)] = jnp.stack([acc[b][:, g * 128:(g + 1) * 128] for g in range(NG)])

    def emb_groups():
        acc = {}

        def end():
            ready.add("emb")
            for b in range(NB):
                emb_s[pl.ds(b, 1)] = jnp.sum(acc[b], axis=0, keepdims=True)

        return ([[_Item(330, None, stat, part(emb_rows, acc, e0))] for e0 in range(0, t_s.shape[1], 128)]
                + [[_Item(40, None, None, end)]])

    def silu(z, scale, shift):
        u = z * scale + shift
        return u + u * jnp.tanh(u)

    def in_row(cv, b, g, h):
        k = (cv * NB + b) * NG + g
        need(("coef", cv, b, static(g) if cv or b else None))
        if cv == 0:
            row = 1 + g * HW + h
            w = jnp.concatenate([xs[b][row, pl.ds(jp, 8, stride=4)] for jp in range(4)]).reshape(2, 2, 8, 128)
            scale, shift = coef[k, 1], coef[k, 0]
            lo, hi = silu(_unpack(w, 0), scale, shift), silu(_unpack(w, 1), scale, shift)
            d = [lo[:, 0], hi[:, 0], lo[:, 1], hi[:, 1]]
        else:
            a = silu(hs[b][1 + h * NG + g], coef[k, pl.ds(1 if h % 4 in (0, 3) else 5, 4)], coef[k, 0])
            d = [a[:, 0], a[:, 2], a[:, 3], a[:, 1]]
        left = jnp.where(sub == 0, 0.0, pltpu.roll(d[3][1], 1, 0))
        right = jnp.where(sub == 7, 0.0, pltpu.roll(d[0][0], 7, 0))
        v = _xf_in([jnp.stack([left, d[3][0]])] + d + [jnp.stack([d[0][1], right])])
        for nu in range(6):
            tb[1 + g * T_ROWS + h % T_ROWS, :, nu] = v[nu]

    def in_col(vn, g, r, nu0, nnu):
        rows = range(4 * r - 1, 4 * r + 5)
        v = [_xf_in([tb[1 + g * T_ROWS + h % T_ROWS, p, pl.ds(nu0, nnu)] if 0 <= h < HW else None for h in rows])
             for p in range(2)]
        for xi in range(6):
            vn[pl.ds(1 + xi * 6 + nu0, nnu), pl.ds(r % TR * 8, 8), lanes(g)] = _pack(v[0][xi], v[1][xi])

    def in_groups(c, g):
        cv, b, r0 = c // 4, (c // 2) % 2, (c % 2) * TR
        src, cost = (xs[b], cfg["c_rowx"]) if cv == 0 else (hs[b], cfg["c_rowh"])
        row = lambda h: [_Item(cost, src, tb, part(in_row, cv, b, g, h))]
        out, nnu = [row(0)] if r0 == 0 else [], cfg["nnu"]
        for r in range(r0, r0 + TR + 1):
            rows = [row(h) for h in range(4 * r + 1, min(4 * r + 5, HW))] if r < r0 + TR else []
            cols = [[_Item(cfg["c_col"] * nnu, tb, vs[c % 2], part(in_col, vs[c % 2], g, r - 1, nu0, nnu))]
                    for nu0 in range(0, 6, nnu)] if r > r0 else []
            out += [grp for _, grp in sorted(
                [((q + 0.25) / len(rows), grp) for q, grp in enumerate(rows)]
                + [((q + 0.75) / len(cols), grp) for q, grp in enumerate(cols)], key=lambda t: t[0])]
        out[-1].append(_Item(0, None, None, part(ready.add, ("in", c, NG - 1 if static(g) is None else g))))
        if c > 1:
            out[0].insert(0, _Item(0, None, None, part(need, ("mm", c * NG - NG - 1))))
        return out

    def out_first(cv, mp, r, p, xi0, nxi, slot):
        y = _xf_out([mp[pl.ds(1 + nu * 6 + xi0, nxi), pl.ds(r % TR * 16 + p, 8, stride=2)] for nu in range(6)])
        for q, j in enumerate((0, 1, 2, 3) if cv else (0, 3, 1, 2)):
            osb[1 + slot * 4 + q, pl.ds(xi0, nxi)] = y[j]

    def out_second(acc, cv, b, n, r, p, jp, slot):
        y = _xf_out([osb[pl.ds(1 + slot * 4 + 2 * jp, 2), xi] for xi in range(6)])
        if not acc: acc.extend(jnp.zeros((8, 128), F32) for q in range(6))
        if cv == 0:
            for i in range(4):
                hs[b][1 + (4 * r + i) * NG + n, p, pl.ds(2 * jp, 2)] = y[i]
            for power, ya, yb in ((jp, y[0], y[3]), (jp + 1, y[1], y[2])):
                s1, s2 = ya + yb, ya * ya + yb * yb
                acc[power] = acc[power] + (s1[0] + s1[1])
                acc[3 + power] = acc[3 + power] + (s2[0] + s2[1])
        else:
            for i in range(4):
                at = (1 + n * HW + 4 * r + i, pl.ds(2 * p + jp, 8, stride=4))
                w, res = xs[b][at], []
                for q in range(2):
                    power = (i in (1, 2)) + (2 * jp + q in (1, 2))
                    res.append(_unpack(w, q) + (y[i][q] * PB ** power if power else y[i][q]))
                xs[b][at] = _pack(*res)

    out_dmas, os_count = [], [0]

    def out_groups(phase):
        c, n = divmod(phase, NG)
        cv, b, r0 = c // 4, (c // 2) % 2, (c % 2) * TR
        mp, acc, nxi = ms[phase % len(ms)], [], cfg["o_nxi"]

        def begin():
            acc.extend(stat[1 + b * NG + n, q] if r0 else jnp.zeros((8, 128), F32) for q in range(6))

        def end():
            for q in range(6):
                stat[1 + b * NG + n, q] = acc[q]

        def send(h0, nr):
            out_dmas.append(pltpu.make_async_copy(xs_bf[b].at[pl.ds(1 + n * HW + h0, nr)],
                                                  o_hbm.at[b, pl.ds(h0, nr), :, lanes(n)],
                                                  sems.at[min(phase - 16, len(cfg["t_split"]))]))
            out_dmas[-1].start()

        units = [(r, p) for r in range(r0, r0 + TR) for p in range(2)]
        send_rows = cfg["last_send"] if phase == 31 else TR
        out = [[_Item(0, None, None, begin)]] if cv == 0 else []
        for q in range(len(units) + 1):
            slot = os_count[0] % 2
            firsts = [[_Item(cfg["c_o1"] * nxi, mp, osb, part(out_first, cv, mp, *units[q], xi0, nxi, slot))]
                      for xi0 in range(0, 6, nxi)] if q < len(units) else []
            seconds = [[_Item(cfg["c_o2"], osb, (hs, xs)[cv][b],
                              part(out_second, acc, cv, b, n, *units[q - 1], jp, 1 - slot))]
                       for jp in range(2)] if q > 0 else []
            os_count[0] += bool(firsts)
            out += [grp for _, grp in sorted(
                [((k + 0.25) / len(firsts), grp) for k, grp in enumerate(firsts)]
                + [((k + 0.75) / len(seconds), grp) for k, grp in enumerate(seconds)], key=lambda t: t[0])]
            if cv == 1 and q > 0 and q % (2 * send_rows) == 0:
                out[-1].append(_Item(0, None, None, part(send, 4 * (r0 + q // 2 - send_rows), 4 * send_rows)))
        if cv == 0:
            out[-1].append(_Item(0, None, None, end))
        out[-1].append(_Item(0, None, None, part(ready.add, ("out", phase))))
        out[0].insert(0, _Item(0, None, None, part(need, ("mm", phase))))
        return out

    def matmul(phase, xi, nu, dues):
        c, n = divmod(phase, NG)
        vc = vs[c % 2]
        need(("in", c, NG - 1), ("w", c // 4, n), *[("out", phase - len(ms))] * (phase >= len(ms)))
        if xi == nu == 5:
            ready.add(("mm", phase))
        cuts = sorted({0, TR} | set(dues))
        blocks = []
        for lo, hi in zip(cuts, cuts[1:]):
            for value in dues.get(lo, ()):
                pace.release(vc, value)
            if dues.get(lo) and cfg["soft"] and (lo % cfg["soft"] or cfg["soft"] == 1):
                pace.release(vc, jnp.zeros((8, 128), U32))
            blocks.append(vc[1 + xi * 6 + nu, pl.ds(lo * 8, (hi - lo) * 8)])
        words = jnp.concatenate(blocks, axis=0)
        lhs = pltpu.bitcast(words, BF16)
        rhs = pltpu.bitcast(us[c // 4][1 + n * 36 + nu * 6 + xi], BF16)
        res = jax.lax.dot_general(lhs, rhs, (((1,), (1,)), ((), ())), preferred_element_type=F32)
        ms[phase % len(ms)][1 + nu * 6 + xi, pl.ds(0, M)] = res
        return res, words

    dsts = lambda it: it.dst if isinstance(it.dst, tuple) else () if it.dst is None else (it.dst,)

    def run_alone(groups, window):
        finished, acc = [], 0
        for it in (it for grp in groups for it in grp):
            ready = [v for t, v in finished if t <= acc - window]
            if it.src is not None and ready:
                pace.release(it.src, ready[-1])
            it.fn()
            acc += it.cost
            for dst in dsts(it):
                finished.append((acc, pace.done(dst)))
            del finished[:-24]

    clock, pending, todo, chain = [], {}, [], []

    def advance(tick):
        while todo and (base + len(clock)) * TICKS <= tick:
            now, dues = (base + len(clock)) * TICKS, {}
            for key in [key for key in pending if key[0] < now + TICKS]:
                dues.setdefault(max(key[0] - now, 0) // 2, []).append(pending.pop(key))
            for rb in range(0, TR if cfg["pop_lag"] else 0, cfg["pop_every"]):
                t = min(now + 2 * rb - cfg["pop_lag"], now - 1)
                if t >= base * TICKS:
                    dues.setdefault(rb, []).append(clock[t // TICKS - base][0][t % TICKS * 8:t % TICKS * 8 + 8])
            clock.append(matmul(*todo.pop(0), dues))

    def run_phase(p, items):
        lead, slack, win = cfg["lead"], cfg["slack"], cfg["win"]
        total, acc, plan, releases = sum(it.cost for it in items), 0, [], {}
        for it in items:
            start = p * SPAN + int(acc / total * SPAN) // win * win - lead
            acc += it.cost
            plan.append((it, start, -(-(p * SPAN + int(acc / total * SPAN) - lead + it.slack(cfg)) // 2) * 2))
            if it.src is not None and start >= base * TICKS and len(plan) % cfg["clk_every"] == 0:
                releases[start, id(it.src)] = it.src
        for it, start, due in plan:
            for key in [key for key in releases if key[0] <= start + cfg["ahead"]]:
                advance(key[0])
                q = key[0] % TICKS
                pace.release(releases.pop(key), clock[key[0] // TICKS - base][1][4 * q:4 * q + 8, :128] if cfg["vclk"] else clock[key[0] // TICKS - base][0][8 * q:8 * q + 8], cfg["clk_slot"])
            advance(start)
            if cfg["chain"] and it.src is not None and len(chain) >= cfg["chain"]:
                pace.release(it.src, chain[-cfg["chain"]])
            elif cfg["kill"] and it.src is not None:
                pace.release(it.src, jnp.zeros((8, 128), it.src.dtype))
            it.fn()
            for dst in dsts(it):
                pending[due, id(dst)] = pace.done(dst)
                chain.append(pending[due, id(dst)])
            del chain[:-32]

    p_lo, p_hi = cfg["only"]
    base = max(p_lo, 0) * 36

    sc = [None, 0]
    def scope(name):
        if not cfg.get("scopes"): return
        if sc[0] is not None: sc[0].__exit__(None, None, None)
        sc[0] = jax.named_scope(f"s_{sc[1]:02d}{name}") if name else None
        sc[1] += 1
        if sc[0] is not None: sc[0].__enter__()
    def waits(dmas):
        scope("wait")
        for d in dmas: d.wait()
        scope("run")
    waits(small)
    for q, ref in enumerate((g1_s, be1_s, g2_s, be2_s)):
        value = ref[...].astype(F32)
        for g in range(NG):
            affine[q, g] = jnp.broadcast_to(value[g * 128:(g + 1) * 128][None, :], (8, 128))
    pace = _Pacer(0)
    for buf in (*xs, *hs, *wr, *us, *vs, *ms, tb, ws, osb, stat):
        pace.init(buf)

    def head(g, _):
        pace.move(g >> 10)
        weights = [[_Item(0, None, None, w0_copy(g).wait)]] + w_groups(0, 0, [g])
        stats = x_stat_groups(0, g, {q * xr: x0_copy(g, q) for q in range(xp)})
        run_alone((weights + stats if cfg["w_lead"] else stats[:-1] + weights[:1] + stats[-1:] + weights[1:])
                  + in_groups(0, g), cfg["alone"])
        return g >> 10

    if p_lo >= 0:
        head = lambda g, z: z + (g >> 10)
    pace.move(jax.lax.fori_loop(0, NG, head, jnp.int32(0)))

    if p_lo >= 0:
        for d in first: d.wait()
        for time, dmas in zip(cfg["t_wait"], late):
            if not p_lo < time < p_hi:
                for d in dmas: d.wait()
        scope("go")
    streams = []
    for c in range(1, 8):
        groups = []
        for g in range(NG):
            if c in (4, 6):
                groups.append([_Item(30, None, None, part(h_stat_end, (c - 4) // 2, g))])
            groups += in_groups(c, g)
        streams.append((groups, *cfg["t_in"][c - 1]))
    streams.append(([grp for g in range(NG) for grp in x_stat_groups(1, g, {})], *cfg["t_stat"]))
    w_times = cfg["t_w"]
    for k, (cv, n) in enumerate([(cv, n) for cv in range(2) for n in range(NG)][1:]):
        streams.append((w_groups(cv, n, range(NG)), *w_times[k]))
    t_out = cfg["t_out"]
    for p in range(31):
        assert p + 1 <= t_out[p] and t_out[p + 1] <= p + len(ms)
        streams.append((out_groups(p), t_out[p], t_out[p + 1]))
    streams.append((emb_groups(), *cfg["t_emb"]))
    for time, dmas in zip(cfg["t_wait"], late):
        if p_lo < 0 or p_lo < time < p_hi:
          streams.insert(0, ([[_Item(0, None, None, part(waits, dmas))]], time, time))
    for time in cfg["t_split"]:
        streams.insert(0, ([[_Item(0, None, None, lambda: waits([out_dmas.pop(0)]) if out_dmas else None)]], time, time))
    phases = _spread(streams)
    if cfg.get("show"):
        print("load", [sum(it.cost for it in phases[p]) + 1728 for p in sorted(phases)])
    for p in range(max(p_lo, 0), min(p_hi, 32)):
        todo.extend((p, xi, nu) for xi in range(6) for nu in range(6))
        cfg = dict(cfg, **(cfg["L"] if p in cfg["light"] else cfg["H"]))
        run_phase(p, phases[p])
        advance((p + 1) * SPAN - 1)
    scope("tail")
    if p_hi > 32:
        run_alone([phases.get(32, [])] + out_groups(31), cfg["alone"])
    scope("last")
    for time, dmas in zip(cfg["t_wait"], late):
        if p_lo < 0 and time >= p_hi:
            for d in dmas: d.wait()
    for d in out_dmas:
        d.wait()
    scope(None)


def H(soft, chain, slack, pop_lag, pop_every=1, kill=1):
    return dict(soft=soft, kill=kill, chain=chain, slack=slack, pop_lag=pop_lag, pop_every=pop_every)


def _lin(points, n):
    out = []
    for i in range(n):
        (i0, v0), (i1, v1) = next((a, b) for a, b in zip(points, points[1:]) if a[0] <= i <= b[0])
        out.append(v0 + (v1 - v0) * (i - i0) / (i1 - i0))
    return tuple(out)


_CFG = dict(
    only=(-1, 33), lead=16, slack=40, win=2, alone=500, n_m=5, ahead=0, vclk=0, clk_slot=0, soft=1, kill=1, chain=7, clk_every=1, pop_every=2, pop_lag=22,
    dslack=(), L=dict(soft=0, kill=0, chain=0, slack=24, pop_lag=0, pop_every=1),
    H=dict(soft=4, kill=1, chain=5, slack=28, pop_lag=20, pop_every=1), light=tuple(range(22, 32)),
    c_rowx=88, c_rowh=80, c_col=42, c_o1=14, c_o2=52, c_w1=90, c_w2=30, c_st=40,
    nnu=1, o_nxi=3, w_nxi=1, w_direct=True, w_lead=False,
    x_pieces=2, stat_rows=2, last_send=2, t_emb=(7.2, 9.8),
    t_wait=(0.0, 1.0, 4.0, 10.0, 16.0), t_split=(22.0, 27.0),
    t_in=((0.0, 3.98), (4.8, 7.98), (8.0, 11.98), (12.0, 15.98), (16.0, 19.98), (20.0, 23.98), (24.0, 27.98)),
    t_stat=(4.0, 6.8),
    t_w=((0.0, 0.98), (1.0, 1.98), (2.0, 2.98), (10.0, 12.2), (12.2, 14.4), (14.4, 16.8), (16.8, 18.95)),
    t_out=_lin(((0, 3.0), (2, 4.2), (5, 8.0), (8, 10.0), (16, 19.0), (20, 21.04), (31, 32.0)), 32),
)


def _resblock(cfg, x, t_emb, g1, be1, w1, w_emb, g2, be2, w2):
    assert x.shape == (NB, C, HW, HW) and w1.shape == w2.shape == (C, C, 3, 3)
    emb_dim = t_emb.shape[1]
    vmem = pltpu.VMEM
    scratch = (
        [vmem((1 + NG * HW, HW, 128), BF16)] * 2
        + [vmem((1 + HW * NG, 2, 4, 8, 128), F32)] * 2
        + [vmem((1 + NG * 9, C, 128), BF16)] * 2
        + [vmem((1 + NG * 36, 64, C), U32)] * 2
        + [vmem((1 + 36, M // 2, C), U32)] * 2
        + [vmem((1 + NG * T_ROWS, 2, 7, 8, 128), F32),
           vmem((1 + 2 * 6, 7, 8, 128), F32),
           vmem((1 + 2 * 4, 7, 8, 128), F32),
           vmem((2 * NB * NG, 9, 8, 128), F32),
           vmem((1 + NB * NG, 6, 8, 128), F32),
           vmem((NB, emb_dim), BF16)]
        + [vmem((C,), BF16)] * 4
        + [vmem((emb_dim, C), BF16), vmem((NB, C), F32), vmem((4, NG, 8, 128), F32), pltpu.SemaphoreType.DMA((NG * (cfg["x_pieces"] + 1) + 6,))]
        + [vmem((1 + 36, M_PITCH, 128), F32)] * cfg["n_m"]
    )
    as_taps = lambda w: jnp.transpose(w, (2, 3, 0, 1)).reshape(9, C, C)
    out = pl.pallas_call(
        functools.partial(_kernel, cfg),
        out_shape=jax.ShapeDtypeStruct((NB, HW, HW, C), x.dtype),
        in_specs=[pl.BlockSpec(memory_space=pl.ANY)] * 9,
        out_specs=pl.BlockSpec(memory_space=pl.ANY),
        scratch_shapes=scratch,
        compiler_params=pltpu.CompilerParams(vmem_limit_bytes=120 * 2 ** 20),
    )(jnp.transpose(x, (0, 2, 3, 1)), t_emb, g1, be1, as_taps(w1), w_emb,
      g2, be2, as_taps(w2))
    return jnp.transpose(out, (0, 3, 1, 2))


@jax.jit
def pallas_standalone__adm_resblock__diffusion_kernel(
    x: jax.Array,
    t_emb: jax.Array,
    g1: jax.Array,
    be1: jax.Array,
    w1: jax.Array,
    w_emb: jax.Array,
    g2: jax.Array,
    be2: jax.Array,
    w2: jax.Array,
):
    return _resblock(_CFG, x, t_emb, g1, be1, w1, w_emb, g2, be2, w2)
```

```python
import functools

import jax
import jax.numpy as jnp
from jax.experimental import pallas as pl
from jax.experimental.pallas import tpu as pltpu

F32, BF16, U32 = jnp.float32, jnp.bfloat16, jnp.uint32

NB, C, HW, NG = 2, 512, 64, 4
EPS = 1e-5
TR = 8
M = 16 * TR
M_PITCH = M + 16
T_ROWS = 33
TICKS = M // 8
ORDER = [(xi, nu) for xi in range(6) for nu in range(6)]

PA, PB = 2.0 / 3.0, 1.5
A2, B2, B3 = PA * PA, PB * PB, PB * PB * PB
DD = A2 - B2


def _xf_in(d):
    p2, q2 = B2 * d[2], A2 * d[2]
    ea, eb = d[4] - p2, d[4] - q2
    p3, q3 = A2 * d[3], B2 * d[3]
    ua, ub = d[1] - p3, d[1] - q3
    v0 = (ea if d[0] is None else d[0] + ea) - q2
    v5 = (ua if d[5] is None else d[5] + ua) - q3
    oa, ob = PB * ua, PA * ub
    return [v0, ea - oa, ea + oa, eb - ob, eb + ob, v5]


def _xf_out(m):
    sa, da, sb, db = m[1] + m[2], m[1] - m[2], m[3] + m[4], m[3] - m[4]
    return [(m[0] + sb) + B3 * sa, PB * da + db, sa + PB * sb, (da + m[5]) + B3 * db]


def _xf_w(g):
    ca, cb = PA ** 3 / (2 * A2 * DD), -1.0 / (2 * B2 * DD)
    ea, eb = ca * g[0] + (ca * A2) * g[2], cb * g[0] + (cb * B2) * g[2]
    oa, ob = (ca * PA) * g[1], (cb * PB) * g[1]
    return [g[0], ea + oa, ea - oa, eb + ob, eb - ob, g[2]]


def _unpack(w, half):
    return pltpu.unpack_elementwise(w, index=half, packed_dtype=BF16, unpacked_dtype=F32)


def _pack(lo, hi):
    return pltpu.pack_elementwise([lo, hi], packed_dtype=BF16)


def _mean_all(v):
    return jnp.sum(jnp.sum(v, axis=0, keepdims=True), axis=1, keepdims=True) * (1.0 / v.size)


class _Item:
    def __init__(self, cost, src, dst, fn):
        self.cost, self.src, self.dst, self.fn = cost, src, dst, fn

    def slack(self, cfg):
        return cfg["slack"] + dict(cfg["dslack"]).get(getattr(getattr(self.fn, "func", None), "__name__", ""), 0)


class _Pacer:
    def __init__(self, zero):
        self.zero = zero

    def move(self, zero):
        self.zero = zero

    def _slot(self, buf, which):
        lanes = pl.ds(0, 128)
        if buf.shape[-2] > 8:
            return (self.zero,) + (0,) * (len(buf.shape) - 3) + (pl.ds(8 * which, 8), lanes)
        return (self.zero,) + (0,) * (len(buf.shape) - 4) + (which, pl.ds(0, 8), lanes)

    def init(self, buf):
        for which in range(2):
            buf[self._slot(buf, which)] = jnp.zeros((8, 128), buf.dtype)

    def release(self, buf, value, which=0):
        if value.dtype != buf.dtype:
            value = pltpu.bitcast(value, buf.dtype)
        buf[self._slot(buf, which)] = value

    def done(self, buf):
        return buf[self._slot(buf, 1)]


def _spread(streams):
    keyed = []
    for groups, lo, hi in streams:
        total = max(sum(it.cost for grp in groups for it in grp), 1)
        acc = 0
        for grp in groups:
            cost = sum(it.cost for it in grp)
            keyed.append((lo + (hi - lo) * (acc + cost / 2) / total, len(keyed), grp))
            acc += cost
    keyed.sort(key=lambda t: t[:2])
    phases = {}
    for time, _, grp in keyed:
        phases.setdefault(int(2 * time), []).extend(grp)
    return phases


def _kernel(cfg, x_hbm, t_hbm, g1_hbm, be1_hbm, w1_hbm, wemb_hbm, g2_hbm, be2_hbm, w2_hbm, o_hbm,
            xs0, xs1, h0, h1, wr1, wr2, u1, u2, v0, v1, tb, osb, coef, stat,
            t_s, g1_s, be1_s, g2_s, be2_s, wemb_s, emb_s, tcol, affine, sems, *ms):
    xs_bf, wr_bf = (xs0, xs1), (wr1, wr2)
    xs = tuple(r.bitcast(U32) for r in xs_bf)
    wr = tuple(r.bitcast(U32) for r in wr_bf)
    hs, us, vs = (h0, h1), (u1, u2), (v0, v1)
    part = functools.partial
    lanes = lambda g: pl.ds(g * 128, 128)

    xp = cfg["x_pieces"]
    xr = HW // xp
    n_head = NG * (xp + 1)

    def x_copy(b, g, r0, nr, sem):
        return pltpu.make_async_copy(x_hbm.at[b, pl.ds(r0, nr), :, lanes(g)],
                                     xs_bf[b].at[pl.ds(1 + g * HW + r0, nr)], sems.at[sem])

    def w_copy(cv, n0, n1, g, sem):
        rows = pl.ds(n0 * 128, (n1 - n0) * 128)
        return pltpu.make_async_copy((w1_hbm, w2_hbm)[cv].at[:, rows, lanes(g)],
                                     wr_bf[cv].at[pl.ds(1 + g * 9, 9), rows], sems.at[sem])

    x0_copy = lambda g, q: x_copy(0, g, q * xr, xr, g * (xp + 1) + q)
    w0_copy = lambda g: w_copy(0, 0, 1, g, g * (xp + 1) + xp)
    w_of = lambda cv, n0, n1, sem: [w_copy(cv, n0, n1, g, n_head + sem) for g in range(NG)]
    small = [pltpu.make_async_copy(s, d, sems.at[n_head]) for s, d in
             ((g1_hbm, g1_s), (be1_hbm, be1_s), (g2_hbm, g2_s), (be2_hbm, be2_s), (t_hbm, t_s))]
    late = [w_of(0, 1, 2, 1), w_of(0, 2, 4, 2),
            [x_copy(1, g, 0, HW, n_head + 3) for g in range(NG)]
            + [pltpu.make_async_copy(wemb_hbm, wemb_s, sems.at[n_head + 3])], w_of(1, 0, 3, 4), w_of(1, 3, 4, 5)]
    first = []
    for g in range(NG):
        xw = [x0_copy(g, q) for q in range(xp)], [w0_copy(g)]
        first += xw[1] + xw[0] if cfg["w_lead"] else xw[0] + xw[1]
    for d in first[:1] + small + first[1:] + [d for dmas in late for d in dmas]:
        d.start()

    ready = set()

    def need(*keys):
        assert p_lo >= 0 or all(key in ready for key in keys), keys

    sub = jax.lax.broadcasted_iota(jnp.int32, (8, 128), 0)

    def w_rows(cv, n, g, ob, xis):
        w = [wr[cv][pl.ds(1 + g * 9 + 3 * i, 3), pl.ds(n * 64 + ob * 8, 8)] for i in range(3)]
        c = [_xf_w([_unpack(wi, half) for wi in w]) for half in range(2)]
        for xi in xis:
            ready.add(("w", cv, n, xi, g, ob))
            u = [_xf_w([ch[xi][j] for j in range(3)]) for ch in c]
            for nu in range(6):
                us[cv][1 + n * 36 + nu * 6 + xi, pl.ds(ob * 8, 8), lanes(g)] = _pack(u[0][nu], u[1][nu])

    def w_groups(cv, n, gs, xis):
        return [[_Item(cfg["c_w"], wr[cv], us[cv], part(w_rows, cv, n, g, ob, xis))] for g in gs for ob in range(8)]

    def set_coef(cv, b, g, mean, var, bias):
        gamma, beta = affine[2 * cv, g], affine[2 * cv + 1, g]
        mu = _mean_all(mean)
        dev = mean - mu
        scale = gamma * jax.lax.rsqrt(_mean_all(jnp.maximum(var, 0.0) + dev * dev) + EPS)
        shift = beta + (bias - mu) * scale
        k = (cv * NB + b) * NG + g
        ready.add(("coef", cv, b, g))
        coef[k, 0] = jnp.broadcast_to(0.5 * shift, (8, 128))
        for q, power in enumerate((0, 0, 1, 1, 1, 1, 2, 2) if cv else (0,)):
            coef[k, 1 + q] = jnp.broadcast_to((0.5 * PB ** power) * scale, (8, 128))

    def x_stat_rows(acc, b, g, r0, nr):
        for r in range(r0, r0 + nr):
            w = xs[b][1 + g * HW + r].reshape(2, 2, 8, 128)
            lo, hi = _unpack(w, 0), _unpack(w, 1)
            if not acc:
                acc.append(lo[0])
            lo, hi = lo - acc[0], hi - acc[0]
            s1, s2 = lo + hi, lo * lo + hi * hi
            s1, s2 = s1[0] + s1[1], s2[0] + s2[1]
            acc[1:] = [acc[1] + s1, acc[2] + s2] if acc[1:] else [s1, s2]
        stat[0, pl.ds(2, 2)] = acc[1]
        stat[0, pl.ds(4, 2)] = acc[2]

    def x_stat_end(acc, b, g):
        if not acc: return
        ref, m1, m2 = acc[0], acc[1] * (1.0 / (HW * 4)), acc[2] * (1.0 / (HW * 4))
        set_coef(0, b, g, (ref + m1).reshape(16, 128), (m2 - m1 * m1).reshape(16, 128), 0.0)

    def x_stat_groups(b, g, waits):
        acc, out, nr = [], [], cfg["stat_rows"]
        for r0 in range(0, HW, nr):
            grp = [_Item(0, None, None, waits[r0].wait)] if r0 in waits else []
            out.append(grp + [_Item(cfg["c_st"] * nr, xs[b], stat, part(x_stat_rows, acc, b, g, r0, nr))])
        out.append([_Item(30, None, None, part(x_stat_end, acc, b, g))])
        return out

    def h_stat_end(b, g):
        need("emb", ("out", (2 * b + 1) * NG + g))
        s = stat[1 + b * NG + g]
        inv = 1.0 / (HW * 8)
        m1 = (s[0] + PB * (s[1] + PB * s[2])) * inv
        m2 = (s[3] + B2 * (s[4] + B2 * s[5])) * inv
        e = emb_s[pl.ds(b, 1), lanes(g)]
        set_coef(1, b, g, m1 + e, m2 - m1 * m1, e)

    def emb_rows(acc, e0):
        if e0 % 128 == 0:
            t = t_s[:, pl.ds(e0, 128)].astype(F32)
            t = t * jax.nn.sigmoid(t)
            for b in range(NB):
                tcol[b] = jnp.broadcast_to(t[b:b + 1], (128, 128)).T
        for r in range(e0, e0 + 32, 8):
            w = wemb_s[pl.ds(r, 8)].astype(F32)
            for b in range(NB):
                term = w * jnp.concatenate([tcol[b, pl.ds(r % 128, 8)]] * NG, axis=1)
                acc[b] = acc[b] + term if b in acc else term
        stat[0, pl.ds(2, NG)] = jnp.stack([acc[NB - 1][:, g * 128:(g + 1) * 128] for g in range(NG)])

    def emb_groups():
        acc = {}

        def end():
            ready.add("emb")
            for b in range(NB):
                emb_s[pl.ds(b, 1)] = jnp.sum(acc[b], axis=0, keepdims=True)

        return ([[_Item(84, None, stat, part(emb_rows, acc, e0))] for e0 in range(0, t_s.shape[1], 32)]
                + [[_Item(40, None, None, end)]])

    def silu(z, scale, shift):
        u = z * scale + shift
        return u + u * jnp.tanh(u)

    def in_row(cv, b, g, h):
        k = (cv * NB + b) * NG + g
        need(("coef", cv, b, g))
        if cv == 0:
            row = 1 + g * HW + h
            w = jnp.concatenate([xs[b][row, pl.ds(jp, 8, stride=4)] for jp in range(4)]).reshape(2, 2, 8, 128)
            scale, shift = coef[k, 1], coef[k, 0]
            lo, hi = silu(_unpack(w, 0), scale, shift), silu(_unpack(w, 1), scale, shift)
            d = [lo[:, 0], hi[:, 0], lo[:, 1], hi[:, 1]]
        else:
            a = silu(hs[b][1 + h * NG + g], coef[k, pl.ds(1 if h % 4 in (0, 3) else 5, 4)], coef[k, 0])
            d = [a[:, 0], a[:, 2], a[:, 3], a[:, 1]]
        left = jnp.where(sub == 0, 0.0, pltpu.roll(d[3][1], 1, 0))
        right = jnp.where(sub == 7, 0.0, pltpu.roll(d[0][0], 7, 0))
        v = _xf_in([jnp.stack([left, d[3][0]])] + d + [jnp.stack([d[0][1], right])])
        for nu in range(6):
            tb[1 + g * T_ROWS + h % T_ROWS, :, nu] = v[nu]

    def in_col(vn, g, r, nu0, nnu):
        rows = range(4 * r - 1, 4 * r + 5)
        v = [_xf_in([tb[1 + g * T_ROWS + h % T_ROWS, p, pl.ds(nu0, nnu)] if 0 <= h < HW else None for h in rows])
             for p in range(2)]
        for xi in range(6):
            vn[pl.ds(1 + xi * 6 + nu0, nnu), pl.ds(r % TR * 8, 8), lanes(g)] = _pack(v[0][xi], v[1][xi])

    def in_groups(c, g):
        cv, b, r0 = c // 4, (c // 2) % 2, (c % 2) * TR
        src, cost = (xs[b], cfg["c_rowx"]) if cv == 0 else (hs[b], cfg["c_rowh"])
        row = lambda h: [_Item(cost, src, tb, part(in_row, cv, b, g, h))]
        out, nnu = [row(0)] if r0 == 0 else [], cfg["nnu"]
        for r in range(r0, r0 + TR + 1):
            rows = [row(h) for h in range(4 * r + 1, min(4 * r + 5, HW))] if r < r0 + TR else []
            cols = [[_Item(cfg["c_col"] * nnu, tb, vs[c % 2], part(in_col, vs[c % 2], g, r - 1, nu0, nnu))]
                    for nu0 in range(0, 6, nnu)] if r > r0 else []
            out += [grp for _, grp in sorted(
                [((q + 0.25) / len(rows), grp) for q, grp in enumerate(rows)]
                + [((q + 0.75) / len(cols), grp) for q, grp in enumerate(cols)], key=lambda t: t[0])]
        out[-1].append(_Item(0, None, None, part(ready.add, ("in", c, g))))
        if c > 1:
            out[0].insert(0, _Item(0, None, None, part(need, ("mm", c * NG - NG - 1))))
        return out

    def out_first(cv, mp, r, p, xi0, nxi, slot):
        y = _xf_out([mp[pl.ds(1 + nu * 6 + xi0, nxi), pl.ds(r % TR * 16 + p, 8, stride=2)] for nu in range(6)])
        for q, j in enumerate((0, 1, 2, 3) if cv else (0, 3, 1, 2)):
            osb[1 + slot * 4 + q, pl.ds(xi0, nxi)] = y[j]

    def out_second(acc, cv, b, n, r, p, jp, slot):
        y = _xf_out([osb[pl.ds(1 + slot * 4 + 2 * jp, 2), xi] for xi in range(6)])
        if not acc: acc.extend(jnp.zeros((8, 128), F32) for q in range(6))
        if cv == 0:
            for i in range(4):
                hs[b][1 + (4 * r + i) * NG + n, p, pl.ds(2 * jp, 2)] = y[i]
            for power, ya, yb in ((jp, y[0], y[3]), (jp + 1, y[1], y[2])):
                s1, s2 = ya + yb, ya * ya + yb * yb
                acc[power] = acc[power] + (s1[0] + s1[1])
                acc[3 + power] = acc[3 + power] + (s2[0] + s2[1])
        else:
            for i in range(4):
                at = (1 + n * HW + 4 * r + i, pl.ds(2 * p + jp, 8, stride=4))
                w, res = xs[b][at], []
                for q in range(2):
                    power = (i in (1, 2)) + (2 * jp + q in (1, 2))
                    res.append(_unpack(w, q) + (y[i][q] * PB ** power if power else y[i][q]))
                xs[b][at] = _pack(*res)

    out_dmas, os_count = [], [0]

    def out_groups(phase):
        c, n = divmod(phase, NG)
        cv, b, r0 = c // 4, (c // 2) % 2, (c % 2) * TR
        mp, acc, nxi = ms[phase % len(ms)], [], cfg["o_nxi"]

        def begin():
            acc.extend(stat[1 + b * NG + n, q] if r0 else jnp.zeros((8, 128), F32) for q in range(6))

        def end():
            for q in range(6):
                stat[1 + b * NG + n, q] = acc[q]

        def send(h0, nr):
            out_dmas.append(lambda: pltpu.make_async_copy(
                xs_bf[b].at[pl.ds(1 + n * HW + h0, nr)], o_hbm.at[b, pl.ds(h0, nr), :, lanes(n)],
                sems.at[min(phase - 16, len(cfg["t_split"]))]))
            out_dmas[-1]().start()

        units = [(r, p) for r in range(r0, r0 + TR) for p in range(2)]
        send_rows = cfg["last_send"] if phase == 31 else TR
        out = [[_Item(0, None, None, begin)]] if cv == 0 else []
        for q in range(len(units) + 1):
            slot = os_count[0] % 2
            firsts = [[_Item(cfg["c_o1"] * nxi, mp, osb, part(out_first, cv, mp, *units[q], xi0, nxi, slot))]
                      for xi0 in range(0, 6, nxi)] if q < len(units) else []
            seconds = [[_Item(cfg["c_o2"], osb, (hs, xs)[cv][b],
                              part(out_second, acc, cv, b, n, *units[q - 1], jp, 1 - slot))]
                       for jp in range(2)] if q > 0 else []
            os_count[0] += bool(firsts)
            out += [grp for _, grp in sorted(
                [((k + 0.25) / len(firsts), grp) for k, grp in enumerate(firsts)]
                + [((k + 0.75) / len(seconds), grp) for k, grp in enumerate(seconds)], key=lambda t: t[0])]
            if cv == 1 and q > 0 and q % (2 * send_rows) == 0:
                out[-1].append(_Item(0, None, None, part(send, 4 * (r0 + q // 2 - send_rows), 4 * send_rows)))
        if cv == 0:
            out[-1].append(_Item(0, None, None, end))
        out[-1].append(_Item(0, None, None, part(ready.add, ("out", phase))))
        out[0].insert(0, _Item(0, None, None, part(need, ("mm", phase))))
        return out

    def load_lhs(vc, ks, cols, dues):
        cuts = sorted({0, TR} | set(dues))
        blocks = [[] for _ in ks]
        for lo, hi in zip(cuts, cuts[1:]):
            for value in dues.get(lo, ()):
                pace.release(vc, value)
            if dues.get(lo) and cfg["soft"] and (lo % cfg["soft"] or cfg["soft"] == 1):
                pace.release(vc, jnp.zeros((8, 128), U32))
            for blk, (xi, nu) in zip(blocks, ks):
                blk.append(vc[1 + xi * 6 + nu, pl.ds(lo * 8, (hi - lo) * 8), cols])
        return [pltpu.bitcast(jnp.concatenate(blk, axis=0), BF16) for blk in blocks]

    def dot(lhs, rhs):
        return jax.lax.dot_general(lhs, pltpu.bitcast(rhs, BF16), (((1,), (1,)), ((), ())),
                                   preferred_element_type=F32)

    def matmul(phase, xi, nu, dues):
        c, n = divmod(phase, NG)
        need(("in", c, NG - 1), ("w", c // 4, n, xi, NG - 1, 7), *[("out", phase - len(ms))] * (phase >= len(ms)))
        if (xi, nu) == ORDER[-1]:
            ready.add(("mm", phase))
        lhs, = load_lhs(vs[c % 2], [(xi, nu)], slice(None), dues)
        res = dot(lhs, us[c // 4][1 + n * 36 + nu * 6 + xi])
        ms[phase % len(ms)][1 + nu * 6 + xi, pl.ds(0, M)] = res
        return res

    def matmul_part(g, ks, dues):
        need(("in", 0, g), ("w", 0, 0, 4, g, 7))
        ready.add(("mm", 0))
        for lhs, (xi, nu) in zip(load_lhs(vs[0], ks, lanes(g), dues), ks):
            res = dot(lhs, us[0][1 + nu * 6 + xi, :, lanes(g)])
            at = (1 + nu * 6 + xi, pl.ds(0, M))
            res = ms[0][at] + res if g else res
            ms[0][at] = res
        return res

    def steps(phase, g=NG - 1):
        if phase == 0:
            return [part(matmul_part, g, ORDER[q:q + 4]) for q in range(0, 36, 4)]
        return [part(matmul, phase, *k) for k in ORDER]

    dsts = lambda it: it.dst if isinstance(it.dst, tuple) else () if it.dst is None else (it.dst,)

    def run_alone(groups, window):
        finished, acc = [], 0
        for it in (it for grp in groups for it in grp):
            ready = [v for t, v in finished if t <= acc - window]
            if it.src is not None and ready:
                pace.release(it.src, ready[-1])
            it.fn()
            acc += it.cost
            for dst in dsts(it):
                finished.append((acc, pace.done(dst)))
            del finished[:-24]

    clock, pending, todo, chain, spent = [], {}, [], [], [0]

    def advance(tick):
        while todo and len(clock) * TICKS <= tick:
            now, dues = len(clock) * TICKS, {}
            for key in [key for key in pending if key[0] < now + TICKS]:
                dues.setdefault(max(key[0] - now, 0) // 2, []).append(pending.pop(key))
            for rb in range(0, TR if cfg["pop_lag"] else 0, cfg["pop_every"]):
                t = min(now + 2 * rb - cfg["pop_lag"], now - 1)
                if t >= 0:
                    dues.setdefault(rb, []).append(clock[t // TICKS][t % TICKS * 8:t % TICKS * 8 + 8])
            clock.append(todo.pop(0)(dues))

    def run_paced(matmuls, items, stretch=1.0):
        lead, slack, win = cfg["lead"], cfg["slack"], cfg["win"]
        t0, span = len(clock) * TICKS, len(matmuls) * TICKS
        total, acc, last = max(sum(it.cost for it in items), 1) / stretch, 0, {}
        todo.extend(matmuls)
        for it in items:
            start = t0 + int(acc / total * span) // win * win - lead
            acc += it.cost
            advance(start)
            if it.src is not None:
                if 0 <= start < t0 + span and last.get(id(it.src)) != start:
                    last[id(it.src)] = start
                    pace.release(it.src, clock[start // TICKS][start % TICKS * 8:start % TICKS * 8 + 8])
                if cfg["chain"]:
                    older = [v for t, v in chain if t <= spent[0] - cfg["chain"]]
                    pace.release(it.src, older[-1] if older else jnp.zeros((8, 128), it.src.dtype))
            it.fn()
            spent[0] += it.cost
            for dst in dsts(it):
                chain.append((spent[0], pace.done(dst)))
                pending[-(-(t0 + int(acc / total * span) - lead + slack) // 2) * 2, id(dst)] = chain[-1][1]
            del chain[:-32]
        advance(t0 + span)

    def forget():
        del clock[:], chain[:]
        pending.clear()

    p_lo, p_hi = cfg["only"]

    sc = [None, 0]
    def scope(name):
        if not cfg.get("scopes"): return
        if sc[0] is not None: sc[0].__exit__(None, None, None)
        sc[0] = jax.named_scope(f"s_{sc[1]:02d}{name}") if name else None
        sc[1] += 1
        if sc[0] is not None: sc[0].__enter__()
    def waits(dmas):
        scope("wait")
        for d in dmas: d.wait()
        scope("run")
    waits(small)
    for q, ref in enumerate((g1_s, be1_s, g2_s, be2_s)):
        value = ref[...].astype(F32)
        for g in range(NG):
            affine[q, g] = jnp.broadcast_to(value[g * 128:(g + 1) * 128][None, :], (8, 128))
    pace = _Pacer(0)
    for buf in (*xs, *hs, *wr, *us, *vs, *ms, tb, osb, stat):
        pace.init(buf)

    pace.move(jax.lax.fori_loop(0, 2, lambda i, z: z + (i >> 10), jnp.int32(0)))

    cfg = dict(cfg, **cfg["HH"])
    for g in range(NG if p_lo < 0 else 0):
        stats = x_stat_groups(0, g, {q * xr: x0_copy(g, q) for q in range(xp)})
        run_alone(stats[:-1], cfg["alone"])
        waits([w0_copy(g)])
        work = stats[-1:] + w_groups(0, 0, [g], (0, 1, 2)) + w_groups(0, 0, [g], (3, 4, 5)) + in_groups(0, g)
        if g == 0:
            run_alone(work, cfg["alone"])
        else:
            run_paced(steps(0, g - 1), [it for grp in work for it in grp], cfg["stretch"])
            forget()

    if p_lo >= 0:
        for d in first: d.wait()
        for time, dmas in zip(cfg["t_wait"], late):
            if not p_lo < time < p_hi:
                for d in dmas: d.wait()
        scope("go")
    streams = []
    for c in range(1, 8):
        groups = []
        for g in range(NG):
            if c in (4, 6):
                groups.append([_Item(30, None, None, part(h_stat_end, (c - 4) // 2, g))])
            groups += in_groups(c, g)
        if c == 1:
            cut = int(len(groups) * cfg["in1"])
            streams += [(groups[:cut], 1.0, 3.5), (groups[cut:], 3.5, 3.98)]
        else:
            streams.append((groups, *cfg["t_in"][c - 2]))
    streams.append(([grp for g in range(NG) for grp in x_stat_groups(1, g, {})], *cfg["t_stat"]))
    w_times = cfg["t_w"]
    for k, (cv, n) in enumerate([(cv, n) for cv in range(2) for n in range(NG)][1:]):
        t = w_times[k]
        streams += [(w_groups(cv, n, range(NG), (0, 1, 2)), t[0], t[1]), (w_groups(cv, n, range(NG), (3, 4, 5)), t[1], t[2])]
    t_out = cfg["t_out"]
    for p in range(31):
        assert p + 1 <= t_out[p] and t_out[p + 1] <= p + len(ms)
        streams.append((out_groups(p), t_out[p], t_out[p + 1]))
    streams.append((emb_groups(), *cfg["t_emb"]))
    for time, dmas in zip(cfg["t_wait"], late):
        if p_lo < 0 or p_lo < time < p_hi:
          streams.insert(0, ([[_Item(0, None, None, part(waits, dmas))]], time, time))
    for time in cfg["t_split"]:
        streams.insert(0, ([[_Item(0, None, None, lambda: waits([out_dmas.pop(0)()]) if out_dmas else None)]], time, time))
    phases = _spread(streams)
    if cfg.get("show"):
        print("load", [2 * sum(it.cost for it in phases[p]) + 1728 for p in sorted(phases)])
    def run_phases(p0, p1):
        nonlocal cfg
        for p in range(p0, p1):
            cfg = dict(cfg, **(cfg["L"] if p in cfg["light"] else cfg["HH"] if p < 4 else cfg["H"]))
            if p == 0:
                run_paced(steps(p), phases[0] + phases[1])
            else:
                run_paced(steps(p)[:18], phases[2 * p])
                run_paced(steps(p)[18:], phases[2 * p + 1])

    p = max(p_lo, 0)
    for p0, p1 in cfg["loops"]:
        if p_lo <= p0 and p1 <= p_hi:
            run_phases(p, p0)
            forget()
            jax.lax.fori_loop(0, pace.zero + 1, lambda i, _: run_phases(p0, p1), None)
            forget()
            p = p1
    run_phases(p, min(p_hi, 32))
    scope("tail")
    if p_hi > 32:
        run_alone([phases.get(64, [])] + out_groups(31), cfg["alone"])
    scope("last")
    for time, dmas in zip(cfg["t_wait"], late):
        if p_lo < 0 and time >= p_hi:
            for d in dmas: d.wait()
    for d in out_dmas:
        d().wait()
    scope(None)


def H(soft, chain, slack, pop_lag, pop_every=1, kill=1):
    return dict(soft=soft, kill=kill, chain=chain, slack=slack, pop_lag=pop_lag, pop_every=pop_every)


def _lin(points, n):
    out = []
    for i in range(n):
        (i0, v0), (i1, v1) = next((a, b) for a, b in zip(points, points[1:]) if a[0] <= i <= b[0])
        out.append(v0 + (v1 - v0) * (i - i0) / (i1 - i0))
    return tuple(out)


_CFG = dict(
    only=(-1, 33), lead=16, slack=40, win=2, alone=500, stretch=1.1, n_m=5, ahead=0, vclk=0, clk_slot=0, soft=1, kill=1, chain=7, clk_every=1, pop_every=2, pop_lag=22,
    dslack=(), L=dict(soft=0, kill=0, chain=0, slack=24, pop_lag=0, pop_every=1),
    H=dict(soft=4, kill=1, chain=140, slack=28, pop_lag=20, pop_every=1), light=tuple(range(22, 32)),
    c_rowx=88, c_rowh=80, c_col=42, c_o1=14, c_o2=52, c_w=140, c_st=40,
    nnu=1, o_nxi=3, w_nxi=1, w_direct=True, w_lead=False,
    x_pieces=2, stat_rows=2, last_send=2, t_emb=(7.2, 9.6),
    t_wait=(0.0, 1.5, 4.0, 10.0, 16.0), t_split=(22.0, 27.0), loops=(),
    HH=dict(soft=4, kill=1, chain=450, slack=24, pop_lag=20, pop_every=1), in1=0.67,
    t_in=((4.8, 7.98), (8.0, 11.98), (12.0, 15.98), (16.0, 19.98), (20.0, 23.98), (24.0, 27.98)),
    t_stat=(4.0, 6.8),
    t_w=((0.0, 0.99, 1.47), (1.5, 1.97, 2.47), (2.5, 2.97, 3.47), (10.0, 11.2, 12.4), (12.4, 13.6, 14.8), (14.8, 16.0, 17.2), (17.2, 18.4, 19.47)),
    t_out=_lin(((0, 4.0), (2, 4.9), (5, 8.0), (8, 10.0), (15, 18.5), (16, 19.5), (20, 21.3), (22, 23.04), (31, 32.0)), 32),
)


def H(soft, chain, slack, pop_lag, pop_every=1, kill=1):
    return dict(soft=soft, kill=kill, chain=chain, slack=slack, pop_lag=pop_lag, pop_every=pop_every)


def _resblock(cfg, x, t_emb, g1, be1, w1, w_emb, g2, be2, w2):
    assert x.shape == (NB, C, HW, HW) and w1.shape == w2.shape == (C, C, 3, 3)
    emb_dim = t_emb.shape[1]
    vmem = pltpu.VMEM
    scratch = (
        [vmem((1 + NG * HW, HW, 128), BF16)] * 2
        + [vmem((1 + HW * NG, 2, 4, 8, 128), F32)] * 2
        + [vmem((1 + NG * 9, C, 128), BF16)] * 2
        + [vmem((1 + NG * 36, 64, C), U32)] * 2
        + [vmem((1 + 36, M // 2, C), U32)] * 2
        + [vmem((1 + NG * T_ROWS, 2, 7, 8, 128), F32),
           vmem((1 + 2 * 4, 7, 8, 128), F32),
           vmem((2 * NB * NG, 9, 8, 128), F32),
           vmem((1 + NB * NG, 6, 8, 128), F32),
           vmem((NB, emb_dim), BF16)]
        + [vmem((C,), BF16)] * 4
        + [vmem((emb_dim, C), BF16), vmem((NB, C), F32), vmem((NB, 128, 128), F32), vmem((4, NG, 8, 128), F32), pltpu.SemaphoreType.DMA((NG * (cfg["x_pieces"] + 1) + 6,))]
        + [vmem((1 + 36, M_PITCH, 128), F32)] * cfg["n_m"]
    )
    as_taps = lambda w: jnp.transpose(w, (2, 3, 0, 1)).reshape(9, C, C)
    out = pl.pallas_call(
        functools.partial(_kernel, cfg),
        out_shape=jax.ShapeDtypeStruct((NB, HW, HW, C), x.dtype),
        in_specs=[pl.BlockSpec(memory_space=pl.ANY)] * 9,
        out_specs=pl.BlockSpec(memory_space=pl.ANY),
        scratch_shapes=scratch,
        compiler_params=pltpu.CompilerParams(vmem_limit_bytes=120 * 2 ** 20),
    )(jnp.transpose(x, (0, 2, 3, 1)), t_emb, g1, be1, as_taps(w1), w_emb,
      g2, be2, as_taps(w2))
    return jnp.transpose(out, (0, 3, 1, 2))


@jax.jit
def pallas_standalone__adm_resblock__diffusion_kernel(
    x: jax.Array,
    t_emb: jax.Array,
    g1: jax.Array,
    be1: jax.Array,
    w1: jax.Array,
    w_emb: jax.Array,
    g2: jax.Array,
    be2: jax.Array,
    w2: jax.Array,
):
    return _resblock(_CFG, x, t_emb, g1, be1, w1, w_emb, g2, be2, w2)
```

```python
import functools

import jax
import jax.numpy as jnp
from jax.experimental import pallas as pl
from jax.experimental.pallas import tpu as pltpu

F32, BF16, U32 = jnp.float32, jnp.bfloat16, jnp.uint32

NB, C, HW, NG = 2, 512, 64, 4
EPS = 1e-5
TR = 8
M = 16 * TR
M_PITCH = M + 16
T_ROWS = 33
TICKS = M // 8
ORDER = [(xi, nu) for xi in range(6) for nu in range(6)]

PA, PB = 2.0 / 3.0, 1.5
A2, B2 = PA * PA, PB * PB
DD = A2 - B2


def _xf_in(d):
    p2, q2 = B2 * d[2], A2 * d[2]
    ea, eb = d[4] - p2, d[4] - q2
    p3, q3 = A2 * d[3], B2 * d[3]
    ua, ub = d[1] - p3, d[1] - q3
    v0 = (ea if d[0] is None else d[0] + ea) - q2
    v5 = (ua if d[5] is None else d[5] + ua) - q3
    oa, ob = PB * ua, PA * ub
    return [v0, ea - oa, ea + oa, eb - ob, eb + ob, v5]


def _xf_out(m):
    sa, da, sb, db = m[1] + m[2], m[1] - m[2], m[3] + m[4], m[3] - m[4]
    return [None if m[0] is None else (m[0] + sb) + sa, PA * da + PB * db, A2 * sa + B2 * sb,
            None if m[5] is None else (PA ** 3 * da + m[5]) + PB ** 3 * db]


def _xf_w(g):
    t = g[2] * (1.0 / (2 * DD))
    ea, eb = g[0] * (1.0 / (2 * A2 * DD)) + t, g[0] * (-1.0 / (2 * B2 * DD)) - t
    oa, ob = g[1] * (PB / (2 * DD)), g[1] * (-PA / (2 * DD))
    return [g[0], ea + oa, ea - oa, eb + ob, eb - ob, g[2]]


def _unpack(w, half):
    return pltpu.unpack_elementwise(w, index=half, packed_dtype=BF16, unpacked_dtype=F32)


def _pack(lo, hi):
    return pltpu.pack_elementwise([lo, hi], packed_dtype=BF16)


def _mean_all(v):
    return jnp.sum(jnp.sum(v, axis=0, keepdims=True), axis=1, keepdims=True) * (1.0 / v.size)


class _Item:
    def __init__(self, cost, src, dst, fn):
        self.cost, self.src, self.dst, self.fn = cost, src, dst, fn

    def slack(self, cfg):
        return cfg["slack"] + dict(cfg["dslack"]).get(getattr(getattr(self.fn, "func", None), "__name__", ""), 0)


class _Pacer:
    def __init__(self, zero):
        self.zero = zero

    def move(self, zero):
        self.zero = zero

    def _slot(self, buf, which):
        lanes = pl.ds(0, 128)
        if buf.shape[-2] > 8:
            return (self.zero,) + (0,) * (len(buf.shape) - 3) + (pl.ds(8 * which, 8), lanes)
        return (self.zero,) + (0,) * (len(buf.shape) - 4) + (which, pl.ds(0, 8), lanes)

    def init(self, buf):
        for which in range(2):
            buf[self._slot(buf, which)] = jnp.zeros((8, 128), buf.dtype)

    def release(self, buf, value, which=0):
        if value.dtype != buf.dtype:
            value = pltpu.bitcast(value, buf.dtype)
        buf[self._slot(buf, which)] = value

    def done(self, buf):
        return buf[self._slot(buf, 1)]


def _spread(streams):
    keyed = []
    for groups, lo, hi in streams:
        total = max(sum(it.cost for grp in groups for it in grp), 1)
        acc = 0
        for grp in groups:
            cost = sum(it.cost for it in grp)
            keyed.append((lo + (hi - lo) * (acc + cost / 2) / total, len(keyed), grp))
            acc += cost
    keyed.sort(key=lambda t: t[:2])
    phases = {}
    for time, _, grp in keyed:
        phases.setdefault(int(2 * time), []).extend(grp)
    return phases


def _kernel(cfg, x_hbm, t_hbm, g1_hbm, be1_hbm, w1_hbm, wemb_hbm, g2_hbm, be2_hbm, w2_hbm, o_hbm,
            xs0, xs1, h0, h1, wr1, wr2, u1, u2, v0, v1, tb, osb, coef, stat,
            t_s, g1_s, be1_s, g2_s, be2_s, wemb_s, emb_s, tcol, affine, sems, *ms):
    xs_bf, wr_bf = (xs0, xs1), (wr1, wr2)
    xs = tuple(r.bitcast(U32) for r in xs_bf)
    wr = tuple(r.bitcast(U32) for r in wr_bf)
    hs, us, vs = (h0, h1), (u1, u2), (v0, v1)
    part = functools.partial
    lanes = lambda g: pl.ds(g * 128, 128)

    xp = cfg["x_pieces"]
    xr = HW // xp
    n_head = NG * (xp + 1)

    def x_copy(b, g, r0, nr, sem):
        return pltpu.make_async_copy(x_hbm.at[b, pl.ds(r0, nr), :, lanes(g)],
                                     xs_bf[b].at[pl.ds(1 + g * HW + r0, nr)], sems.at[sem])

    def w_copy(cv, n0, n1, g, sem):
        rows = pl.ds(n0 * 128, (n1 - n0) * 128)
        return pltpu.make_async_copy((w1_hbm, w2_hbm)[cv].at[:, rows, lanes(g)],
                                     wr_bf[cv].at[pl.ds(1 + g * 9, 9), rows], sems.at[sem])

    x0_copy = lambda g, q: x_copy(0, g, q * xr, xr, g * (xp + 1) + q)
    w0_copy = lambda g: w_copy(0, 0, 1, g, g * (xp + 1) + xp)
    w_of = lambda cv, n0, n1, sem: [w_copy(cv, n0, n1, g, n_head + sem) for g in range(NG)]
    small = [pltpu.make_async_copy(s, d, sems.at[n_head]) for s, d in
             ((g1_hbm, g1_s), (be1_hbm, be1_s), (g2_hbm, g2_s), (be2_hbm, be2_s), (t_hbm, t_s))]
    late = [w_of(0, 1, 2, 1), w_of(0, 2, 4, 2),
            [x_copy(1, g, 0, HW, n_head + 3) for g in range(NG)]
            + [pltpu.make_async_copy(wemb_hbm, wemb_s, sems.at[n_head + 3])], w_of(1, 0, 3, 4), w_of(1, 3, 4, 5)]
    first = []
    for g in range(NG):
        xw = [x0_copy(g, q) for q in range(xp)], [w0_copy(g)]
        first += xw[1] + xw[0] if cfg["w_lead"] else xw[0] + xw[1]
    for d in first[:1] + small + first[1:] + [d for dmas in late for d in dmas]:
        d.start()

    ready = set()

    def need(*keys):
        assert p_lo >= 0 or all(key in ready for key in keys), keys

    sub = jax.lax.broadcasted_iota(jnp.int32, (8, 128), 0)

    def w_rows(cv, n, g, ob, xis):
        w = [wr[cv][pl.ds(1 + g * 9 + 3 * i, 3), pl.ds(n * 64 + ob * 8, 8)] for i in range(3)]
        c = [_xf_w([_unpack(wi, half) for wi in w]) for half in range(2)]
        for xi in xis:
            ready.add(("w", cv, n, xi, g, ob))
            u = [_xf_w([ch[xi][j] for j in range(3)]) for ch in c]
            for nu in range(6):
                us[cv][1 + n * 36 + nu * 6 + xi, pl.ds(ob * 8, 8), lanes(g)] = _pack(u[0][nu], u[1][nu])

    def w_groups(cv, n, gs, xis):
        return [[_Item(cfg["c_w"] * len(xis), wr[cv], us[cv], part(w_rows, cv, n, g, ob, xis))] for g in gs for ob in range(8)]

    def set_coef(cv, b, g, mean, var, bias):
        gamma, beta = affine[2 * cv, g], affine[2 * cv + 1, g]
        mu = _mean_all(mean)
        dev = mean - mu
        scale = gamma * jax.lax.rsqrt(_mean_all(jnp.maximum(var, 0.0) + dev * dev) + EPS)
        shift = beta + (bias - mu) * scale
        k = (cv * NB + b) * NG + g
        ready.add(("coef", cv, b, g))
        coef[k, 0] = jnp.broadcast_to(0.5 * shift, (8, 128))
        coef[k, 1] = jnp.broadcast_to(0.5 * scale, (8, 128))

    def x_stat_rows(acc, b, g, r0, nr):
        for r in range(r0, r0 + nr):
            w = xs[b][1 + g * HW + r].reshape(2, 2, 8, 128)
            lo, hi = _unpack(w, 0), _unpack(w, 1)
            if not acc:
                acc.append(lo[0])
            lo, hi = lo - acc[0], hi - acc[0]
            s1, s2 = lo + hi, lo * lo + hi * hi
            s1, s2 = s1[0] + s1[1], s2[0] + s2[1]
            acc[1:] = [acc[1] + s1, acc[2] + s2] if acc[1:] else [s1, s2]
        stat[0, pl.ds(2, 2)] = acc[1]
        stat[0, pl.ds(4, 2)] = acc[2]

    def x_stat_end(acc, b, g):
        if not acc: return
        ref, m1, m2 = acc[0], acc[1] * (1.0 / (HW * 4)), acc[2] * (1.0 / (HW * 4))
        set_coef(0, b, g, (ref + m1).reshape(16, 128), (m2 - m1 * m1).reshape(16, 128), 0.0)

    def x_stat_groups(b, g, waits):
        acc, out, nr = [], [], cfg["stat_rows"]
        for r0 in range(0, HW, nr):
            grp = [_Item(0, None, None, waits[r0].wait)] if r0 in waits else []
            out.append(grp + [_Item(cfg["c_st"] * nr, xs[b], stat, part(x_stat_rows, acc, b, g, r0, nr))])
        out.append([_Item(30, None, None, part(x_stat_end, acc, b, g))])
        return out

    def h_stat_end(b, g):
        need("emb", ("out", (2 * b + 1) * NG + g))
        s = stat[1 + b * NG + g, pl.ds(0, 2)]
        inv = 1.0 / (HW * 8)
        m1, m2 = s[0] * inv, s[1] * inv
        e = emb_s[pl.ds(b, 1), lanes(g)]
        set_coef(1, b, g, m1 + e, m2 - m1 * m1, e)

    def emb_rows(acc, e0):
        if e0 % 128 == 0:
            t = t_s[:, pl.ds(e0, 128)].astype(F32)
            t = t * jax.nn.sigmoid(t)
            for b in range(NB):
                tcol[b] = jnp.broadcast_to(t[b:b + 1], (128, 128)).T
        for r in range(e0, e0 + 32, 8):
            w = wemb_s[pl.ds(r, 8)].astype(F32)
            for b in range(NB):
                term = w * jnp.concatenate([tcol[b, pl.ds(r % 128, 8)]] * NG, axis=1)
                acc[b] = acc[b] + term if b in acc else term
        stat[0, pl.ds(2, NG)] = jnp.stack([acc[NB - 1][:, g * 128:(g + 1) * 128] for g in range(NG)])

    def emb_groups():
        acc = {}

        def end():
            ready.add("emb")
            for b in range(NB):
                emb_s[pl.ds(b, 1)] = jnp.sum(acc[b], axis=0, keepdims=True)

        return ([[_Item(84, None, stat, part(emb_rows, acc, e0))] for e0 in range(0, t_s.shape[1], 32)]
                + [[_Item(40, None, None, end)]])

    def silu(z, scale, shift):
        u = z * scale + shift
        return u + u * jnp.tanh(u)

    def in_row(cv, b, g, h):
        k = (cv * NB + b) * NG + g
        need(("coef", cv, b, g))
        if cv == 0:
            row = 1 + g * HW + h
            w = jnp.concatenate([xs[b][row, pl.ds(jp, 8, stride=4)] for jp in range(4)]).reshape(2, 2, 8, 128)
            scale, shift = coef[k, 1], coef[k, 0]
            lo, hi = silu(_unpack(w, 0), scale, shift), silu(_unpack(w, 1), scale, shift)
            d = [lo[:, 0], hi[:, 0], lo[:, 1], hi[:, 1]]
        else:
            a = silu(hs[b][1 + h * NG + g], coef[k, 1], coef[k, 0])
            d = [a[:, j] for j in range(4)]
        left = jnp.where(sub == 0, 0.0, pltpu.roll(d[3][1], 1, 0))
        right = jnp.where(sub == 7, 0.0, pltpu.roll(d[0][0], 7, 0))
        v = _xf_in([jnp.stack([left, d[3][0]])] + d + [jnp.stack([d[0][1], right])])
        for nu in range(6):
            tb[1 + g * T_ROWS + h % T_ROWS, :, nu] = v[nu]

    def in_col(vn, g, r, nu0, nnu):
        rows = range(4 * r - 1, 4 * r + 5)
        v = [_xf_in([tb[1 + g * T_ROWS + h % T_ROWS, p, pl.ds(nu0, nnu)] if 0 <= h < HW else None for h in rows])
             for p in range(2)]
        for xi in range(6):
            vn[pl.ds(1 + xi * 6 + nu0, nnu), pl.ds(r % TR * 8, 8), lanes(g)] = _pack(v[0][xi], v[1][xi])

    def in_groups(c, g):
        cv, b, r0 = c // 4, (c // 2) % 2, (c % 2) * TR
        src, cost = (xs[b], cfg["c_rowx"]) if cv == 0 else (hs[b], cfg["c_rowh"])
        row = lambda h: [_Item(cost, src, tb, part(in_row, cv, b, g, h))]
        out, nnu = [row(0)] if r0 == 0 else [], cfg["nnu"]
        for r in range(r0, r0 + TR + 1):
            rows = [row(h) for h in range(4 * r + 1, min(4 * r + 5, HW))] if r < r0 + TR else []
            cols = [[_Item(cfg["c_col"] * nnu, tb, vs[c % 2], part(in_col, vs[c % 2], g, r - 1, nu0, nnu))]
                    for nu0 in range(0, 6, nnu)] if r > r0 else []
            out += [grp for _, grp in sorted(
                [((q + 0.25) / len(rows), grp) for q, grp in enumerate(rows)]
                + [((q + 0.75) / len(cols), grp) for q, grp in enumerate(cols)], key=lambda t: t[0])]
        out[-1].append(_Item(0, None, None, part(ready.add, ("in", c, g))))
        if c > 1:
            out[0].insert(0, _Item(0, None, None, part(need, ("mm", c * NG - NG - 1))))
        return out

    def out_first(mp, r, p, xi0, nxi, slot):
        y = _xf_out([mp[pl.ds(1 + nu * 6 + xi0, nxi), pl.ds(r % TR * 16 + p, 8, stride=2)] for nu in range(6)])
        for j in range(4):
            osb[1 + slot * 4 + j, pl.ds(xi0, nxi)] = y[j]

    def out_second(acc, cv, b, n, r, p, jp, slot, rows=(0, 1, 2, 3)):
        y = _xf_out([None if (xi == 0 and 0 not in rows) or (xi == 5 and 3 not in rows) else
                     osb[pl.ds(1 + slot * 4 + 2 * jp, 2), xi] for xi in range(6)])
        if cv == 0:
            if not acc: acc.extend(jnp.zeros((8, 128), F32) for q in range(2))
            for i in rows:
                hs[b][1 + (4 * r + i) * NG + n, p, pl.ds(2 * jp, 2)] = y[i]
            s1 = (y[0] + y[1]) + (y[2] + y[3])
            s2 = (y[0] * y[0] + y[1] * y[1]) + (y[2] * y[2] + y[3] * y[3])
            acc[:] = acc[0] + (s1[0] + s1[1]), acc[1] + (s2[0] + s2[1])
        else:
            for i in rows:
                at = (1 + n * HW + 4 * r + i, pl.ds(2 * p + jp, 8, stride=4))
                w = xs[b][at]
                xs[b][at] = _pack(_unpack(w, 0) + y[i][0], _unpack(w, 1) + y[i][1])

    def send(phase, h0, nr):
        b, n = phase // 8 % 2, phase % NG
        out_dmas.append(lambda: pltpu.make_async_copy(
            xs_bf[b].at[pl.ds(1 + n * HW + h0, nr)], o_hbm.at[b, pl.ds(h0, nr), :, lanes(n)],
            sems.at[min(phase - 16, len(cfg["t_split"]))]))
        out_dmas[-1]().start()

    def last_items():
        mp, units = ms[31 % len(ms)], [(r, p) for r in range(TR, 2 * TR) for p in range(2)]
        first = lambda q, xi0, nxi: _Item(16 * nxi, mp, osb, part(out_first, mp, *units[q], xi0, nxi, 2 + q))
        second = lambda q, rows: [_Item(cost, None, xs[1], part(out_second, None, 1, 1, NG - 1, *units[q], jp, 2 + q, rows))
                                  for cost in [10 + 6 * len(rows)] for jp in range(2)]
        out = [[first(q, 1, 2) for q in range(16)], [], [], []]
        for items, xi0, nxi, rows in zip(out[1:], (3, 0, 5), (2, 1, 1), ((1, 2), (0,), (3,))):
            lag = cfg["last_lag"]
            for q in range(16 + lag):
                items += [first(q, xi0, nxi)] if q < 16 else []
                items += second(q - lag, rows) if q >= lag else []
            if rows != (1, 2):
                items += [_Item(0, None, None, part(send, 31, 4 * r + rows[0], 1 if rows[0] else 3))
                          for r in range(TR, 2 * TR)]
        return out

    out_dmas, os_count = [], [0]

    def out_groups(phase):
        c, n = divmod(phase, NG)
        cv, b, r0 = c // 4, (c // 2) % 2, (c % 2) * TR
        mp, acc, nxi = ms[phase % len(ms)], [], cfg["o_nxi"]

        def begin():
            acc.extend(stat[1 + b * NG + n, q] if r0 else jnp.zeros((8, 128), F32) for q in range(2))

        def end():
            for q in range(2):
                stat[1 + b * NG + n, q] = acc[q]

        units = [(r, p) for r in range(r0, r0 + TR) for p in range(2)]
        out = [[_Item(0, None, None, begin)]] if cv == 0 else []
        for q in range(len(units) + 1):
            slot = os_count[0] % 2
            firsts = [[_Item(cfg["c_o1"] * nxi, mp, osb, part(out_first, mp, *units[q], xi0, nxi, slot))]
                      for xi0 in range(0, 6, nxi)] if q < len(units) else []
            seconds = [[_Item(cfg["c_o2"], osb, (hs, xs)[cv][b],
                              part(out_second, acc, cv, b, n, *units[q - 1], jp, 1 - slot))]
                       for jp in range(2)] if q > 0 else []
            os_count[0] += bool(firsts)
            out += [grp for _, grp in sorted(
                [((k + 0.25) / len(firsts), grp) for k, grp in enumerate(firsts)]
                + [((k + 0.75) / len(seconds), grp) for k, grp in enumerate(seconds)], key=lambda t: t[0])]
        out[-1].append(_Item(0, None, None, part(send, phase, 4 * r0, 4 * TR) if cv else end))
        out[-1].append(_Item(0, None, None, part(ready.add, ("out", phase))))
        out[0].insert(0, _Item(0, None, None, part(need, ("mm", phase))))
        return out

    def load_lhs(vc, ks, cols, dues):
        cuts = sorted({0, TR} | set(dues))
        blocks = [[] for _ in ks]
        for lo, hi in zip(cuts, cuts[1:]):
            for value in dues.get(lo, ()):
                pace.release(vc, value)
            if dues.get(lo) and cfg["soft"] and (lo % cfg["soft"] or cfg["soft"] == 1):
                pace.release(vc, jnp.zeros((8, 128), U32))
            for blk, (xi, nu) in zip(blocks, ks):
                blk.append(vc[1 + xi * 6 + nu, pl.ds(lo * 8, (hi - lo) * 8), cols])
        return [pltpu.bitcast(jnp.concatenate(blk, axis=0), BF16) for blk in blocks]

    def dot(lhs, rhs):
        return jax.lax.dot_general(lhs, pltpu.bitcast(rhs, BF16), (((1,), (1,)), ((), ())),
                                   preferred_element_type=F32)

    def matmul(phase, xi, nu, dues):
        c, n = divmod(phase, NG)
        need(("in", c, NG - 1), ("w", c // 4, n, xi, NG - 1, 7), *[("out", phase - len(ms))] * (phase >= len(ms)))
        if (xi, nu) == ORDER[-1]:
            ready.add(("mm", phase))
        lhs, = load_lhs(vs[c % 2], [(xi, nu)], slice(None), dues)
        res = dot(lhs, us[c // 4][1 + n * 36 + nu * 6 + xi])
        ms[phase % len(ms)][1 + nu * 6 + xi, pl.ds(0, M)] = res
        return res

    def matmul_part(g, ks, dues):
        need(("in", 0, g), ("w", 0, 0, 4, g, 7))
        ready.add(("mm", 0))
        for lhs, (xi, nu) in zip(load_lhs(vs[0], ks, lanes(g), dues), ks):
            res = dot(lhs, us[0][1 + nu * 6 + xi, :, lanes(g)])
            at = (1 + nu * 6 + xi, pl.ds(0, M))
            res = ms[0][at] + res if g else res
            ms[0][at] = res
        return res

    def steps(phase, g=NG - 1):
        if phase == 0:
            return [part(matmul_part, g, ORDER[q:q + 4]) for q in range(0, 36, 4)]
        return [part(matmul, phase, *k) for k in ORDER]

    dsts = lambda it: it.dst if isinstance(it.dst, tuple) else () if it.dst is None else (it.dst,)

    def run_alone(groups, window):
        finished, acc = [], 0
        for it in (it for grp in groups for it in grp):
            ready = [v for t, v in finished if t <= acc - window]
            if it.src is not None and ready:
                pace.release(it.src, ready[-1])
            it.fn()
            acc += it.cost
            for dst in dsts(it):
                finished.append((acc, pace.done(dst)))
            del finished[:-24]

    clock, pending, todo, chain, spent = [], {}, [], [], [0]

    def advance(tick):
        while todo and len(clock) * TICKS <= tick:
            now, dues = len(clock) * TICKS, {}
            for key in [key for key in pending if key[0] < now + TICKS]:
                dues.setdefault(max(key[0] - now, 0) // 2, []).append(pending.pop(key))
            for rb in range(0, TR if cfg["pop_lag"] else 0, cfg["pop_every"]):
                t = min(now + 2 * rb - cfg["pop_lag"], now - 1)
                if t >= 0:
                    dues.setdefault(rb, []).append(clock[t // TICKS][t % TICKS * 8:t % TICKS * 8 + 8])
            clock.append(todo.pop(0)(dues))

    def run_paced(matmuls, items, stretch=1.0):
        lead, slack, win = cfg["lead"], cfg["slack"], cfg["win"]
        t0, span = len(clock) * TICKS, len(matmuls) * TICKS
        total, acc, last = max(sum(it.cost for it in items), 1) / stretch, 0, {}
        todo.extend(matmuls)
        for it in items:
            start = t0 + int(acc / total * span) // win * win - lead
            acc += it.cost
            advance(start)
            if it.src is not None:
                if 0 <= start < t0 + span and last.get(id(it.src)) != start:
                    last[id(it.src)] = start
                    pace.release(it.src, clock[start // TICKS][start % TICKS * 8:start % TICKS * 8 + 8])
                if cfg["chain"]:
                    older = [v for t, v in chain if t <= spent[0] - cfg["chain"]]
                    pace.release(it.src, older[-1] if older else jnp.zeros((8, 128), it.src.dtype))
            it.fn()
            spent[0] += it.cost
            for dst in dsts(it):
                chain.append((spent[0], pace.done(dst)))
                pending[-(-(t0 + int(acc / total * span) - lead + slack) // 2) * 2, id(dst)] = chain[-1][1]
            del chain[:-32]
        advance(t0 + span)

    def forget():
        del clock[:], chain[:]
        pending.clear()

    p_lo, p_hi = cfg["only"]

    sc = [None, 0]
    def scope(name):
        if not cfg.get("scopes"): return
        if sc[0] is not None: sc[0].__exit__(None, None, None)
        sc[0] = jax.named_scope(f"s_{sc[1]:02d}{name}") if name else None
        sc[1] += 1
        if sc[0] is not None: sc[0].__enter__()
    def waits(dmas):
        scope("wait")
        for d in dmas: d.wait()
        scope("run")
    waits(small)
    for q, ref in enumerate((g1_s, be1_s, g2_s, be2_s)):
        value = ref[...].astype(F32)
        for g in range(NG):
            affine[q, g] = jnp.broadcast_to(value[g * 128:(g + 1) * 128][None, :], (8, 128))
    pace = _Pacer(0)
    for buf in (*xs, *hs, *wr, *us, *vs, *ms, tb, osb, stat):
        pace.init(buf)

    pace.move(jax.lax.fori_loop(0, 2, lambda i, z: z + (i >> 10), jnp.int32(0)))

    cfg = dict(cfg, **cfg["HH"])
    for g in range(NG if p_lo < 0 else 0):
        stats = x_stat_groups(0, g, {q * xr: x0_copy(g, q) for q in range(xp)})
        run_alone(stats[:-1], cfg["alone"])
        waits([w0_copy(g)])
        work = stats[-1:] + sum((w_groups(0, 0, [g], xis) for xis in cfg["w0"]), []) + in_groups(0, g)
        if g == 0:
            run_alone(work, cfg["alone"])
        else:
            run_paced(steps(0, g - 1), [it for grp in work for it in grp], cfg["stretch"])
            forget()

    if p_lo >= 0:
        for d in first: d.wait()
        for time, dmas in zip(cfg["t_wait"], late):
            if not p_lo < time < p_hi:
                for d in dmas: d.wait()
        scope("go")
    streams = []
    for c in range(1, 8):
        groups = []
        for g in range(NG):
            if c in (4, 6):
                groups.append([_Item(30, None, None, part(h_stat_end, (c - 4) // 2, g))])
            groups += in_groups(c, g)
        if c == 1:
            cut = int(len(groups) * cfg["in1"])
            streams += [(groups[:cut], 1.0, 3.5), (groups[cut:], 3.5, 3.98)]
        else:
            streams.append((groups, *cfg["t_in"][c - 2]))
    streams.append(([grp for g in range(NG) for grp in x_stat_groups(1, g, {})], *cfg["t_stat"]))
    w_times = cfg["t_w"]
    for k, (cv, n) in enumerate([(cv, n) for cv in range(2) for n in range(NG)][1:]):
        t = w_times[k]
        streams += [(w_groups(cv, n, range(NG), (0, 1, 2)), t[0], t[1]), (w_groups(cv, n, range(NG), (3, 4, 5)), t[1], t[2])]
    t_out = cfg["t_out"]
    for p in range(31):
        assert t_out[p + 1] <= p + len(ms)
        streams.append((out_groups(p), t_out[p], t_out[p + 1]))
    streams.append((emb_groups(), *cfg["t_emb"]))
    for time, dmas in zip(cfg["t_wait"], late):
        if p_lo < 0 or p_lo < time < p_hi:
          streams.insert(0, ([[_Item(0, None, None, part(waits, dmas))]], time, time))
    for time in cfg["t_split"]:
        streams.insert(0, ([[_Item(0, None, None, lambda: waits([out_dmas.pop(0)()]) if out_dmas else None)]], time, time))
    phases, last = _spread(streams), last_items()
    if cfg.get("show"):
        print("load", [2 * sum(it.cost for it in phases[p]) + 1728 for p in sorted(phases)])
    def run_phases(p0, p1):
        nonlocal cfg
        for p in range(p0, p1):
            cfg = dict(cfg, **(cfg["L"] if p in cfg["light"] else cfg["HH"] if p < 4 else cfg["Z"] if p == 31 else cfg["H"]))
            if p == 0:
                run_paced(steps(p), phases[0] + phases[1])
            elif p == 31:
                rows = [steps(p)[6 * xi:6 * xi + 6] for xi in (1, 2, 3, 4, 0, 5)]
                late_start = lambda items: [_Item(int(sum(it.cost for it in items) * cfg["late"]), None, None, lambda: None)] + items
                run_paced(rows[0] + rows[1] + rows[2], phases[2 * p] + phases.get(2 * p + 1, []))
                for step in range(3):
                    run_paced(rows[3 + step], late_start(last[step]) if step else last[step])
            else:
                run_paced(steps(p)[:18], phases[2 * p])
                run_paced(steps(p)[18:], phases[2 * p + 1])

    p = max(p_lo, 0)
    for p0, p1 in cfg["loops"]:
        if p_lo <= p0 and p1 <= p_hi:
            run_phases(p, p0)
            forget()
            jax.lax.fori_loop(0, pace.zero + 1, lambda i, _: run_phases(p0, p1), None)
            forget()
            p = p1
    run_phases(p, min(p_hi, 32))
    scope("tail")
    if p_hi > 32:
        run_alone([last[3]], cfg["alone"])
    scope("last")
    for time, dmas in zip(cfg["t_wait"], late):
        if p_lo < 0 and time >= p_hi:
            for d in dmas: d.wait()
    for d in out_dmas:
        d().wait()
    scope(None)


def H(soft, chain, slack, pop_lag, pop_every=1, kill=1):
    return dict(soft=soft, kill=kill, chain=chain, slack=slack, pop_lag=pop_lag, pop_every=pop_every)


def _lin(points, n):
    out = []
    for i in range(n):
        (i0, v0), (i1, v1) = next((a, b) for a, b in zip(points, points[1:]) if a[0] <= i <= b[0])
        out.append(v0 + (v1 - v0) * (i - i0) / (i1 - i0))
    return tuple(out)


_CFG = dict(
    only=(-1, 33), lead=16, slack=40, win=2, alone=500, stretch=1.1, n_m=5, ahead=0, vclk=0, clk_slot=0, soft=1, kill=1, chain=7, clk_every=1, pop_every=2, pop_lag=22,
    dslack=(), L=dict(soft=0, kill=0, chain=0, slack=24, pop_lag=0, pop_every=1),
    H=dict(soft=4, kill=1, chain=140, slack=28, pop_lag=20, pop_every=1), light=tuple(range(22, 31)),
    c_rowx=88, c_rowh=80, c_col=42, c_o1=16, c_o2=56, c_w=46, w0=((0, 1, 2), (3, 4, 5)), c_st=40,
    nnu=1, o_nxi=3, w_nxi=1, w_direct=True, w_lead=False,
    x_pieces=2, stat_rows=2, last_send=2, last_lag=2, late=0.2, Z=dict(soft=0, kill=0, chain=0, slack=40, pop_lag=0, pop_every=1), t_emb=(7.2, 9.6),
    t_wait=(0.0, 1.5, 4.0, 10.0, 16.0), t_split=(22.0, 27.0), loops=(),
    HH=dict(soft=4, kill=1, chain=450, slack=24, pop_lag=20, pop_every=1), in1=0.67,
    t_in=((4.8, 7.98), (8.0, 11.98), (12.0, 15.98), (16.0, 19.98), (20.0, 23.98), (24.0, 27.98)),
    t_stat=(4.0, 6.8),
    t_w=((0.0, 0.99, 1.47), (1.5, 1.97, 2.47), (2.5, 2.97, 3.47), (10.0, 11.2, 12.4), (12.4, 13.6, 14.8), (14.8, 16.0, 17.2), (17.2, 18.4, 19.47)),
    t_out=_lin(((0, 4.0), (2, 4.9), (5, 8.0), (8, 10.0), (15, 18.5), (16, 19.5), (20, 21.3), (22, 23.04), (29, 30.04), (30, 31.04), (31, 31.49)), 32),
)


def H(soft, chain, slack, pop_lag, pop_every=1, kill=1):
    return dict(soft=soft, kill=kill, chain=chain, slack=slack, pop_lag=pop_lag, pop_every=pop_every)


def _resblock(cfg, x, t_emb, g1, be1, w1, w_emb, g2, be2, w2):
    assert x.shape == (NB, C, HW, HW) and w1.shape == w2.shape == (C, C, 3, 3)
    emb_dim = t_emb.shape[1]
    vmem = pltpu.VMEM
    scratch = (
        [vmem((1 + NG * HW, HW, 128), BF16)] * 2
        + [vmem((1 + HW * NG, 2, 4, 8, 128), F32)] * 2
        + [vmem((1 + NG * 9, C, 128), BF16)] * 2
        + [vmem((1 + NG * 36, 64, C), U32)] * 2
        + [vmem((1 + 36, M // 2, C), U32)] * 2
        + [vmem((1 + NG * T_ROWS, 2, 7, 8, 128), F32),
           vmem((1 + 18 * 4, 7, 8, 128), F32),
           vmem((2 * NB * NG, 2, 8, 128), F32),
           vmem((1 + NB * NG, 6, 8, 128), F32),
           vmem((NB, emb_dim), BF16)]
        + [vmem((C,), BF16)] * 4
        + [vmem((emb_dim, C), BF16), vmem((NB, C), F32), vmem((NB, 128, 128), F32), vmem((4, NG, 8, 128), F32), pltpu.SemaphoreType.DMA((NG * (cfg["x_pieces"] + 1) + 6,))]
        + [vmem((1 + 36, M_PITCH, 128), F32)] * cfg["n_m"]
    )
    as_taps = lambda w: jnp.transpose(w, (2, 3, 0, 1)).reshape(9, C, C)
    out = pl.pallas_call(
        functools.partial(_kernel, cfg),
        out_shape=jax.ShapeDtypeStruct((NB, HW, HW, C), x.dtype),
        in_specs=[pl.BlockSpec(memory_space=pl.ANY)] * 9,
        out_specs=pl.BlockSpec(memory_space=pl.ANY),
        scratch_shapes=scratch,
        compiler_params=pltpu.CompilerParams(vmem_limit_bytes=120 * 2 ** 20),
    )(jnp.transpose(x, (0, 2, 3, 1)), t_emb, g1, be1, as_taps(w1), w_emb,
      g2, be2, as_taps(w2))
    return jnp.transpose(out, (0, 3, 1, 2))


@jax.jit
def pallas_standalone__adm_resblock__diffusion_kernel(
    x: jax.Array,
    t_emb: jax.Array,
    g1: jax.Array,
    be1: jax.Array,
    w1: jax.Array,
    w_emb: jax.Array,
    g2: jax.Array,
    be2: jax.Array,
    w2: jax.Array,
):
    return _resblock(_CFG, x, t_emb, g1, be1, w1, w_emb, g2, be2, w2)
```

```python
import functools

import jax
import jax.numpy as jnp
from jax.experimental import pallas as pl
from jax.experimental.pallas import tpu as pltpu

F32, BF16, U32 = jnp.float32, jnp.bfloat16, jnp.uint32

NB, C, HW, NG = 2, 512, 64, 4
EPS = 1e-5
TR = 8
M = 16 * TR
M_PITCH = M + 16
T_ROWS = 33
TICKS = M // 8
ORDER = [(xi, nu) for xi in range(6) for nu in range(6)]

PA, PB = 2.0 / 3.0, 1.5
A2, B2 = PA * PA, PB * PB
DD = A2 - B2


def _xf_in(d):
    p2, q2 = B2 * d[2], A2 * d[2]
    ea, eb = d[4] - p2, d[4] - q2
    p3, q3 = A2 * d[3], B2 * d[3]
    ua, ub = d[1] - p3, d[1] - q3
    v0 = (ea if d[0] is None else d[0] + ea) - q2
    v5 = (ua if d[5] is None else d[5] + ua) - q3
    oa, ob = PB * ua, PA * ub
    return [v0, ea - oa, ea + oa, eb - ob, eb + ob, v5]


def _xf_out(m):
    sa, da, sb, db = m[1] + m[2], m[1] - m[2], m[3] + m[4], m[3] - m[4]
    return [None if m[0] is None else (m[0] + sb) + sa, PA * da + PB * db, A2 * sa + B2 * sb,
            None if m[5] is None else (PA ** 3 * da + m[5]) + PB ** 3 * db]


def _xf_w(g):
    t = g[2] * (1.0 / (2 * DD))
    ea, eb = g[0] * (1.0 / (2 * A2 * DD)) + t, g[0] * (-1.0 / (2 * B2 * DD)) - t
    oa, ob = g[1] * (PB / (2 * DD)), g[1] * (-PA / (2 * DD))
    return [g[0], ea + oa, ea - oa, eb + ob, eb - ob, g[2]]


def _unpack(w, half):
    return pltpu.unpack_elementwise(w, index=half, packed_dtype=BF16, unpacked_dtype=F32)


def _pack(lo, hi):
    return pltpu.pack_elementwise([lo, hi], packed_dtype=BF16)


def _mean_all(v):
    return jnp.sum(jnp.sum(v, axis=0, keepdims=True), axis=1, keepdims=True) * (1.0 / v.size)


class _Item:
    def __init__(self, cost, src, dst, fn):
        self.cost, self.src, self.dst, self.fn = cost, src, dst, fn

    def slack(self, cfg):
        return cfg["slack"] + dict(cfg["dslack"]).get(getattr(getattr(self.fn, "func", None), "__name__", ""), 0)


class _Pacer:
    def __init__(self, zero):
        self.zero = zero

    def move(self, zero):
        self.zero = zero

    def _slot(self, buf, which):
        lanes = pl.ds(0, 128)
        if buf.shape[-2] > 8:
            return (self.zero,) + (0,) * (len(buf.shape) - 3) + (pl.ds(8 * which, 8), lanes)
        return (self.zero,) + (0,) * (len(buf.shape) - 4) + (which, pl.ds(0, 8), lanes)

    def init(self, buf):
        for which in range(2):
            buf[self._slot(buf, which)] = jnp.zeros((8, 128), buf.dtype)

    def release(self, buf, value, which=0):
        if value.dtype != buf.dtype:
            value = pltpu.bitcast(value, buf.dtype)
        buf[self._slot(buf, which)] = value

    def done(self, buf):
        return buf[self._slot(buf, 1)]


def _spread(streams):
    keyed = []
    for groups, lo, hi in streams:
        total = max(sum(it.cost for grp in groups for it in grp), 1)
        acc = 0
        for grp in groups:
            cost = sum(it.cost for it in grp)
            keyed.append((lo + (hi - lo) * (acc + cost / 2) / total, len(keyed), grp))
            acc += cost
    keyed.sort(key=lambda t: t[:2])
    phases = {}
    for time, _, grp in keyed:
        phases.setdefault(int(2 * time), []).extend(grp)
    return phases


def _kernel(cfg, x_hbm, t_hbm, g1_hbm, be1_hbm, w1_hbm, wemb_hbm, g2_hbm, be2_hbm, w2_hbm, o_hbm,
            xs0, xs1, h0, h1, wr1, wr2, u1, u2, v0, v1, tb, osb, coef, stat,
            t_s, g1_s, be1_s, g2_s, be2_s, wemb_s, emb_s, tcol, affine, sems, *ms):
    xs_bf, wr_bf = (xs0, xs1), (wr1, wr2)
    xs = tuple(r.bitcast(U32) for r in xs_bf)
    wr = tuple(r.bitcast(U32) for r in wr_bf)
    hs, us, vs = (h0, h1), (u1, u2), (v0, v1)
    part = functools.partial
    lanes = lambda g: pl.ds(g * 128, 128)

    xp = cfg["x_pieces"]
    xr = HW // xp
    n_head = NG * (xp + 1)

    def x_copy(b, g, r0, nr, sem):
        return pltpu.make_async_copy(x_hbm.at[b, pl.ds(r0, nr), :, lanes(g)],
                                     xs_bf[b].at[pl.ds(1 + g * HW + r0, nr)], sems.at[sem])

    def w_copy(cv, n0, n1, g, sem):
        rows = pl.ds(n0 * 128, (n1 - n0) * 128)
        return pltpu.make_async_copy((w1_hbm, w2_hbm)[cv].at[:, rows, lanes(g)],
                                     wr_bf[cv].at[pl.ds(1 + g * 9, 9), rows], sems.at[sem])

    x0_copy = lambda g, q: x_copy(0, g, q * xr, xr, g * (xp + 1) + q)
    w0_copy = lambda g: w_copy(0, 0, 1, g, g * (xp + 1) + xp)
    w_of = lambda cv, n0, n1, sem: [w_copy(cv, n0, n1, g, n_head + sem) for g in range(NG)]
    small = [pltpu.make_async_copy(s, d, sems.at[n_head]) for s, d in
             ((g1_hbm, g1_s), (be1_hbm, be1_s), (g2_hbm, g2_s), (be2_hbm, be2_s), (t_hbm, t_s))]
    late = [w_of(0, 1, 2, 1), w_of(0, 2, 4, 2),
            [x_copy(1, g, 0, HW, n_head + 3) for g in range(NG)]
            + [pltpu.make_async_copy(wemb_hbm, wemb_s, sems.at[n_head + 3])], w_of(1, 0, 2, 4), w_of(1, 2, 3, 5), w_of(1, 3, 4, 6)]
    first = []
    for g in range(NG):
        xw = [x0_copy(g, q) for q in range(xp)], [w0_copy(g)]
        first += xw[1] + xw[0] if cfg["w_lead"] else xw[0] + xw[1]
    for d in first[:1] + small + first[1:] + [d for dmas in late for d in dmas]:
        d.start()

    ready = set()

    def need(*keys):
        assert p_lo >= 0 or all(key in ready for key in keys), keys

    sub = jax.lax.broadcasted_iota(jnp.int32, (8, 128), 0)

    def w_rows(cv, n, g, ob, xis):
        w = [wr[cv][pl.ds(1 + g * 9 + 3 * i, 3), pl.ds(n * 64 + ob * 8, 8)] for i in range(3)]
        c = [_xf_w([_unpack(wi, half) for wi in w]) for half in range(2)]
        for xi in xis:
            ready.add(("w", cv, n, xi, g, ob))
            u = [_xf_w([ch[xi][j] for j in range(3)]) for ch in c]
            for nu in range(6):
                us[cv][1 + n * 36 + nu * 6 + xi, pl.ds(ob * 8, 8), lanes(g)] = _pack(u[0][nu], u[1][nu])

    def w_groups(cv, n, gs, xis):
        return [[_Item(cfg["c_w"] * len(xis), wr[cv], us[cv], part(w_rows, cv, n, g, ob, xis))] for g in gs for ob in range(8)]

    def set_coef(cv, b, g, mean, var, bias):
        gamma, beta = affine[2 * cv, g], affine[2 * cv + 1, g]
        mu = _mean_all(mean)
        dev = mean - mu
        scale = gamma * jax.lax.rsqrt(_mean_all(jnp.maximum(var, 0.0) + dev * dev) + EPS)
        shift = beta + (bias - mu) * scale
        k = (cv * NB + b) * NG + g
        ready.add(("coef", cv, b, g))
        coef[k, 0] = jnp.broadcast_to(0.5 * shift, (8, 128))
        coef[k, 1] = jnp.broadcast_to(0.5 * scale, (8, 128))

    def x_stat_rows(acc, b, g, r0, nr):
        for r in range(r0, r0 + nr):
            w = xs[b][1 + g * HW + r].reshape(2, 2, 8, 128)
            lo, hi = _unpack(w, 0), _unpack(w, 1)
            if not acc:
                acc.append(lo[0])
            lo, hi = lo - acc[0], hi - acc[0]
            s1, s2 = lo + hi, lo * lo + hi * hi
            s1, s2 = s1[0] + s1[1], s2[0] + s2[1]
            acc[1:] = [acc[1] + s1, acc[2] + s2] if acc[1:] else [s1, s2]
        stat[0, pl.ds(2, 2)] = acc[1]
        stat[0, pl.ds(4, 2)] = acc[2]

    def x_stat_end(acc, b, g):
        if not acc: return
        ref, m1, m2 = acc[0], acc[1] * (1.0 / (HW * 4)), acc[2] * (1.0 / (HW * 4))
        set_coef(0, b, g, (ref + m1).reshape(16, 128), (m2 - m1 * m1).reshape(16, 128), 0.0)

    def x_stat_groups(b, g, waits):
        acc, out, nr = [], [], cfg["stat_rows"]
        for r0 in range(0, HW, nr):
            grp = [_Item(0, None, None, waits[r0].wait)] if r0 in waits else []
            out.append(grp + [_Item(cfg["c_st"] * nr, xs[b], stat, part(x_stat_rows, acc, b, g, r0, nr))])
        out.append([_Item(30, None, None, part(x_stat_end, acc, b, g))])
        return out

    def h_stat_end(b, g):
        need("emb", ("out", (2 * b + 1) * NG + g))
        s = stat[1 + b * NG + g, pl.ds(0, 2)]
        inv = 1.0 / (HW * 8)
        m1, m2 = s[0] * inv, s[1] * inv
        e = emb_s[pl.ds(b, 1), lanes(g)]
        set_coef(1, b, g, m1 + e, m2 - m1 * m1, e)

    def emb_rows(acc, e0):
        if e0 % 128 == 0:
            t = t_s[:, pl.ds(e0, 128)].astype(F32)
            t = t * jax.nn.sigmoid(t)
            for b in range(NB):
                tcol[b] = jnp.broadcast_to(t[b:b + 1], (128, 128)).T
        for r in range(e0, e0 + 32, 8):
            w = wemb_s[pl.ds(r, 8)].astype(F32)
            for b in range(NB):
                term = w * jnp.concatenate([tcol[b, pl.ds(r % 128, 8)]] * NG, axis=1)
                acc[b] = acc[b] + term if b in acc else term
        stat[0, pl.ds(2, NG)] = jnp.stack([acc[NB - 1][:, g * 128:(g + 1) * 128] for g in range(NG)])

    def emb_groups():
        acc = {}

        def end():
            ready.add("emb")
            for b in range(NB):
                emb_s[pl.ds(b, 1)] = jnp.sum(acc[b], axis=0, keepdims=True)

        return ([[_Item(84, None, stat, part(emb_rows, acc, e0))] for e0 in range(0, t_s.shape[1], 32)]
                + [[_Item(40, None, None, end)]])

    def silu(z, scale, shift):
        u = z * scale + shift
        return u + u * jnp.tanh(u)

    def in_row(cv, b, g, h):
        k = (cv * NB + b) * NG + g
        need(("coef", cv, b, g))
        if cv == 0:
            row = 1 + g * HW + h
            w = jnp.concatenate([xs[b][row, pl.ds(jp, 8, stride=4)] for jp in range(4)]).reshape(2, 2, 8, 128)
            scale, shift = coef[k, 1], coef[k, 0]
            lo, hi = silu(_unpack(w, 0), scale, shift), silu(_unpack(w, 1), scale, shift)
            d = [lo[:, 0], hi[:, 0], lo[:, 1], hi[:, 1]]
        else:
            a = silu(hs[b][1 + h * NG + g], coef[k, 1], coef[k, 0])
            d = [a[:, j] for j in range(4)]
        left = jnp.where(sub == 0, 0.0, pltpu.roll(d[3][1], 1, 0))
        right = jnp.where(sub == 7, 0.0, pltpu.roll(d[0][0], 7, 0))
        v = _xf_in([jnp.stack([left, d[3][0]])] + d + [jnp.stack([d[0][1], right])])
        for nu in range(6):
            tb[1 + g * T_ROWS + h % T_ROWS, :, nu] = v[nu]

    def in_col(vn, g, r, nu0, nnu):
        rows = range(4 * r - 1, 4 * r + 5)
        v = [_xf_in([tb[1 + g * T_ROWS + h % T_ROWS, p, pl.ds(nu0, nnu)] if 0 <= h < HW else None for h in rows])
             for p in range(2)]
        for xi in range(6):
            vn[pl.ds(1 + xi * 6 + nu0, nnu), pl.ds(r % TR * 8, 8), lanes(g)] = _pack(v[0][xi], v[1][xi])

    def in_groups(c, g):
        cv, b, r0 = c // 4, (c // 2) % 2, (c % 2) * TR
        src, cost = (xs[b], cfg["c_rowx"]) if cv == 0 else (hs[b], cfg["c_rowh"])
        row = lambda h: [_Item(cost, src, tb, part(in_row, cv, b, g, h))]
        out, nnu = [row(0)] if r0 == 0 else [], cfg["nnu"]
        for r in range(r0, r0 + TR + 1):
            rows = [row(h) for h in range(4 * r + 1, min(4 * r + 5, HW))] if r < r0 + TR else []
            cols = [[_Item(cfg["c_col"] * nnu, tb, vs[c % 2], part(in_col, vs[c % 2], g, r - 1, nu0, nnu))]
                    for nu0 in range(0, 6, nnu)] if r > r0 else []
            out += [grp for _, grp in sorted(
                [((q + 0.25) / len(rows), grp) for q, grp in enumerate(rows)]
                + [((q + 0.75) / len(cols), grp) for q, grp in enumerate(cols)], key=lambda t: t[0])]
        out[-1].append(_Item(0, None, None, part(ready.add, ("in", c, g))))
        if c > 1:
            out[0].insert(0, _Item(0, None, None, part(need, ("mm", c * NG - NG - 1))))
        return out

    def out_first(mp, r, p, xi0, nxi, slot):
        y = _xf_out([mp[pl.ds(1 + nu * 6 + xi0, nxi), pl.ds(r % TR * 16 + p, 8, stride=2)] for nu in range(6)])
        for j in range(4):
            osb[1 + slot * 4 + j, pl.ds(xi0, nxi)] = y[j]

    def out_second(acc, cv, b, n, r, p, jp, slot, rows=(0, 1, 2, 3)):
        y = _xf_out([None if (xi == 0 and 0 not in rows) or (xi == 5 and 3 not in rows) else
                     osb[pl.ds(1 + slot * 4 + 2 * jp, 2), xi] for xi in range(6)])
        if cv == 0:
            if not acc: acc.extend(jnp.zeros((8, 128), F32) for q in range(2))
            for i in rows:
                hs[b][1 + (4 * r + i) * NG + n, p, pl.ds(2 * jp, 2)] = y[i]
            s1 = (y[0] + y[1]) + (y[2] + y[3])
            s2 = (y[0] * y[0] + y[1] * y[1]) + (y[2] * y[2] + y[3] * y[3])
            acc[:] = acc[0] + (s1[0] + s1[1]), acc[1] + (s2[0] + s2[1])
        else:
            for i in rows:
                at = (1 + n * HW + 4 * r + i, pl.ds(2 * p + jp, 8, stride=4))
                w = xs[b][at]
                xs[b][at] = _pack(_unpack(w, 0) + y[i][0], _unpack(w, 1) + y[i][1])

    def send(phase, h0, nr):
        b, n = phase // 8 % 2, phase % NG
        out_dmas.append(lambda: pltpu.make_async_copy(
            xs_bf[b].at[pl.ds(1 + n * HW + h0, nr)], o_hbm.at[b, pl.ds(h0, nr), :, lanes(n)],
            sems.at[min(phase - 16, len(cfg["t_split"]))]))
        out_dmas[-1]().start()

    def last_items():
        mp, units = ms[31 % len(ms)], [(r, p) for r in range(TR, 2 * TR) for p in range(2)]
        first = lambda q, xi0, nxi: _Item(16 * nxi, mp, osb, part(out_first, mp, *units[q], xi0, nxi, 2 + q))
        second = lambda q, rows: [_Item(cost, None, xs[1], part(out_second, None, 1, 1, NG - 1, *units[q], jp, 2 + q, rows))
                                  for cost in [10 + 6 * len(rows)] for jp in range(2)]
        out = [[first(q, 1, 2) for q in range(16)], [], [], []]
        for items, xi0, nxi, rows in zip(out[1:], (3, 0, 5), (2, 1, 1), ((1, 2), (0,), (3,))):
            lag = cfg["last_lag"]
            for q in range(16 + lag):
                items += [first(q, xi0, nxi)] if q < 16 else []
                items += second(q - lag, rows) if q >= lag else []
            if rows != (1, 2):
                items += [_Item(0, None, None, part(send, 31, 4 * r + rows[0], 1 if rows[0] else 3))
                          for r in range(TR, 2 * TR)]
        return out

    out_dmas, os_count = [], [0]

    def out_groups(phase):
        c, n = divmod(phase, NG)
        cv, b, r0 = c // 4, (c // 2) % 2, (c % 2) * TR
        mp, acc, nxi = ms[phase % len(ms)], [], cfg["o_nxi"]

        def begin():
            acc.extend(stat[1 + b * NG + n, q] if r0 else jnp.zeros((8, 128), F32) for q in range(2))

        def end():
            for q in range(2):
                stat[1 + b * NG + n, q] = acc[q]

        units = [(r, p) for r in range(r0, r0 + TR) for p in range(2)]
        out = [[_Item(0, None, None, begin)]] if cv == 0 else []
        for q in range(len(units) + 1):
            slot = os_count[0] % 2
            firsts = [[_Item(cfg["c_o1"] * nxi, mp, osb, part(out_first, mp, *units[q], xi0, nxi, slot))]
                      for xi0 in range(0, 6, nxi)] if q < len(units) else []
            seconds = [[_Item(cfg["c_o2"], osb, (hs, xs)[cv][b],
                              part(out_second, acc, cv, b, n, *units[q - 1], jp, 1 - slot))]
                       for jp in range(2)] if q > 0 else []
            os_count[0] += bool(firsts)
            out += [grp for _, grp in sorted(
                [((k + 0.25) / len(firsts), grp) for k, grp in enumerate(firsts)]
                + [((k + 0.75) / len(seconds), grp) for k, grp in enumerate(seconds)], key=lambda t: t[0])]
        out[-1].append(_Item(0, None, None, part(send, phase, 4 * r0, 4 * TR) if cv else end))
        out[-1].append(_Item(0, None, None, part(ready.add, ("out", phase))))
        out[0].insert(0, _Item(0, None, None, part(need, ("mm", phase))))
        return out

    def load_lhs(vc, ks, cols, dues):
        cuts = sorted({0, TR} | set(dues))
        blocks = [[] for _ in ks]
        for lo, hi in zip(cuts, cuts[1:]):
            for value in dues.get(lo, ()):
                pace.release(vc, value)
            if dues.get(lo) and cfg["soft"] and (lo % cfg["soft"] or cfg["soft"] == 1):
                pace.release(vc, jnp.zeros((8, 128), U32))
            for blk, (xi, nu) in zip(blocks, ks):
                blk.append(vc[1 + xi * 6 + nu, pl.ds(lo * 8, (hi - lo) * 8), cols])
        return [pltpu.bitcast(jnp.concatenate(blk, axis=0), BF16) for blk in blocks]

    def dot(lhs, rhs):
        return jax.lax.dot_general(lhs, pltpu.bitcast(rhs, BF16), (((1,), (1,)), ((), ())),
                                   preferred_element_type=F32)

    def matmul(phase, xi, nu, dues):
        c, n = divmod(phase, NG)
        need(("in", c, NG - 1), ("w", c // 4, n, xi, NG - 1, 7), *[("out", phase - len(ms))] * (phase >= len(ms)))
        if (xi, nu) == ORDER[-1]:
            ready.add(("mm", phase))
        lhs, = load_lhs(vs[c % 2], [(xi, nu)], slice(None), dues)
        res = dot(lhs, us[c // 4][1 + n * 36 + nu * 6 + xi])
        ms[phase % len(ms)][1 + nu * 6 + xi, pl.ds(0, M)] = res
        return res

    def matmul_part(g, ks, dues):
        need(("in", 0, g), ("w", 0, 0, 4, g, 7))
        ready.add(("mm", 0))
        for lhs, (xi, nu) in zip(load_lhs(vs[0], ks, lanes(g), dues), ks):
            res = dot(lhs, us[0][1 + nu * 6 + xi, :, lanes(g)])
            at = (1 + nu * 6 + xi, pl.ds(0, M))
            res = ms[0][at] + res if g else res
            ms[0][at] = res
        return res

    def steps(phase, g=NG - 1):
        if phase == 0:
            return [part(matmul_part, g, ORDER[q:q + 4]) for q in range(0, 36, 4)]
        return [part(matmul, phase, *k) for k in ORDER]

    dsts = lambda it: it.dst if isinstance(it.dst, tuple) else () if it.dst is None else (it.dst,)

    def run_alone(groups, window):
        finished, acc = [], 0
        for it in (it for grp in groups for it in grp):
            ready = [v for t, v in finished if t <= acc - window]
            if it.src is not None and ready:
                pace.release(it.src, ready[-1])
            it.fn()
            acc += it.cost
            for dst in dsts(it):
                finished.append((acc, pace.done(dst)))
            del finished[:-24]

    clock, pending, todo, chain, spent = [], {}, [], [], [0]

    def advance(tick):
        while todo and len(clock) * TICKS <= tick:
            now, dues = len(clock) * TICKS, {}
            for key in [key for key in pending if key[0] < now + TICKS]:
                dues.setdefault(max(key[0] - now, 0) // 2, []).append(pending.pop(key))
            for rb in range(0, TR if cfg["pop_lag"] else 0, cfg["pop_every"]):
                t = min(now + 2 * rb - cfg["pop_lag"], now - 1)
                if t >= 0:
                    dues.setdefault(rb, []).append(clock[t // TICKS][t % TICKS * 8:t % TICKS * 8 + 8])
            clock.append(todo.pop(0)(dues))

    def run_paced(matmuls, items, stretch=1.0):
        lead, slack, win = cfg["lead"], cfg["slack"], cfg["win"]
        t0, span = len(clock) * TICKS, len(matmuls) * TICKS
        total, acc, last = max(sum(it.cost for it in items), 1) / stretch, 0, {}
        todo.extend(matmuls)
        for it in items:
            start = t0 + int(acc / total * span) // win * win - lead
            acc += it.cost
            advance(start)
            if it.src is not None:
                if 0 <= start < t0 + span and last.get(id(it.src)) != start:
                    last[id(it.src)] = start
                    pace.release(it.src, clock[start // TICKS][start % TICKS * 8:start % TICKS * 8 + 8])
                if cfg["chain"]:
                    older = [v for t, v in chain if t <= spent[0] - cfg["chain"]]
                    pace.release(it.src, older[-1] if older else jnp.zeros((8, 128), it.src.dtype))
            it.fn()
            spent[0] += it.cost
            for dst in dsts(it):
                chain.append((spent[0], pace.done(dst)))
                pending[-(-(t0 + int(acc / total * span) - lead + slack) // 2) * 2, id(dst)] = chain[-1][1]
            del chain[:-32]
        advance(t0 + span)

    def forget():
        del clock[:], chain[:]
        pending.clear()

    p_lo, p_hi = cfg["only"]

    sc = [None, 0]
    def scope(name):
        if not cfg.get("scopes"): return
        if sc[0] is not None: sc[0].__exit__(None, None, None)
        sc[0] = jax.named_scope(f"s_{sc[1]:02d}{name}") if name else None
        sc[1] += 1
        if sc[0] is not None: sc[0].__enter__()
    def waits(dmas):
        scope("wait")
        for d in dmas: d.wait()
        scope("run")
    waits(small)
    for q, ref in enumerate((g1_s, be1_s, g2_s, be2_s)):
        value = ref[...].astype(F32)
        for g in range(NG):
            affine[q, g] = jnp.broadcast_to(value[g * 128:(g + 1) * 128][None, :], (8, 128))
    pace = _Pacer(0)
    for buf in (*xs, *hs, *wr, *us, *vs, *ms, tb, osb, stat):
        pace.init(buf)

    pace.move(jax.lax.fori_loop(0, 2, lambda i, z: z + (i >> 10), jnp.int32(0)))

    cfg = dict(cfg, **cfg["HH"])
    for g in range(NG if p_lo < 0 else 0):
        stats = x_stat_groups(0, g, {q * xr: x0_copy(g, q) for q in range(xp)})
        run_alone(stats[:-1], cfg["alone"])
        waits([w0_copy(g)])
        work = stats[-1:] + sum((w_groups(0, 0, [g], xis) for xis in cfg["w0"]), []) + in_groups(0, g)
        if g == 0:
            run_alone(work, cfg["alone"])
        else:
            run_paced(steps(0, g - 1), [it for grp in work for it in grp], cfg["stretch"])
            forget()

    if p_lo >= 0:
        for d in first: d.wait()
        for time, dmas in zip(cfg["t_wait"], late):
            if not p_lo < time < p_hi:
                for d in dmas: d.wait()
        scope("go")
    streams = []
    for c in range(1, 8):
        groups = []
        for g in range(NG):
            if c in (4, 6):
                groups.append([_Item(30, None, None, part(h_stat_end, (c - 4) // 2, g))])
            groups += in_groups(c, g)
        if c == 1:
            cut = int(len(groups) * cfg["in1"])
            streams += [(groups[:cut], 1.0, 3.5), (groups[cut:], 3.5, 3.98)]
        else:
            streams.append((groups, *cfg["t_in"][c - 2]))
    streams.append(([grp for g in range(NG) for grp in x_stat_groups(1, g, {})], *cfg["t_stat"]))
    w_times = cfg["t_w"]
    for k, (cv, n) in enumerate([(cv, n) for cv in range(2) for n in range(NG)][1:]):
        t = w_times[k]
        streams += [(w_groups(cv, n, range(NG), (0, 1, 2)), t[0], t[1]), (w_groups(cv, n, range(NG), (3, 4, 5)), t[1], t[2])]
    t_out = cfg["t_out"]
    for p in range(31):
        assert t_out[p + 1] <= p + len(ms)
        streams.append((out_groups(p), t_out[p], t_out[p + 1]))
    streams.append((emb_groups(), *cfg["t_emb"]))
    for time, dmas in zip(cfg["t_wait"], late):
        if p_lo < 0 or p_lo < time < p_hi:
          streams.insert(0, ([[_Item(0, None, None, part(waits, dmas))]], time, time))
    for time in cfg["t_split"]:
        streams.insert(0, ([[_Item(0, None, None, lambda: waits([out_dmas.pop(0)()]) if out_dmas else None)]], time, time))
    phases, last = _spread(streams), last_items()
    if cfg.get("show"):
        print("load", [2 * sum(it.cost for it in phases[p]) + 1728 for p in sorted(phases)])
    def run_phases(p0, p1):
        nonlocal cfg
        for p in range(p0, p1):
            cfg = dict(cfg, **(cfg["L"] if p in cfg["light"] else cfg["HH"] if p < 4 else cfg["Z"] if p == 31 else cfg["H"]))
            if p == 0:
                run_paced(steps(p), phases[0] + phases[1])
            elif p == 31:
                rows = [steps(p)[6 * xi:6 * xi + 6] for xi in (1, 2, 3, 4, 0, 5)]
                late_start = lambda items: [_Item(int(sum(it.cost for it in items) * cfg["late"]), None, None, lambda: None)] + items
                run_paced(rows[0] + rows[1] + rows[2], phases[2 * p] + phases.get(2 * p + 1, []))
                for step in range(3):
                    run_paced(rows[3 + step], late_start(last[step]) if step else last[step])
            else:
                run_paced(steps(p)[:18], phases[2 * p])
                run_paced(steps(p)[18:], phases[2 * p + 1])

    p = max(p_lo, 0)
    for p0, p1 in cfg["loops"]:
        if p_lo <= p0 and p1 <= p_hi:
            run_phases(p, p0)
            forget()
            jax.lax.fori_loop(0, pace.zero + 1, lambda i, _: run_phases(p0, p1), None)
            forget()
            p = p1
    run_phases(p, min(p_hi, 32))
    scope("tail")
    if p_hi > 32:
        run_alone([last[3]], cfg["alone"])
    scope("last")
    for time, dmas in zip(cfg["t_wait"], late):
        if p_lo < 0 and time >= p_hi:
            for d in dmas: d.wait()
    for d in out_dmas:
        d().wait()
    scope(None)


def H(soft, chain, slack, pop_lag, pop_every=1, kill=1):
    return dict(soft=soft, kill=kill, chain=chain, slack=slack, pop_lag=pop_lag, pop_every=pop_every)


def _lin(points, n):
    out = []
    for i in range(n):
        (i0, v0), (i1, v1) = next((a, b) for a, b in zip(points, points[1:]) if a[0] <= i <= b[0])
        out.append(v0 + (v1 - v0) * (i - i0) / (i1 - i0))
    return tuple(out)


_CFG = dict(
    only=(-1, 33), lead=16, slack=40, win=2, alone=500, stretch=1.1, n_m=6, ahead=0, vclk=0, clk_slot=0, soft=1, kill=1, chain=7, clk_every=1, pop_every=2, pop_lag=22,
    dslack=(), L=dict(soft=0, kill=0, chain=0, slack=24, pop_lag=0, pop_every=1),
    H=dict(soft=4, kill=1, chain=140, slack=28, pop_lag=20, pop_every=1), light=tuple(range(24, 31)),
    c_rowx=88, c_rowh=80, c_col=42, c_o1=16, c_o2=56, c_w=46, w0=((0, 1, 2), (3, 4, 5)), c_st=40,
    nnu=1, o_nxi=3, w_nxi=1, w_direct=True, w_lead=False,
    x_pieces=2, stat_rows=2, last_send=2, last_lag=2, late=0.2, Z=dict(soft=0, kill=0, chain=0, slack=40, pop_lag=0, pop_every=1), t_emb=(4.0, 4.9),
    t_wait=(0.0, 1.5, 4.0, 8.0, 12.0, 16.0), t_split=(20.0, 24.0), loops=(),
    HH=dict(soft=4, kill=1, chain=450, slack=24, pop_lag=20, pop_every=1), in1=0.67,
    t_in=((4.8, 7.98), (8.0, 11.98), (12.0, 15.98), (16.0, 19.98), (20.0, 23.98), (24.0, 27.98)),
    t_stat=(4.0, 6.8),
    t_w=((0.0, 0.99, 1.47), (1.5, 1.97, 2.47), (2.5, 2.97, 3.47), (8.0, 9.5, 11.0), (11.0, 12.4, 13.8), (13.8, 15.2, 16.6), (16.6, 18.0, 19.47)),
    t_out=_lin(((0, 4.0), (1, 4.8), (2, 6.8), (4, 8.2), (17, 19.5), (23, 24.04), (30, 31.04), (31, 31.49)), 32),
)


def H(soft, chain, slack, pop_lag, pop_every=1, kill=1):
    return dict(soft=soft, kill=kill, chain=chain, slack=slack, pop_lag=pop_lag, pop_every=pop_every)


def _resblock(cfg, x, t_emb, g1, be1, w1, w_emb, g2, be2, w2):
    assert x.shape == (NB, C, HW, HW) and w1.shape == w2.shape == (C, C, 3, 3)
    emb_dim = t_emb.shape[1]
    vmem = pltpu.VMEM
    scratch = (
        [vmem((1 + NG * HW, HW, 128), BF16)] * 2
        + [vmem((1 + HW * NG, 2, 4, 8, 128), F32)] * 2
        + [vmem((1 + NG * 9, C, 128), BF16)] * 2
        + [vmem((1 + NG * 36, 64, C), U32)] * 2
        + [vmem((1 + 36, M // 2, C), U32)] * 2
        + [vmem((1 + NG * T_ROWS, 2, 7, 8, 128), F32),
           vmem((1 + 18 * 4, 7, 8, 128), F32),
           vmem((2 * NB * NG, 2, 8, 128), F32),
           vmem((1 + NB * NG, 6, 8, 128), F32),
           vmem((NB, emb_dim), BF16)]
        + [vmem((C,), BF16)] * 4
        + [vmem((emb_dim, C), BF16), vmem((NB, C), F32), vmem((NB, 128, 128), F32), vmem((4, NG, 8, 128), F32), pltpu.SemaphoreType.DMA((NG * (cfg["x_pieces"] + 1) + 7,))]
        + [vmem((1 + 36, M_PITCH, 128), F32)] * cfg["n_m"]
    )
    as_taps = lambda w: jnp.transpose(w, (2, 3, 0, 1)).reshape(9, C, C)
    out = pl.pallas_call(
        functools.partial(_kernel, cfg),
        out_shape=jax.ShapeDtypeStruct((NB, HW, HW, C), x.dtype),
        in_specs=[pl.BlockSpec(memory_space=pl.ANY)] * 9,
        out_specs=pl.BlockSpec(memory_space=pl.ANY),
        scratch_shapes=scratch,
        compiler_params=pltpu.CompilerParams(vmem_limit_bytes=120 * 2 ** 20),
    )(jnp.transpose(x, (0, 2, 3, 1)), t_emb, g1, be1, as_taps(w1), w_emb,
      g2, be2, as_taps(w2))
    return jnp.transpose(out, (0, 3, 1, 2))


@jax.jit
def pallas_standalone__adm_resblock__diffusion_kernel(
    x: jax.Array,
    t_emb: jax.Array,
    g1: jax.Array,
    be1: jax.Array,
    w1: jax.Array,
    w_emb: jax.Array,
    g2: jax.Array,
    be2: jax.Array,
    w2: jax.Array,
):
    return _resblock(_CFG, x, t_emb, g1, be1, w1, w_emb, g2, be2, w2)
```

```python
import functools

import jax
import jax.numpy as jnp
from jax.experimental import pallas as pl
from jax.experimental.pallas import tpu as pltpu

F32, BF16, U32 = jnp.float32, jnp.bfloat16, jnp.uint32

NB, C, HW, NG = 2, 512, 64, 4
EPS = 1e-5
TR = 8
M = 16 * TR
M_PITCH = M + 16
N_RES = 6
T_ROWS = 33
TICKS = M // 8
LAST = 8 * NG - 1

PA, PB = 2.0 / 3.0, 1.5
A2, B2 = PA * PA, PB * PB
DD = A2 - B2

T_WAIT = (0, 1.5, 4, 8, 12, 16)
T_SENT = (20, 24, 28)
T_IN = ((4.8, 7.98), (8, 11.98), (12, 15.98), (16, 19.98), (20, 23.98), (24, 27.98))
T_STAT, T_EMB = (4, 6.8), (4, 4.9)
T_W = ((0, 0.99, 1.47), (1.5, 1.97, 2.47), (2.5, 2.97, 3.47),
       (8, 9.5, 11), (11, 12.4, 13.8), (13.8, 15.2, 16.6), (16.6, 18, 19.47))
T_OUT = ((0, 4), (1, 4.8), (2, 6.8), (4, 8.2), (17, 19.5), (23, 24.04), (30, 31.04), (31, 31.49))


def _xf_in(d):
    p2, q2 = B2 * d[2], A2 * d[2]
    ea, eb = d[4] - p2, d[4] - q2
    p3, q3 = A2 * d[3], B2 * d[3]
    ua, ub = d[1] - p3, d[1] - q3
    v0 = (ea if d[0] is None else d[0] + ea) - q2
    v5 = (ua if d[5] is None else d[5] + ua) - q3
    oa, ob = PB * ua, PA * ub
    return [v0, ea - oa, ea + oa, eb - ob, eb + ob, v5]


def _xf_out(m):
    sa, da, sb, db = m[1] + m[2], m[1] - m[2], m[3] + m[4], m[3] - m[4]
    return [None if m[0] is None else (m[0] + sb) + sa, PA * da + PB * db, A2 * sa + B2 * sb,
            None if m[5] is None else (PA ** 3 * da + m[5]) + PB ** 3 * db]


def _xf_w(g):
    t = g[2] * (1.0 / (2 * DD))
    ea, eb = g[0] * (1.0 / (2 * A2 * DD)) + t, g[0] * (-1.0 / (2 * B2 * DD)) - t
    oa, ob = g[1] * (PB / (2 * DD)), g[1] * (-PA / (2 * DD))
    return [g[0], ea + oa, ea - oa, eb + ob, eb - ob, g[2]]


def _unpack(word, half):
    return pltpu.unpack_elementwise(word, index=half, packed_dtype=BF16, unpacked_dtype=F32)


def _pack(lo, hi):
    return pltpu.pack_elementwise([lo, hi], packed_dtype=BF16)


def _mean_all(v):
    return jnp.sum(jnp.sum(v, axis=0, keepdims=True), axis=1, keepdims=True) * (1.0 / v.size)


def _lanes(g):
    return pl.ds(g * 128, 128)


class _Item:
    def __init__(self, fn, *args, cost=0, src=None, dst=None):
        self.run, self.cost, self.src, self.dst = functools.partial(fn, *args), cost, src, dst


def _interleave(streams):
    keyed = []
    for groups, start, end in streams:
        total, spent = max(sum(it.cost for grp in groups for it in grp), 1), 0
        for grp in groups:
            cost = sum(it.cost for it in grp)
            keyed.append((start + (end - start) * (spent + cost / 2) / total, len(keyed), grp))
            spent += cost
    halves = {}
    for time, _, grp in sorted(keyed, key=lambda t: t[:2]):
        halves.setdefault(int(2 * time), []).extend(grp)
    return halves


def _alternate(first, second):
    keyed = ([((q + 0.25) / len(first), grp) for q, grp in enumerate(first)]
             + [((q + 0.75) / len(second), grp) for q, grp in enumerate(second)])
    return [grp for _, grp in sorted(keyed, key=lambda t: t[0])]


class _Pacer:
    LEAD, RESULT_LAG = 16, 20

    def __init__(self):
        self.zero = 0
        self.restart()

    def restart(self):
        self.results, self.todo, self.due, self.finished, self.spent = [], [], {}, [], 0

    def _slot(self, buf, which):
        if buf.shape[-2] > 8:
            return (self.zero,) + (0,) * (len(buf.shape) - 3) + (pl.ds(8 * which, 8), _lanes(0))
        return (self.zero,) + (0,) * (len(buf.shape) - 4) + (which, pl.ds(0, 8), _lanes(0))

    def clear(self, buf, which=0):
        buf[self._slot(buf, which)] = jnp.zeros((8, 128), buf.dtype)

    def hold(self, buf, value):
        buf[self._slot(buf, 0)] = value if value.dtype == buf.dtype else pltpu.bitcast(value, buf.dtype)

    def _tick(self, t):
        return self.results[t // TICKS][t % TICKS * 8:t % TICKS * 8 + 8]

    def _emit(self, item):
        item.run()
        self.spent += item.cost
        if item.dst is not None:
            self.finished = self.finished[-31:] + [(self.spent, item.dst[self._slot(item.dst, 1)])]

    def _older(self, window):
        return [value for spent, value in self.finished if spent <= self.spent - window]

    def _advance(self, tick):
        while self.todo and len(self.results) * TICKS <= tick:
            now, before = len(self.results) * TICKS, {}
            for key in [key for key in self.due if key[0] < now + TICKS]:
                before.setdefault(max(key[0] - now, 0) // 2, []).append(self.due.pop(key))
            for block in range(TR if self.window else 0):
                t = min(now + 2 * block - self.RESULT_LAG, now - 1)
                if t >= 0:
                    before.setdefault(block, []).append(self._tick(t))
            self.results.append(self.todo.pop(0)(before))

    def load_blocks(self, buf, where, before):
        cuts, out = sorted({0, TR} | set(before)), [[] for _ in where]
        for lo, hi in zip(cuts, cuts[1:]):
            for value in before.get(lo, ()):
                self.hold(buf, value)
            if lo in before and lo % 4 and self.window:
                self.clear(buf)
            for blocks, (k, cols) in zip(out, where):
                blocks.append(buf[k, pl.ds(lo * 8, (hi - lo) * 8), cols])
        return [jnp.concatenate(blocks, axis=0) for blocks in out]

    def run_alone(self, items, window=500):
        self.restart()
        for item in items:
            for value in self._older(window)[-1:] if item.src is not None else ():
                self.hold(item.src, value)
            self._emit(item)
        self.restart()

    def run(self, matmuls, items, window, slack, stretch=1.0):
        t0, span, self.window = len(self.results) * TICKS, len(matmuls) * TICKS, window
        total, spent, held = max(sum(it.cost for it in items), 1) / stretch, 0, {}
        self.todo.extend(matmuls)
        for item in items:
            start = t0 + int(spent / total * span) // 2 * 2 - self.LEAD
            spent += item.cost
            self._advance(start)
            if item.src is not None:
                if 0 <= start < t0 + span and held.get(id(item.src)) != start:
                    held[id(item.src)] = start
                    self.hold(item.src, self._tick(start))
                if window and self._older(window):
                    self.hold(item.src, self._older(window)[-1])
                elif window:
                    self.clear(item.src)
            self._emit(item)
            if item.dst is not None:
                end = t0 + int(spent / total * span) - self.LEAD + slack
                self.due[-(-end // 2) * 2, id(item.dst)] = self.finished[-1][1]
        self._advance(t0 + span)


def _kernel(x_hbm, t_hbm, g1_hbm, be1_hbm, w1_hbm, wemb_hbm, g2_hbm, be2_hbm, w2_hbm, o_hbm,
            xs0, xs1, h0, h1, wr1, wr2, u1, u2, v0, v1, tb, osb, coef, stat,
            t_s, g1_s, be1_s, g2_s, be2_s, wemb_s, emb_s, tcol, affine, sems, *ms):
    xs_bf, wr_bf = (xs0, xs1), (wr1, wr2)
    xs = tuple(r.bitcast(U32) for r in xs_bf)
    wr = tuple(r.bitcast(U32) for r in wr_bf)
    hs, us, vs = (h0, h1), (u1, u2), (v0, v1)
    pace = _Pacer()

    ready = set()

    def need(*keys):
        assert all(key in ready for key in keys), keys

    def x_copy(b, g, r0, nr, sem):
        return pltpu.make_async_copy(x_hbm.at[b, pl.ds(r0, nr), :, :, _lanes(g)],
                                     xs_bf[b].at[pl.ds(1 + g * 2 * TR + r0, nr)], sems.at[sem])

    def w_copy(cv, n0, n1, g, sem):
        rows = pl.ds(n0 * 128, (n1 - n0) * 128)
        return pltpu.make_async_copy((w1_hbm, w2_hbm)[cv].at[:, rows, _lanes(g)],
                                     wr_bf[cv].at[pl.ds(1 + g * 9, 9), rows], sems.at[sem])

    def wait(copies):
        for copy in copies:
            copy.wait()

    early = [[x_copy(0, g, 0, TR, 3 * g), x_copy(0, g, TR, TR, 3 * g + 1), w_copy(0, 0, 1, g, 3 * g + 2)]
             for g in range(NG)]
    small = [pltpu.make_async_copy(src, dst, sems.at[3 * NG]) for src, dst in
             ((g1_hbm, g1_s), (be1_hbm, be1_s), (g2_hbm, g2_s), (be2_hbm, be2_s), (t_hbm, t_s))]
    w_all = lambda cv, n0, n1, sem: [w_copy(cv, n0, n1, g, 3 * NG + sem) for g in range(NG)]
    late = [w_all(0, 1, 2, 1), w_all(0, 2, 4, 2),
            [x_copy(1, g, 0, 2 * TR, 3 * NG + 3) for g in range(NG)]
            + [pltpu.make_async_copy(wemb_hbm, wemb_s, sems.at[3 * NG + 3])],
            w_all(1, 0, 2, 4), w_all(1, 2, 3, 5), w_all(1, 3, 4, 6)]
    for copies in [early[0][:1], small, early[0][1:]] + early[1:] + late:
        for copy in copies:
            copy.start()

    def w_rows(cv, n, g, ob, xis):
        w = [wr[cv][pl.ds(1 + g * 9 + 3 * i, 3), pl.ds(n * 64 + ob * 8, 8)] for i in range(3)]
        c = [_xf_w([_unpack(wi, half) for wi in w]) for half in range(2)]
        for xi in xis:
            ready.add(("w", cv, n, xi, g, ob))
            u = [_xf_w([ch[xi][j] for j in range(3)]) for ch in c]
            for nu in range(6):
                us[cv][1 + n * 36 + nu * 6 + xi, pl.ds(ob * 8, 8), _lanes(g)] = _pack(u[0][nu], u[1][nu])

    def w_groups(cv, n, gs, xis):
        return [[_Item(w_rows, cv, n, g, ob, xis, cost=138, src=wr[cv], dst=us[cv])]
                for g in gs for ob in range(8)]

    def set_coef(cv, b, g, mean, var, bias):
        mu = _mean_all(mean)
        dev = mean - mu
        scale = affine[2 * cv, g] * jax.lax.rsqrt(_mean_all(jnp.maximum(var, 0.0) + dev * dev) + EPS)
        shift = affine[2 * cv + 1, g] + (bias - mu) * scale
        coef[(cv * NB + b) * NG + g] = jnp.stack([0.5 * shift, 0.5 * scale])
        ready.add(("coef", cv, b, g))

    def x_row(g, h):
        return 1 + g * 2 * TR + h // 4, h % 4

    def x_stat_rows(acc, b, g, h0):
        for h in (h0, h0 + 1):
            w = xs[b][x_row(g, h)].reshape(2, 2, 8, 128)
            lo, hi = _unpack(w, 0), _unpack(w, 1)
            if not acc:
                acc.append(lo[0])
            lo, hi = lo - acc[0], hi - acc[0]
            s1, s2 = lo + hi, lo * lo + hi * hi
            s1, s2 = s1[0] + s1[1], s2[0] + s2[1]
            acc[1:] = [acc[1] + s1, acc[2] + s2] if acc[1:] else [s1, s2]
        stat[0, pl.ds(2, 2)], stat[0, pl.ds(4, 2)] = acc[1:]

    def x_stat_end(acc, b, g):
        m1, m2 = acc[1] * (1.0 / (HW * 4)), acc[2] * (1.0 / (HW * 4))
        set_coef(0, b, g, (acc[0] + m1).reshape(16, 128), (m2 - m1 * m1).reshape(16, 128), 0.0)

    def x_stat_groups(b, g):
        acc = []
        return ([[_Item(x_stat_rows, acc, b, g, h0, cost=80, src=xs[b], dst=stat)] for h0 in range(0, HW, 2)]
                + [[_Item(x_stat_end, acc, b, g, cost=30)]])

    def h_stat_end(b, g):
        need("emb", ("out", (2 * b + 1) * NG + g))
        m = stat[1 + b * NG + g, pl.ds(0, 2)] * (1.0 / (HW * 8))
        e = emb_s[pl.ds(b, 1), _lanes(g)]
        set_coef(1, b, g, m[0] + e, m[1] - m[0] * m[0], e)

    def emb_rows(acc, e0):
        if e0 % 128 == 0:
            t = t_s[:, pl.ds(e0, 128)].astype(F32)
            t = t * jax.nn.sigmoid(t)
            for b in range(NB):
                tcol[b] = jnp.broadcast_to(t[b:b + 1], (128, 128)).T
        for e in range(e0, e0 + 32, 8):
            w = wemb_s[pl.ds(e, 8)].astype(F32)
            for b in range(NB):
                term = w * jnp.concatenate([tcol[b, pl.ds(e % 128, 8)]] * NG, axis=1)
                acc[b] = acc[b] + term if b in acc else term
        stat[0, pl.ds(2, NG)] = jnp.stack([acc[NB - 1][:, g * 128:(g + 1) * 128] for g in range(NG)])

    def emb_end(acc):
        for b in range(NB):
            emb_s[pl.ds(b, 1)] = jnp.sum(acc[b], axis=0, keepdims=True)
        ready.add("emb")

    def emb_groups():
        acc = {}
        return ([[_Item(emb_rows, acc, e0, cost=84, dst=stat)] for e0 in range(0, t_s.shape[1], 32)]
                + [[_Item(emb_end, acc, cost=40)]])

    sublane = jax.lax.broadcasted_iota(jnp.int32, (8, 128), 0)

    def in_row(cv, b, g, h):
        need(("coef", cv, b, g))
        shift, scale = (coef[(cv * NB + b) * NG + g, q] for q in range(2))

        def silu(z):
            u = z * scale + shift
            return u + u * jnp.tanh(u)

        if cv == 0:
            w = jnp.concatenate([xs[b][(*x_row(g, h), pl.ds(jp, 8, stride=4))] for jp in range(4)])
            lo, hi = (silu(_unpack(w.reshape(2, 2, 8, 128), half)) for half in range(2))
            d = [lo[:, 0], hi[:, 0], lo[:, 1], hi[:, 1]]
        else:
            a = silu(hs[b][1 + h * NG + g])
            d = [a[:, j] for j in range(4)]
        left = jnp.where(sublane == 0, 0.0, pltpu.roll(d[3][1], 1, 0))
        right = jnp.where(sublane == 7, 0.0, pltpu.roll(d[0][0], 7, 0))
        v = _xf_in([jnp.stack([left, d[3][0]])] + d + [jnp.stack([d[0][1], right])])
        for nu in range(6):
            tb[1 + g * T_ROWS + h % T_ROWS, :, nu] = v[nu]

    def in_col(c, g, r, nu):
        v = [_xf_in([tb[1 + g * T_ROWS + h % T_ROWS, p, nu] if 0 <= h < HW else None
                     for h in range(4 * r - 1, 4 * r + 5)]) for p in range(2)]
        for xi in range(6):
            vs[c % 2][1 + xi * 6 + nu, pl.ds(r % TR * 8, 8), _lanes(g)] = _pack(v[0][xi], v[1][xi])

    def in_groups(c, g):
        cv, b, r0 = c // 4, c // 2 % 2, c % 2 * TR
        row = lambda h: [_Item(in_row, cv, b, g, h, cost=80 if cv else 88, src=(xs, hs)[cv][b], dst=tb)]
        out = [] if r0 else [row(0)]
        for r in range(r0, r0 + TR + 1):
            rows = [row(h) for h in range(4 * r + 1, min(4 * r + 5, HW))] if r < r0 + TR else []
            cols = [[_Item(in_col, c, g, r - 1, nu, cost=42, src=tb, dst=vs[c % 2])]
                    for nu in range(6)] if r > r0 else []
            out += _alternate(rows, cols)
        if c > 1:
            out[0].insert(0, _Item(need, ("mm", (c - 1) * NG - 1)))
        out[-1].append(_Item(ready.add, ("in", c, g)))
        return out

    def out_first(phase, r, p, xi0, nxi, slot):
        y = _xf_out([ms[phase % N_RES][pl.ds(1 + nu * 6 + xi0, nxi), pl.ds(r % TR * 16 + p, 8, stride=2)]
                     for nu in range(6)])
        for j in range(4):
            osb[1 + slot * 4 + j, pl.ds(xi0, nxi)] = y[j]

    def out_second(acc, phase, r, p, jp, slot, rows):
        b, n = phase // 8 % 2, phase % NG
        y = _xf_out([None if (xi == 0 and 0 not in rows) or (xi == 5 and 3 not in rows) else
                     osb[pl.ds(1 + slot * 4 + 2 * jp, 2), xi] for xi in range(6)])
        if phase < 16:
            for i in rows:
                hs[b][1 + (4 * r + i) * NG + n, p, pl.ds(2 * jp, 2)] = y[i]
            s1 = (y[0] + y[1]) + (y[2] + y[3])
            s2 = (y[0] * y[0] + y[1] * y[1]) + (y[2] * y[2] + y[3] * y[3])
            acc[:] = acc[0] + (s1[0] + s1[1]), acc[1] + (s2[0] + s2[1])
        else:
            for i in rows:
                at = (*x_row(n, 4 * r + i), pl.ds(2 * p + jp, 8, stride=4))
                w = xs[b][at]
                xs[b][at] = _pack(_unpack(w, 0) + y[i][0], _unpack(w, 1) + y[i][1])

    sent = []

    def send(phase, i0=0, ni=4):
        b, r0, n = phase // 8 % 2, phase // 4 % 2 * TR, phase % NG
        sent.append(pltpu.make_async_copy(xs_bf[b].at[pl.ds(1 + n * 2 * TR + r0, TR), pl.ds(i0, ni)],
                                          o_hbm.at[b, pl.ds(r0, TR), pl.ds(i0, ni), :, _lanes(n)],
                                          sems.at[min(phase - 16, len(T_SENT))]))
        sent[-1].start()

    out_slot = [0]

    def out_groups(phase):
        b, r0, n = phase // 8 % 2, phase // 4 % 2 * TR, phase % NG
        acc, units = [], [(r, p) for r in range(r0, r0 + TR) for p in range(2)]

        def begin():
            need(("mm", phase))
            if phase < 16:
                acc.extend(stat[1 + b * NG + n, q] if r0 else jnp.zeros((8, 128), F32) for q in range(2))

        def end():
            ready.add(("out", phase))
            if phase < 16:
                stat[1 + b * NG + n, pl.ds(0, 2)] = jnp.stack(acc)
            else:
                send(phase)

        out = [[_Item(begin)]]
        for q in range(len(units) + 1):
            slot = out_slot[0] % 2
            first = [[_Item(out_first, phase, *units[q], xi0, 3, slot, cost=48, src=ms[phase % N_RES], dst=osb)]
                     for xi0 in (0, 3)] if q < len(units) else []
            second = [[_Item(out_second, acc, phase, *units[q - 1], jp, 1 - slot, (0, 1, 2, 3), cost=56,
                             src=osb, dst=(hs, xs)[phase // 16][b])] for jp in range(2)] if q else []
            out_slot[0] += bool(first)
            out += _alternate(first, second)
        out[-1].append(_Item(end))
        return out

    def last_out_items(xi0, nxi, rows):
        units, out = [(r, p) for r in range(TR, 2 * TR) for p in range(2)], []
        for q in range(len(units) + 2):
            if q < len(units):
                out.append(_Item(out_first, LAST, *units[q], xi0, nxi, 2 + q, cost=16 * nxi,
                                 src=ms[LAST % N_RES], dst=osb))
            if q >= 2 and rows:
                out += [_Item(out_second, None, LAST, *units[q - 2], jp, q, rows, cost=10 + 6 * len(rows),
                              dst=xs[1]) for jp in range(2)]
        return out

    def dot(lhs, rhs):
        return jax.lax.dot_general(pltpu.bitcast(lhs, BF16), pltpu.bitcast(rhs, BF16),
                                   (((1,), (1,)), ((), ())), preferred_element_type=F32)

    def matmul(phase, xi, nu, before):
        c, n = divmod(phase, NG)
        need(("in", c, NG - 1), ("w", c // 4, n, xi, NG - 1, 7), *[("out", phase - N_RES)] * (phase >= N_RES))
        lhs, = pace.load_blocks(vs[c % 2], [(1 + xi * 6 + nu, slice(None))], before)
        res = dot(lhs, us[c // 4][1 + n * 36 + nu * 6 + xi])
        ms[phase % N_RES][1 + nu * 6 + xi, pl.ds(0, M)] = res
        if xi == nu == 5:
            ready.add(("mm", phase))
        return res

    def matmul_part(g, ks, before):
        need(("in", 0, g), ("w", 0, 0, 5, g, 7))
        lhs = pace.load_blocks(vs[0], [(1 + k, _lanes(g)) for k in ks], before)
        for k, lhs_k in zip(ks, lhs):
            at = 1 + k % 6 * 6 + k // 6
            res = dot(lhs_k, us[0][at, :, _lanes(g)])
            res = ms[0][at, pl.ds(0, M)] + res if g else res
            ms[0][at, pl.ds(0, M)] = res
        if (g, ks[-1]) == (NG - 1, 35):
            ready.add(("mm", 0))
        return res

    def parts(g):
        return [functools.partial(matmul_part, g, range(k, k + 4)) for k in range(0, 36, 4)]

    def matmuls(phase, xis):
        return [functools.partial(matmul, phase, xi, nu) for xi in xis for nu in range(6)]

    wait(small)
    for q, ref in enumerate((g1_s, be1_s, g2_s, be2_s)):
        value = ref[...].astype(F32)
        for g in range(NG):
            affine[q, g] = jnp.broadcast_to(value[g * 128:(g + 1) * 128][None, :], (8, 128))
    for buf in (*xs, *hs, *wr, *us, *vs, *ms, tb, osb, stat):
        pace.clear(buf, 0)
        pace.clear(buf, 1)
    pace.zero = jax.lax.fori_loop(0, 2, lambda i, zero: zero + (i >> 10), jnp.int32(0))

    flat = lambda groups: [item for grp in groups for item in grp]
    for g, (top, bottom, weights) in enumerate(early):
        stats = flat(x_stat_groups(0, g))
        pace.run_alone([_Item(top.wait)] + stats[:HW // 4] + [_Item(bottom.wait)] + stats[HW // 4:-1])
        weights.wait()
        work = stats[-1:] + flat(w_groups(0, 0, [g], (0, 1, 2)) + w_groups(0, 0, [g], (3, 4, 5)) + in_groups(0, g))
        if g:
            pace.run(parts(g - 1), work, 450, 24, stretch=1.1)
            pace.restart()
        else:
            pace.run_alone(work)

    streams = [([[_Item(wait, copies)]], time, time) for time, copies in zip(T_WAIT, late)]
    streams += [([[_Item(lambda: sent.pop(0).wait())]], time, time) for time in T_SENT]
    groups = [grp for g in range(NG) for grp in in_groups(1, g)]
    cut = int(len(groups) * 0.67)
    streams += [(groups[:cut], 1, 3.5), (groups[cut:], 3.5, 3.98)]
    for c, window in enumerate(T_IN, 2):
        groups = []
        for g in range(NG):
            groups += [[_Item(h_stat_end, (c - 4) // 2, g, cost=30)]] if c in (4, 6) else []
            groups += in_groups(c, g)
        streams.append((groups, *window))
    streams.append(([grp for g in range(NG) for grp in x_stat_groups(1, g)], *T_STAT))
    for k, (start, middle, end) in enumerate(T_W, 1):
        streams += [(w_groups(k // NG, k % NG, range(NG), (0, 1, 2)), start, middle),
                    (w_groups(k // NG, k % NG, range(NG), (3, 4, 5)), middle, end)]
    for (p0, start), (p1, end) in zip(T_OUT, T_OUT[1:]):
        step = (end - start) / (p1 - p0)
        streams += [(out_groups(p), start + step * (p - p0), start + step * (p + 1 - p0)) for p in range(p0, p1)]
    streams.append((emb_groups(), *T_EMB))
    work = _interleave(streams)

    pace.run(parts(NG - 1), work[0] + work[1], 450, 24)
    for phase in range(1, LAST):
        for half, xis in enumerate(((0, 1, 2), (3, 4, 5))):
            pace.run(matmuls(phase, xis), work[2 * phase + half], *((450, 24) if phase < NG else (140, 28)))
    delayed = lambda items: [_Item(lambda: None, cost=sum(it.cost for it in items) // 5)] + items
    pace.run(matmuls(LAST, (1, 2, 3)), work[2 * LAST], 0, 40)
    pace.run(matmuls(LAST, (4,)), last_out_items(1, 2, ()), 0, 40)
    pace.run(matmuls(LAST, (0,)), delayed(last_out_items(3, 2, (1, 2))), 0, 40)
    pace.run(matmuls(LAST, (5,)), delayed(last_out_items(0, 1, (0,)) + [_Item(send, LAST, 0, 3)]), 0, 40)
    pace.run_alone(last_out_items(5, 1, (3,)) + [_Item(send, LAST, 3, 1)])
    wait(sent)


@jax.jit
def pallas_standalone__adm_resblock__diffusion_kernel(
    x: jax.Array,
    t_emb: jax.Array,
    g1: jax.Array,
    be1: jax.Array,
    w1: jax.Array,
    w_emb: jax.Array,
    g2: jax.Array,
    be2: jax.Array,
    w2: jax.Array,
):
    emb_dim = t_emb.shape[1]
    assert x.shape == (NB, C, HW, HW) and w1.shape == w2.shape == (C, C, 3, 3) and emb_dim % 128 == 0
    vmem = pltpu.VMEM
    scratch = (
        [vmem((1 + NG * HW // 4, 4, HW, 128), BF16)] * NB
        + [vmem((1 + HW * NG, 2, 4, 8, 128), F32)] * NB
        + [vmem((1 + NG * 9, C, 128), BF16)] * 2
        + [vmem((1 + NG * 36, 64, C), U32)] * 2
        + [vmem((1 + 36, M // 2, C), U32)] * 2
        + [vmem((1 + NG * T_ROWS, 2, 7, 8, 128), F32),
           vmem((1 + 18 * 4, 7, 8, 128), F32),
           vmem((2 * NB * NG, 2, 8, 128), F32),
           vmem((1 + NB * NG, 6, 8, 128), F32),
           vmem((NB, emb_dim), BF16)]
        + [vmem((C,), BF16)] * 4
        + [vmem((emb_dim, C), BF16), vmem((NB, C), F32), vmem((NB, 128, 128), F32),
           vmem((4, NG, 8, 128), F32), pltpu.SemaphoreType.DMA((3 * NG + 7,))]
        + [vmem((1 + 36, M_PITCH, 128), F32)] * N_RES
    )
    nhwc = (NB, HW // 4, 4, HW, C)
    taps = lambda w: jnp.transpose(w, (2, 3, 0, 1)).reshape(9, C, C)
    out = pl.pallas_call(
        _kernel,
        out_shape=jax.ShapeDtypeStruct(nhwc, x.dtype),
        in_specs=[pl.BlockSpec(memory_space=pl.ANY)] * 9,
        out_specs=pl.BlockSpec(memory_space=pl.ANY),
        scratch_shapes=scratch,
        compiler_params=pltpu.CompilerParams(vmem_limit_bytes=120 * 2 ** 20),
    )(jnp.transpose(x, (0, 2, 3, 1)).reshape(nhwc), t_emb, g1, be1, taps(w1), w_emb, g2, be2, taps(w2))
    return jnp.transpose(out.reshape(NB, HW, HW, C), (0, 3, 1, 2))
```

```python
import functools

import jax
import jax.numpy as jnp
from jax.experimental import pallas as pl
from jax.experimental.pallas import tpu as pltpu

F32, BF16, U32 = jnp.float32, jnp.bfloat16, jnp.uint32

NB, C, HW, NG = 2, 512, 64, 4
EPS = 1e-5
TR = 8
M = 16 * TR
M_PITCH = M + 8
N_RES = 6
T_ROWS = 33
TICKS = M // 8
LAST = 8 * NG - 1

PA, PB = 2.0 / 3.0, 1.5
A2, B2 = PA * PA, PB * PB
DD = A2 - B2

T_WAIT = (0, 1.5, 4, 8, 12, 16)
T_SENT = (20, 24)
T_IN = ((4.8, 7.98), (8, 11.98), (12, 15.98), (16, 19.98), (20, 23.98), (24, 27.98))
T_STAT, T_EMB = (4, 6.8), (4, 4.9)
T_W = ((0, 0.99, 1.47), (1.5, 1.97, 2.47), (2.5, 2.97, 3.47),
       (8, 9.5, 11), (11, 12.4, 13.8), (13.8, 15.2, 16.6), (16.6, 18, 19.47))
T_OUT = ((0, 4), (1, 4.8), (2, 6.8), (4, 8.2), (17, 19.5), (23, 24.04), (30, 31.04), (31, 31.49))


def _xf_in(d):
    p2, q2 = B2 * d[2], A2 * d[2]
    ea, eb = d[4] - p2, d[4] - q2
    p3, q3 = A2 * d[3], B2 * d[3]
    ua, ub = d[1] - p3, d[1] - q3
    v0 = (ea if d[0] is None else d[0] + ea) - q2
    v5 = (ua if d[5] is None else d[5] + ua) - q3
    oa, ob = PB * ua, PA * ub
    return [v0, ea - oa, ea + oa, eb - ob, eb + ob, v5]


def _xf_out(m):
    sa, da, sb, db = m[1] + m[2], m[1] - m[2], m[3] + m[4], m[3] - m[4]
    return [None if m[0] is None else (m[0] + sb) + sa, PA * da + PB * db, A2 * sa + B2 * sb,
            None if m[5] is None else (PA ** 3 * da + m[5]) + PB ** 3 * db]


def _xf_w(g):
    t = g[2] * (1.0 / (2 * DD))
    ea, eb = g[0] * (1.0 / (2 * A2 * DD)) + t, g[0] * (-1.0 / (2 * B2 * DD)) - t
    oa, ob = g[1] * (PB / (2 * DD)), g[1] * (-PA / (2 * DD))
    return [g[0], ea + oa, ea - oa, eb + ob, eb - ob, g[2]]


def _unpack(word, half):
    return pltpu.bitcast(word & jnp.uint32(0xFFFF0000) if half else word << 16, F32)


def _pack(lo, hi):
    bits = pltpu.bitcast(jnp.concatenate([lo, hi]).astype(BF16).astype(F32), U32)
    return (bits[:8] >> 16) | bits[8:]


def _operand(words):
    rows = words.shape[0] * 8
    return pltpu.bitcast(jnp.concatenate([words[:, g].reshape(rows, 128) for g in range(words.shape[1])], axis=1), BF16)


def _mean_all(v):
    return jnp.sum(jnp.sum(v, axis=0, keepdims=True), axis=1, keepdims=True) * (1.0 / v.size)


def _lanes(g):
    return pl.ds(g * 128, 128)


class _Item:
    def __init__(self, fn, *args, cost=0, src=None, dst=None):
        self.run, self.cost, self.src, self.dst = functools.partial(fn, *args), cost, src, dst


def _interleave(streams):
    keyed = []
    for groups, start, end in streams:
        total, spent = max(sum(it.cost for grp in groups for it in grp), 1), 0
        for grp in groups:
            cost = sum(it.cost for it in grp)
            keyed.append((start + (end - start) * (spent + cost / 2) / total, len(keyed), grp))
            spent += cost
    halves = {}
    for time, _, grp in sorted(keyed, key=lambda t: t[:2]):
        halves.setdefault(int(2 * time), []).extend(grp)
    return halves


def _alternate(first, second):
    keyed = ([((q + 0.25) / len(first), grp) for q, grp in enumerate(first)]
             + [((q + 0.75) / len(second), grp) for q, grp in enumerate(second)])
    return [grp for _, grp in sorted(keyed, key=lambda t: t[0])]


class _Pacer:
    LEAD, RESULT_LAG = 16, 20

    def __init__(self):
        self.zero = 0
        self.restart()

    def restart(self):
        self.results, self.todo, self.due, self.finished, self.spent = [], [], {}, [], 0

    def _slot(self, buf, which):
        if buf.shape[-2] > 8:
            return (self.zero,) + (0,) * (len(buf.shape) - 3) + (pl.ds(8 * which, 8), _lanes(0))
        return (self.zero,) + (0,) * (len(buf.shape) - 4) + (which, pl.ds(0, 8), _lanes(0))

    def clear(self, buf, which=0):
        buf[self._slot(buf, which)] = jnp.zeros((8, 128), buf.dtype)

    def hold(self, buf, value):
        buf[self._slot(buf, 0)] = value if value.dtype == buf.dtype else pltpu.bitcast(value, buf.dtype)

    def _tick(self, t):
        return self.results[t // TICKS][t % TICKS * 8:t % TICKS * 8 + 8]

    def _emit(self, item):
        item.run()
        self.spent += item.cost
        if item.dst is not None:
            self.finished = self.finished[-31:] + [(self.spent, item.dst[self._slot(item.dst, 1)])]

    def _older(self, window):
        return [value for spent, value in self.finished if spent <= self.spent - window]

    def _advance(self, tick):
        while self.todo and len(self.results) * TICKS <= tick:
            now, before = len(self.results) * TICKS, {}
            for key in [key for key in self.due if key[0] < now + TICKS]:
                before.setdefault(max(key[0] - now, 0) // 2, []).append(self.due.pop(key))
            for block in range(0, TR if self.window else 0, 1 if self.window > 200 else 2):
                t = min(now + 2 * block - self.RESULT_LAG, now - 1)
                if t >= 0:
                    before.setdefault(block, []).append(self._tick(t))
            self.results.append(self.todo.pop(0)(before))

    def load_blocks(self, buf, where, before):
        cuts, out = sorted({0, TR} | set(before)), [[] for _ in where]
        for lo, hi in zip(cuts, cuts[1:]):
            for value in before.get(lo, ()):
                self.hold(buf, value)
            if lo in before and lo % 4 and self.window:
                self.clear(buf)
            for blocks, (k, slabs) in zip(out, where):
                blocks.append(buf[k, pl.ds(lo, hi - lo), slabs])
        return [jnp.concatenate(blocks, axis=0) for blocks in out]

    def run_alone(self, items, window=500):
        self.restart()
        for item in items:
            for value in self._older(window)[-1:] if item.src is not None else ():
                self.hold(item.src, value)
            self._emit(item)
        self.restart()

    def run(self, matmuls, items, window, slack, stretch=1.0):
        t0, span, self.window = len(self.results) * TICKS, len(matmuls) * TICKS, window
        total, spent, held = max(sum(it.cost for it in items), 1) / stretch, 0, {}
        self.todo.extend(matmuls)
        for item in items:
            start = t0 + int(spent / total * span) // 2 * 2 - self.LEAD
            spent += item.cost
            self._advance(start)
            if item.src is not None:
                if 0 <= start < t0 + span and held.get(id(item.src)) != start:
                    held[id(item.src)] = start
                    self.hold(item.src, self._tick(start))
                if window and self._older(window):
                    self.hold(item.src, self._older(window)[-1])
                elif window:
                    self.clear(item.src)
            self._emit(item)
            if item.dst is not None:
                end = t0 + int(spent / total * span) - self.LEAD + slack
                self.due[-(-end // 2) * 2, id(item.dst)] = self.finished[-1][1]
        self._advance(t0 + span)


def _kernel(x_hbm, t_hbm, g1_hbm, be1_hbm, w1_hbm, wemb_hbm, g2_hbm, be2_hbm, w2_hbm, o_hbm,
            xs0, xs1, h0, h1, wr1, wr2, u1, u2, v0, v1, tb, osb, coef, stat,
            t_s, g1_s, be1_s, g2_s, be2_s, wemb_s, emb_s, tcol, affine, sems, *ms):
    xs_bf, wr_bf = (xs0, xs1), (wr1, wr2)
    xs = tuple(r.bitcast(U32) for r in xs_bf)
    wr = tuple(r.bitcast(U32) for r in wr_bf)
    hs, us_bf, vs_bf = (h0, h1), (u1, u2), (v0, v1)
    us, vs = tuple(r.bitcast(U32) for r in us_bf), tuple(r.bitcast(U32) for r in vs_bf)
    pace = _Pacer()

    ready = set()

    def need(*keys):
        assert all(key in ready for key in keys), keys

    def x_copy(b, g, r0, nr, sem):
        return pltpu.make_async_copy(x_hbm.at[b, pl.ds(r0, nr), :, :, _lanes(g)],
                                     xs_bf[b].at[pl.ds(1 + g * 2 * TR + r0, nr)], sems.at[sem])

    def w_copy(cv, n0, n1, g, sem):
        rows = pl.ds(n0 * 128, (n1 - n0) * 128)
        return pltpu.make_async_copy((w1_hbm, w2_hbm)[cv].at[:, rows, _lanes(g)],
                                     wr_bf[cv].at[pl.ds(1 + g * 9, 9), rows], sems.at[sem])

    def wait(copies):
        for copy in copies:
            copy.wait()

    early = [[x_copy(0, g, 0, TR, 3 * g), x_copy(0, g, TR, TR, 3 * g + 1), w_copy(0, 0, 1, g, 3 * g + 2)]
             for g in range(NG)]
    small = [pltpu.make_async_copy(src, dst, sems.at[3 * NG]) for src, dst in
             ((g1_hbm, g1_s), (be1_hbm, be1_s), (g2_hbm, g2_s), (be2_hbm, be2_s), (t_hbm, t_s))]
    w_all = lambda cv, n0, n1, sem: [w_copy(cv, n0, n1, g, 3 * NG + sem) for g in range(NG)]
    late = [w_all(0, 1, 2, 1), w_all(0, 2, 4, 2),
            [x_copy(1, g, 0, 2 * TR, 3 * NG + 3) for g in range(NG)]
            + [pltpu.make_async_copy(wemb_hbm, wemb_s, sems.at[3 * NG + 3])],
            w_all(1, 0, 2, 4), w_all(1, 2, 3, 5), w_all(1, 3, 4, 6)]
    for copies in [early[0][:1], small, early[0][1:]] + early[1:] + late:
        for copy in copies:
            copy.start()

    def w_rows(cv, n, g, ob, xis):
        w = [wr[cv][pl.ds(1 + g * 9 + 3 * i, 3), pl.ds(n * 64 + ob * 8, 8)] for i in range(3)]
        c = _xf_w([pltpu.bitcast(wi, BF16).astype(F32) for wi in w])
        for xi in xis:
            ready.add(("w", cv, n, xi, g, ob))
            u = _xf_w([c[xi][j] for j in range(3)])
            for nu in range(6):
                us_bf[cv][1 + n * 36 + nu * 6 + xi, ob, g] = u[nu].astype(BF16)

    def w_groups(cv, n, gs, xis):
        return [[_Item(w_rows, cv, n, g, ob, xis, cost=138, src=wr[cv], dst=us[cv])]
                for g in gs for ob in range(8)]

    def set_coef(cv, b, g, mean, var, bias):
        mu = _mean_all(mean)
        dev = mean - mu
        scale = affine[2 * cv, g] * jax.lax.rsqrt(_mean_all(jnp.maximum(var, 0.0) + dev * dev) + EPS)
        shift = affine[2 * cv + 1, g] + (bias - mu) * scale
        coef[(cv * NB + b) * NG + g] = jnp.stack([0.5 * shift, 0.5 * scale])
        ready.add(("coef", cv, b, g))

    def x_row(g, h):
        return 1 + g * 2 * TR + h // 4, h % 4

    def x_stat_rows(acc, b, g, h0):
        for h in (h0, h0 + 1):
            w = xs[b][x_row(g, h)].reshape(2, 2, 8, 128)
            lo, hi = _unpack(w, 0), _unpack(w, 1)
            if not acc:
                acc.append(lo[0])
            lo, hi = lo - acc[0], hi - acc[0]
            s1, s2 = lo + hi, lo * lo + hi * hi
            s1, s2 = s1[0] + s1[1], s2[0] + s2[1]
            acc[1:] = [acc[1] + s1, acc[2] + s2] if acc[1:] else [s1, s2]
        stat[0, pl.ds(2, 2)], stat[0, pl.ds(4, 2)] = acc[1:]

    def x_stat_end(acc, b, g):
        m1, m2 = acc[1] * (1.0 / (HW * 4)), acc[2] * (1.0 / (HW * 4))
        set_coef(0, b, g, (acc[0] + m1).reshape(16, 128), (m2 - m1 * m1).reshape(16, 128), 0.0)

    def x_stat_groups(b, g):
        acc = []
        return ([[_Item(x_stat_rows, acc, b, g, h0, cost=80, src=xs[b], dst=stat)] for h0 in range(0, HW, 2)]
                + [[_Item(x_stat_end, acc, b, g, cost=30)]])

    def h_stat_end(b, g):
        need("emb", ("out", (2 * b + 1) * NG + g))
        m = stat[1 + b * NG + g, pl.ds(0, 2)] * (1.0 / (HW * 8))
        e = emb_s[pl.ds(b, 1), _lanes(g)]
        set_coef(1, b, g, m[0] + e, m[1] - m[0] * m[0], e)

    def emb_rows(acc, e0):
        if e0 % 128 == 0:
            t = t_s[:, pl.ds(e0, 128)].astype(F32)
            t = t * jax.nn.sigmoid(t)
            for b in range(NB):
                tcol[b] = jnp.broadcast_to(t[b:b + 1], (128, 128)).T
        for e in range(e0, e0 + 32, 8):
            w = wemb_s[pl.ds(e, 8)].astype(F32)
            for b in range(NB):
                term = w * jnp.concatenate([tcol[b, pl.ds(e % 128, 8)]] * NG, axis=1)
                acc[b] = acc[b] + term if b in acc else term
        stat[0, pl.ds(2, NG)] = jnp.stack([acc[NB - 1][:, g * 128:(g + 1) * 128] for g in range(NG)])

    def emb_end(acc):
        for b in range(NB):
            emb_s[pl.ds(b, 1)] = jnp.sum(acc[b], axis=0, keepdims=True)
        ready.add("emb")

    def emb_groups():
        acc = {}
        return ([[_Item(emb_rows, acc, e0, cost=84, dst=stat)] for e0 in range(0, t_s.shape[1], 32)]
                + [[_Item(emb_end, acc, cost=40)]])

    sublane = jax.lax.broadcasted_iota(jnp.int32, (8, 128), 0)

    def in_row(cv, b, g, h):
        need(("coef", cv, b, g))
        shift, scale = (coef[(cv * NB + b) * NG + g, q] for q in range(2))

        def silu(z):
            u = z * scale + shift
            return u + u * jnp.tanh(u)

        if cv == 0:
            w = jnp.concatenate([xs[b][(*x_row(g, h), pl.ds(jp, 8, stride=4))] for jp in range(4)])
            lo, hi = (silu(_unpack(w.reshape(2, 2, 8, 128), half)) for half in range(2))
            d = [lo[:, 0], hi[:, 0], lo[:, 1], hi[:, 1]]
        else:
            a = silu(hs[b][1 + h * NG + g])
            d = [a[:, j] for j in range(4)]
        left = jnp.where(sublane == 0, 0.0, pltpu.roll(d[3][1], 1, 0))
        right = jnp.where(sublane == 7, 0.0, pltpu.roll(d[0][0], 7, 0))
        v = _xf_in([jnp.stack([left, d[3][0]])] + d + [jnp.stack([d[0][1], right])])
        for nu in range(6):
            tb[1 + g * T_ROWS + h % T_ROWS, :, nu] = v[nu]

    def in_col(c, g, r, nu):
        v = _xf_in([tb[1 + g * T_ROWS + h % T_ROWS, :, nu].reshape(16, 128) if 0 <= h < HW else None
                    for h in range(4 * r - 1, 4 * r + 5)])
        for xi in range(6):
            vs_bf[c % 2][1 + xi * 6 + nu, r % TR, g] = v[xi].astype(BF16)

    def in_groups(c, g):
        cv, b, r0 = c // 4, c // 2 % 2, c % 2 * TR
        row = lambda h: [_Item(in_row, cv, b, g, h, cost=80 if cv else 88, src=(xs, hs)[cv][b], dst=tb)]
        out = [] if r0 else [row(0)]
        for r in range(r0, r0 + TR + 1):
            rows = [row(h) for h in range(4 * r + 1, min(4 * r + 5, HW))] if r < r0 + TR else []
            cols = [[_Item(in_col, c, g, r - 1, nu, cost=42, src=tb, dst=vs[c % 2])]
                    for nu in range(6)] if r > r0 else []
            out += _alternate(rows, cols)
        if c > 1:
            out[0].insert(0, _Item(need, ("mm", (c - 1) * NG - 1)))
        out[-1].append(_Item(ready.add, ("in", c, g)))
        return out

    def out_first(phase, r, p, xi0, nxi, slot):
        y = _xf_out([ms[phase % N_RES][pl.ds(1 + nu * 6 + xi0, nxi), pl.ds(r % TR * 16 + p * 8, 8)]
                     for nu in range(6)])
        for j in range(4):
            osb[1 + slot * 4 + j, pl.ds(xi0, nxi)] = y[j]

    def out_second(acc, phase, r, p, jp, slot, rows):
        b, n = phase // 8 % 2, phase % NG
        y = _xf_out([None if (xi == 0 and 0 not in rows) or (xi == 5 and 3 not in rows) else
                     osb[pl.ds(1 + slot * 4 + 2 * jp, 2), xi] for xi in range(6)])
        if phase < 16:
            for i in rows:
                hs[b][1 + (4 * r + i) * NG + n, p, pl.ds(2 * jp, 2)] = y[i]
            s1 = (y[0] + y[1]) + (y[2] + y[3])
            s2 = (y[0] * y[0] + y[1] * y[1]) + (y[2] * y[2] + y[3] * y[3])
            acc[:] = acc[0] + (s1[0] + s1[1]), acc[1] + (s2[0] + s2[1])
        else:
            for i in rows:
                at = (*x_row(n, 4 * r + i), pl.ds(2 * p + jp, 8, stride=4))
                w = xs[b][at]
                xs[b][at] = _pack(_unpack(w, 0) + y[i][0], _unpack(w, 1) + y[i][1])

    sent = []

    def send(phase, i0=0, ni=4):
        b, r0, n = phase // 8 % 2, phase // 4 % 2 * TR, phase % NG
        sent.append(pltpu.make_async_copy(xs_bf[b].at[pl.ds(1 + n * 2 * TR + r0, TR), pl.ds(i0, ni)],
                                          o_hbm.at[b, pl.ds(r0, TR), pl.ds(i0, ni), :, _lanes(n)],
                                          sems.at[min(phase - 16, len(T_SENT))]))
        sent[-1].start()

    out_slot = [0]

    def out_groups(phase):
        b, r0, n = phase // 8 % 2, phase // 4 % 2 * TR, phase % NG
        acc, units = [], [(r, p) for r in range(r0, r0 + TR) for p in range(2)]

        def begin():
            need(("mm", phase))
            if phase < 16:
                acc.extend(stat[1 + b * NG + n, q] if r0 else jnp.zeros((8, 128), F32) for q in range(2))

        def end():
            ready.add(("out", phase))
            if phase < 16:
                stat[1 + b * NG + n, pl.ds(0, 2)] = jnp.stack(acc)
            else:
                send(phase)

        out = [[_Item(begin)]]
        for q in range(len(units) + 1):
            slot = out_slot[0] % 2
            first = [[_Item(out_first, phase, *units[q], xi0, 3, slot, cost=48, src=ms[phase % N_RES], dst=osb)]
                     for xi0 in (0, 3)] if q < len(units) else []
            second = [[_Item(out_second, acc, phase, *units[q - 1], jp, 1 - slot, (0, 1, 2, 3), cost=56,
                             src=osb, dst=(hs, xs)[phase // 16][b])] for jp in range(2)] if q else []
            out_slot[0] += bool(first)
            out += _alternate(first, second)
        out[-1].append(_Item(end))
        return out

    def last_out_items(xi0, nxi, rows):
        units, out = [(r, p) for r in range(TR, 2 * TR) for p in range(2)], []
        for q in range(len(units) + 2):
            if q < len(units):
                out.append(_Item(out_first, LAST, *units[q], xi0, nxi, 2 + q, cost=16 * nxi,
                                 src=ms[LAST % N_RES], dst=osb))
            if q >= 2 and rows:
                out += [_Item(out_second, None, LAST, *units[q - 2], jp, q, rows, cost=10 + 6 * len(rows),
                              dst=xs[1]) for jp in range(2)]
        return out

    def dot(lhs, rhs):
        return jax.lax.dot_general(_operand(lhs), _operand(rhs), (((1,), (1,)), ((), ())),
                                   preferred_element_type=F32)

    def matmul(phase, xi, nu, before):
        c, n = divmod(phase, NG)
        need(("in", c, NG - 1), ("w", c // 4, n, xi, NG - 1, 7), *[("out", phase - N_RES)] * (phase >= N_RES))
        lhs, = pace.load_blocks(vs[c % 2], [(1 + xi * 6 + nu, slice(None))], before)
        res = dot(lhs, us[c // 4][1 + n * 36 + nu * 6 + xi])
        ms[phase % N_RES][1 + nu * 6 + xi, pl.ds(0, M)] = res
        if xi == nu == 5:
            ready.add(("mm", phase))
        return res

    def matmul_part(g, ks, before):
        need(("in", 0, g), ("w", 0, 0, 5, g, 7))
        lhs = pace.load_blocks(vs[0], [(1 + k, pl.ds(g, 1)) for k in ks], before)
        for k, lhs_k in zip(ks, lhs):
            at = 1 + k % 6 * 6 + k // 6
            res = dot(lhs_k, us[0][at, :, pl.ds(g, 1)])
            res = ms[0][at, pl.ds(0, M)] + res if g else res
            ms[0][at, pl.ds(0, M)] = res
        if (g, ks[-1]) == (NG - 1, 35):
            ready.add(("mm", 0))
        return res

    def parts(g):
        return [functools.partial(matmul_part, g, range(k, k + 4)) for k in range(0, 36, 4)]

    def matmuls(phase, xis):
        return [functools.partial(matmul, phase, xi, nu) for xi in xis for nu in range(6)]

    wait(small)
    for q, ref in enumerate((g1_s, be1_s, g2_s, be2_s)):
        value = ref[...].astype(F32)
        for g in range(NG):
            affine[q, g] = jnp.broadcast_to(value[g * 128:(g + 1) * 128][None, :], (8, 128))
    for buf in (*xs, *hs, *wr, *us, *vs, *ms, tb, osb, stat):
        pace.clear(buf, 0)
        pace.clear(buf, 1)
    pace.zero = jax.lax.fori_loop(0, 2, lambda i, zero: zero + (i >> 10), jnp.int32(0))

    flat = lambda groups: [item for grp in groups for item in grp]
    for g, (top, bottom, weights) in enumerate(early):
        stats = flat(x_stat_groups(0, g))
        pace.run_alone([_Item(top.wait)] + stats[:HW // 4] + [_Item(bottom.wait)] + stats[HW // 4:-1])
        weights.wait()
        work = stats[-1:] + flat(w_groups(0, 0, [g], (0, 1, 2)) + w_groups(0, 0, [g], (3, 4, 5)) + in_groups(0, g))
        if g:
            pace.run(parts(g - 1), work, 450, 24, stretch=1.1)
            pace.restart()
        else:
            pace.run_alone(work)

    streams = [([[_Item(wait, copies)]], time, time) for time, copies in zip(T_WAIT, late)]
    streams += [([[_Item(lambda: sent.pop(0).wait())]], time, time) for time in T_SENT]
    groups = [grp for g in range(NG) for grp in in_groups(1, g)]
    cut = int(len(groups) * 0.67)
    streams += [(groups[:cut], 1, 3.5), (groups[cut:], 3.5, 3.98)]
    for c, window in enumerate(T_IN, 2):
        groups = []
        for g in range(NG):
            groups += [[_Item(h_stat_end, (c - 4) // 2, g, cost=30)]] if c in (4, 6) else []
            groups += in_groups(c, g)
        streams.append((groups, *window))
    streams.append(([grp for g in range(NG) for grp in x_stat_groups(1, g)], *T_STAT))
    for k, (start, middle, end) in enumerate(T_W, 1):
        streams += [(w_groups(k // NG, k % NG, range(NG), (0, 1, 2)), start, middle),
                    (w_groups(k // NG, k % NG, range(NG), (3, 4, 5)), middle, end)]
    for (p0, start), (p1, end) in zip(T_OUT, T_OUT[1:]):
        step = (end - start) / (p1 - p0)
        streams += [(out_groups(p), start + step * (p - p0), start + step * (p + 1 - p0)) for p in range(p0, p1)]
    streams.append((emb_groups(), *T_EMB))
    work = _interleave(streams)

    pace.run(parts(NG - 1), work[0] + work[1], 450, 24)
    for phase in range(1, LAST):
        for half, xis in enumerate(((0, 1, 2), (3, 4, 5))):
            window, slack = (450, 24) if phase < 4 else (110, 26) if phase < 24 else (0, 24)
            pace.run(matmuls(phase, xis), work[2 * phase + half], window, slack)
    delayed = lambda items: [_Item(lambda: None, cost=sum(it.cost for it in items) // 5)] + items
    pace.run(matmuls(LAST, (1, 2, 3)), work[2 * LAST], 0, 40)
    pace.run(matmuls(LAST, (4,)), last_out_items(1, 2, ()), 0, 40)
    pace.run(matmuls(LAST, (0,)), delayed(last_out_items(3, 2, (1, 2)) + [_Item(send, LAST, 1, 2)]), 0, 40)
    pace.run(matmuls(LAST, (5,)), delayed(last_out_items(0, 1, (0,)) + [_Item(send, LAST, 0, 1)]), 0, 40)
    pace.run_alone(last_out_items(5, 1, (3,)) + [_Item(send, LAST, 3, 1)])
    wait(sent)


@jax.jit
def pallas_standalone__adm_resblock__diffusion_kernel(
    x: jax.Array,
    t_emb: jax.Array,
    g1: jax.Array,
    be1: jax.Array,
    w1: jax.Array,
    w_emb: jax.Array,
    g2: jax.Array,
    be2: jax.Array,
    w2: jax.Array,
):
    emb_dim = t_emb.shape[1]
    assert x.shape == (NB, C, HW, HW) and w1.shape == w2.shape == (C, C, 3, 3) and emb_dim % 128 == 0
    vmem = pltpu.VMEM
    scratch = (
        [vmem((1 + NG * HW // 4, 4, HW, 128), BF16)] * NB
        + [vmem((1 + HW * NG, 2, 4, 8, 128), F32)] * NB
        + [vmem((1 + NG * 9, C, 128), BF16)] * 2
        + [vmem((1 + NG * 36, 8, NG, 16, 128), BF16)] * 2
        + [vmem((1 + 36, TR, NG, 16, 128), BF16)] * 2
        + [vmem((1 + NG * T_ROWS, 2, 7, 8, 128), F32),
           vmem((1 + 18 * 4, 7, 8, 128), F32),
           vmem((2 * NB * NG, 2, 8, 128), F32),
           vmem((1 + NB * NG, 6, 8, 128), F32),
           vmem((NB, emb_dim), BF16)]
        + [vmem((C,), BF16)] * 4
        + [vmem((emb_dim, C), BF16), vmem((NB, C), F32), vmem((NB, 128, 128), F32),
           vmem((4, NG, 8, 128), F32), pltpu.SemaphoreType.DMA((3 * NG + 7,))]
        + [vmem((1 + 36, M_PITCH, 128), F32)] * N_RES
    )
    nhwc = (NB, HW // 4, 4, HW, C)
    taps = lambda w: jnp.transpose(w, (2, 3, 0, 1)).reshape(9, C, C)
    out = pl.pallas_call(
        _kernel,
        out_shape=jax.ShapeDtypeStruct(nhwc, x.dtype),
        in_specs=[pl.BlockSpec(memory_space=pl.ANY)] * 9,
        out_specs=pl.BlockSpec(memory_space=pl.ANY),
        scratch_shapes=scratch,
        compiler_params=pltpu.CompilerParams(vmem_limit_bytes=120 * 2 ** 20),
    )(jnp.transpose(x, (0, 2, 3, 1)).reshape(nhwc), t_emb, g1, be1, taps(w1), w_emb, g2, be2, taps(w2))
    return jnp.transpose(out.reshape(NB, HW, HW, C), (0, 3, 1, 2))
```
